```python
import jax
import jax.numpy as jnp

def _softmax(x, axis=-1):
    return jax.nn.softmax(x, axis=axis)
def _gelu(x):
    return jax.nn.gelu(x, approximate=True)
def _silu(x):
    return jax.nn.silu(x)
def _sigmoid(x):
    return jax.nn.sigmoid(x)
def _layernorm(x, axis=-1, eps=1e-5):
    m = jnp.mean(x, axis=axis, keepdims=True)
    v = jnp.var(x, axis=axis, keepdims=True)
    return (x - m) / jnp.sqrt(v + eps)
def _scatter_add(tgt, idx, src, axis=0):
    return tgt.at[idx].add(src)
def _segment_sum(src, seg, n):
    return jax.ops.segment_sum(src, seg, n)
class _Rng:
    def __init__(self, key):
        self._k = key
    def _next(self):
        self._k, sub = jax.random.split(self._k)
        return sub
    def normal(self, shape):
        return jax.random.normal(self._next(), shape, dtype=jnp.bfloat16)
    def randint(self, lo, hi, shape):
        return jax.random.randint(self._next(), shape, lo, hi, dtype=jnp.int32)
    def uniform(self, shape, lo=0.0, hi=1.0):
        return jax.random.uniform(self._next(), shape, jnp.bfloat16, lo, hi)
    def permutation(self, n):
        return jax.random.permutation(self._next(), n)


kernel_name = 'interleave_layers__sliding_block__moe_arch_mod__prompt'

def setup_inputs():
    _rng = _Rng(jax.random.key(int.from_bytes(__import__("os").urandom(4), "little")))
    _w = (lambda a: (lambda t: t.astype(jnp.bfloat16) if jnp.issubdtype(t.dtype, jnp.floating) else t)(jnp.asarray(a)))
    def _A_setup():
        B, S, D = 1, 2048, 1024
        return {
            "x": _w((lambda *s: _rng.normal(s) * 0.05)(B, S, D)),
            "wqkv": _w((lambda *s: _rng.normal(s) * 0.05)(D, 3 * D)),
            "wo": _w((lambda *s: _rng.normal(s) * 0.05)(D, D)),
        }
    _A_in = _A_setup()

    def _B_setup():
        B, S, D, F, C = 1, 2048, 1024, 3584, 1
        return {
            "x": _w((lambda *s: _rng.normal(s) * 0.05)(B, S, D)),
            "w_r": _w((lambda *s: _rng.normal(s) * 0.05)(D)),
            "w_gate": _w((lambda *s: _rng.normal(s) * 0.05)(D, F)),
            "w_up": _w((lambda *s: _rng.normal(s) * 0.05)(D, F)),
            "w_down": _w((lambda *s: _rng.normal(s) * 0.05)(F, D)),
        }
    _B_in = _B_setup()

    return {
        "A_x": _A_in["x"],
        "A_wqkv": _A_in["wqkv"],
        "A_wo": _A_in["wo"],
        "B_x": _B_in["x"],
        "B_w_r": _B_in["w_r"],
        "B_w_gate": _B_in["w_gate"],
        "B_w_up": _B_in["w_up"],
        "B_w_down": _B_in["w_down"],
    }

def reference(A_x, A_wqkv, A_wo, B_x, B_w_r, B_w_gate, B_w_up, B_w_down):
    def _A_ref(x, wqkv, wo):
        B, S, D = x.shape
        H = 32; Dh = D // H; W = 256
        qkv = (lambda x, *d: x.transpose(*d))((x @ wqkv).reshape(B, S, 3, H, Dh), 2, 0, 3, 1, 4)
        q, k, v = qkv[0], qkv[1], qkv[2]
        scores = jnp.einsum("bhqd,bhkd->bhqk", q, k) * (Dh ** -0.5)
        idx = jnp.arange(S)
        mask = (idx[:, None] - idx[None, :] >= 0) & (idx[:, None] - idx[None, :] < W)
        scores = jnp.where(mask[None, None], scores, -1e9)
        p = _softmax(scores, axis=-1)
        o = jnp.einsum("bhqk,bhkd->bhqd", p, v)
        return (lambda x, *d: x.transpose(*d))(o, 0, 2, 1, 3).reshape(B, S, D) @ wo

    def _B_ref(x, w_r, w_gate, w_up, w_down):
        B, S, D = x.shape
        C = 1
        r = x @ w_r
        idx = jnp.argsort(-r, axis=-1)[:, :C]
        idx_e = jnp.repeat(idx.reshape(B, C, 1), D, axis=2)
        x_sel = jnp.take_along_axis(x, idx_e, axis=1)
        g = _silu(x_sel @ w_gate)
        u = x_sel @ w_up
        y = (g * u) @ w_down
        r_sel = _sigmoid(jnp.take_along_axis(r, idx, axis=1))
        y = y * r_sel.reshape(B, C, 1)
        b_off = (jnp.arange(B) * S).reshape(B, 1)
        flat_idx = (idx + b_off).reshape(B * C)
        zero = (x * 0.0).reshape(B * S, D)
        upd = _scatter_add(zero, flat_idx, y.reshape(B * C, D), axis=0)
        return x + upd.reshape(B, S, D)

    x = A_x
    x = x + _A_ref(_layernorm(x, axis=-1), A_wqkv, A_wo)
    x = x + _B_ref(_layernorm(x, axis=-1), B_w_r, B_w_gate, B_w_up, B_w_down)
    x = x + _A_ref(_layernorm(x, axis=-1), A_wqkv, A_wo)
    x = x + _B_ref(_layernorm(x, axis=-1), B_w_r, B_w_gate, B_w_up, B_w_down)
    return x
```

```python
import math

import jax
import jax.numpy as jnp
from jax import lax
import jax.experimental.pallas as pl
import jax.experimental.pallas.tpu as pltpu

S = 2048
D = 1024
NH = 32
DH = 32
FF = 3584
QB = 128
NQB = S // QB
MB = 256
NMB = S // MB
EPS = 1e-5
QSCALE = (DH ** -0.5) * math.log2(math.e)
NEG = -1e30
BIG = 2 ** 30

F32 = jnp.float32
BF16 = jnp.bfloat16
U32 = jnp.uint32
I32 = jnp.int32

NT = (((1,), (1,)), ((), ()))
TN = (((0,), (0,)), ((), ()))


def _rnd(v):
    return v.astype(BF16).astype(F32)


def _ln(xf):
    m = jnp.mean(xf, axis=-1, keepdims=True)
    xc = xf - m
    v = jnp.mean(xc * xc, axis=-1, keepdims=True)
    return xc * lax.rsqrt(v + EPS)


def _kernel(x_hbm, wqkv_hbm, wo_hbm, wr_ref, wg_hbm, wu_hbm, wd_hbm, out_hbm,
            xbuf, x1_u, h_u, q_u, k_u, vt_u, wqkv, wvt_u, wo, wg, wu, wd,
            s0, s1, p0, p1, p2, ot_u, ya, ysum, rmax_ref, ridx_ref, zs,
            sem_x, sem_w, sem_o):
    x1_b = x1_u.bitcast(BF16)
    h_b = h_u.bitcast(BF16)
    q_b = q_u.bitcast(BF16)
    k_b = k_u.bitcast(BF16)
    vt_b = vt_u.bitcast(BF16)
    wvt_b = wvt_u.bitcast(BF16)
    ot_b = ot_u.bitcast(BF16)
    sbufs = (s0, s1)
    pbufs_u = (p0, p1, p2)
    pbufs_b = tuple(p.bitcast(BF16) for p in pbufs_u)

    def x_copy(j):
        return pltpu.make_async_copy(x_hbm.at[pl.ds(j * MB, MB), :],
                                     xbuf.at[pl.ds(j * MB, MB), :], sem_x.at[j])

    w_copies = [
        pltpu.make_async_copy(wqkv_hbm, wqkv, sem_w.at[0]),
        pltpu.make_async_copy(wo_hbm, wo, sem_w.at[1]),
        pltpu.make_async_copy(wg_hbm, wg, sem_w.at[2]),
        pltpu.make_async_copy(wu_hbm, wu, sem_w.at[3]),
        pltpu.make_async_copy(wd_hbm, wd, sem_w.at[4]),
    ]
    x_copy(0).start()
    w_copies[0].start()
    for j in range(1, NMB):
        x_copy(j).start()

    for t in range(4):
        zs[t] = 0

    w_copies[0].wait()
    for j in range(NMB):
        x_copy(j).wait()
    for c in w_copies[1:]:
        c.start()

    eye = (lax.broadcasted_iota(I32, (128, 128), 0)
           == lax.broadcasted_iota(I32, (128, 128), 1)).astype(F32).astype(BF16)
    for t in range(D // 128):
        wv_t = wqkv[:, 2 * D + 128 * t:2 * D + 128 * (t + 1)]
        wvt_b[128 * t:128 * (t + 1), :] = lax.dot_general(
            eye, wv_t, NT, preferred_element_type=F32).astype(BF16)

    def ln1(src_row0, dst_row0):
        for c in range(MB // 64):
            xf = xbuf[pl.ds(src_row0 + 64 * c, 64), :].astype(F32)
            h_b[pl.ds(dst_row0 + 64 * c, 64), :] = _ln(xf).astype(BF16)

    def proj(base):
        h = h_b[pl.ds(base, MB), :]
        q = jnp.dot(h, wqkv[:, 0:D], preferred_element_type=F32)
        q_b[pl.ds(base, MB), :] = (q * QSCALE).astype(BF16)
        k = jnp.dot(h, wqkv[:, D:2 * D], preferred_element_type=F32)
        k_b[pl.ds(base, MB), :] = k.astype(BF16)
        vt = lax.dot_general(wvt_b[...], h, NT, preferred_element_type=F32)
        vt_b[:, pl.ds(base, MB)] = vt.astype(BF16)

    def phase_a():
        ln1(0, 0)

        def body(j, carry):
            base = pl.multiple_of(j * MB, MB)
            nxt = pl.multiple_of(jnp.minimum(j + 1, NMB - 1) * MB, MB)
            proj(base)
            ln1(nxt, base + MB)
            return carry

        lax.fori_loop(0, NMB, body, 0)

    def phase_b_iter(i, nkb, do_prev):
        zst = zs[0]
        zld = zs[1]
        zl2 = zs[2]
        r0 = i * QB if isinstance(i, int) else pl.multiple_of(i * QB, QB)

        lane = lax.broadcasted_iota(I32, (QB, QB), 1)
        row = lax.broadcasted_iota(I32, (QB, QB), 0)
        newmask = row <= lane
        l2 = lax.broadcasted_iota(I32, (QB // 2, QB), 1)
        r2 = lax.broadcasted_iota(I32, (QB // 2, QB), 0) * 2
        pm_new = (jnp.where(r2 <= l2, U32(0xFFFF), U32(0))
                  | jnp.where(r2 + 1 <= l2, U32(0xFFFF0000), U32(0)))
        pm_old = ~pm_new
        nrow = 128 if nkb == 1 else 256

        mx = {}
        rl = {}

        def qk(g):
            cs = slice(128 * g, 128 * (g + 1))
            q4u = pltpu.bitcast(q_b[pl.ds(r0, QB), cs], U32)
            qms = []
            for j in range(4):
                hm = jnp.where((l2 >= 32 * j) & (l2 < 32 * (j + 1)), U32(0xFFFFFFFF), U32(0))
                qms.append(pltpu.bitcast(q4u & hm, BF16))
            qm = jnp.concatenate(qms, axis=0)
            parts = []
            if nkb == 3:
                for c in range(8):
                    parts.append(k_b[pl.ds(r0 - 256 + 16 * c, 16), cs])
                    parts.append(k_b[pl.ds(r0 + 16 * c, 16), cs])
            else:
                parts.append(k_b[pl.ds(r0, 128), cs])
            if nkb >= 2:
                parts.append(k_b[pl.ds(r0 - 128, 128), cs])
            kk = jnp.concatenate(parts, axis=0)
            st = lax.dot_general(kk, qm, NT, preferred_element_type=F32)
            sref = sbufs[g % 2]
            for j in range(4):
                s = st[:, 128 * j:128 * (j + 1)]
                if nkb == 3:
                    fs = [jnp.where(newmask[16 * c:16 * c + 16], s[32 * c + 16:32 * c + 32],
                                    s[32 * c:32 * c + 16]) for c in range(8)]
                    f = jnp.concatenate(fs + [s[256:384]], axis=0)
                elif nkb == 2:
                    f = jnp.concatenate([jnp.where(newmask, s[0:128], NEG), s[128:256]], axis=0)
                else:
                    f = jnp.where(newmask, s, NEG)
                sref[zst + j, 0:nrow, :] = f
                mx[(g, j)] = jnp.max(f.reshape(nrow // 8, 8, 128), axis=0)

        def ex(g, j):
            m = jnp.broadcast_to(jnp.max(mx.pop((g, j)), axis=0, keepdims=True), (16, 128))
            sref = sbufs[g % 2]
            pref = pbufs_b[g % 3]
            z16 = pl.multiple_of(zst * 16, 16)
            for c in range(nrow // 16):
                p = jnp.exp2(sref[zld + j, 16 * c:16 * c + 16, :] - m)
                pref[pl.ds(z16 + 16 * c, 16), 128 * j:128 * (j + 1)] = p.astype(BF16)

        def pv(g, j):
            h = 4 * g + j
            pref = pbufs_u[g % 3]
            ls = slice(128 * j, 128 * (j + 1))
            z8 = pl.multiple_of(zld * 8, 8)
            pf = pref[pl.ds(z8, 64), ls]
            if nkb == 3:
                pmid = pref[pl.ds(z8 + 64, 64), ls]
                p = jnp.concatenate([pf & pm_old, pmid, pf & pm_new], axis=0)
                vt = vt_b[32 * h:32 * (h + 1), pl.ds(r0 - 256, 384)]
            elif nkb == 2:
                pmid = pref[pl.ds(z8 + 64, 64), ls]
                p = jnp.concatenate([pmid, pf], axis=0)
                vt = vt_b[32 * h:32 * (h + 1), pl.ds(r0 - 128, 256)]
            else:
                p = pf
                vt = vt_b[32 * h:32 * (h + 1), pl.ds(r0, 128)]
            ot = jnp.dot(vt, pltpu.bitcast(p, BF16), preferred_element_type=F32)
            z8b = pl.multiple_of(zl2 * 8, 8)
            pp = pref[pl.ds(z8b, nrow // 2), ls]
            x = (pltpu.bitcast(pp & U32(0xFFFF0000), F32)
                 + pltpu.bitcast(pp << 16, F32)).reshape(nrow // 16, 8, 128)
            while x.shape[0] > 1:
                n = x.shape[0] // 2
                x = x[:n] + x[n:]
            l = jnp.sum(x[0], axis=0, keepdims=True)
            o = (ot * (1.0 / l)).astype(BF16)
            ot_b[32 * (h % 16):32 * (h % 16) + 32, 128 * (h // 16):128 * (h // 16) + 128] = o

        def op_a():
            y = lax.dot_general(ot_b[:, 0:128], wo[0:512, :], TN, preferred_element_type=F32)
            ya[...] = y

        def op_b():
            y = lax.dot_general(ot_b[:, 128:256], wo[512:1024, :], TN,
                                preferred_element_type=F32)
            z8 = pl.multiple_of(zst * 8, 8)
            ysum[pl.ds(z8, QB), :] = y + ya[...]

        for s in range(10):
            if s < 8:
                qk(s)
            if s == 0 and do_prev:
                op_b()
                ln2(i - 1)
            if 1 <= s <= 8:
                for j in range(4):
                    ex(s - 1, j)
            if s == 8:
                op_a()
            if s >= 2:
                for j in range(4):
                    pv(s - 2, j)

    def op_b_tail():
        y = lax.dot_general(ot_b[:, 128:256], wo[512:1024, :], TN, preferred_element_type=F32)
        z8 = pl.multiple_of(zs[0] * 8, 8)
        ysum[pl.ds(z8, QB), :] = y + ya[...]

    def ln2(b):
        zld = zs[1]
        rb = b * QB if isinstance(b, int) else pl.multiple_of(b * QB, QB)
        wr = wr_ref[...].astype(F32)
        CH = 32
        bm = None
        bi = None
        sub = lax.broadcasted_iota(I32, (8, 1), 0)
        for c in range(QB // CH):
            z8 = pl.multiple_of(zld * 8, 8)
            a = _rnd(ysum[pl.ds(z8 + CH * c, CH), :])
            x0 = xbuf[pl.ds(rb + CH * c, CH), :].astype(F32)
            x1h = (x0 + a).astype(BF16)
            x1_b[pl.ds(rb + CH * c, CH), :] = x1h
            x1 = x1h.astype(F32)
            h2 = _rnd(_ln(x1))
            xbuf[pl.ds(rb + CH * c, CH), :] = (x1 + h2).astype(BF16)
            r = _rnd(jnp.sum(h2 * wr, axis=-1, keepdims=True))
            for t in range(CH // 8):
                rt = r[8 * t:8 * t + 8]
                it = sub + (rb + CH * c + 8 * t)
                if bm is None:
                    bm, bi = rt, it
                else:
                    better = rt > bm
                    bm = jnp.where(better, rt, bm)
                    bi = jnp.where(better, it, bi)
        om = rmax_ref[:, 0:1]
        oi = ridx_ref[:, 0:1]
        better = bm > om
        rmax_ref[:, 0:1] = jnp.where(better, bm, om)
        ridx_ref[:, 0:1] = jnp.where(better, bi, oi)

    def out_copy(b):
        return pltpu.make_async_copy(xbuf.at[pl.ds(b * QB, QB), :],
                                     out_hbm.at[pl.ds(b * QB, QB), :], sem_o.at[0])

    def phase_b(layer):
        rmax_ref[...] = jnp.full(rmax_ref.shape, -jnp.inf, F32)
        ridx_ref[...] = jnp.zeros(ridx_ref.shape, I32)
        phase_b_iter(0, 1, False)
        phase_b_iter(1, 2, True)

        def body(i, carry):
            @pl.when(layer == 1)
            def _():
                out_copy(i - 2).start()
            phase_b_iter(i, 3, True)
            return carry

        lax.fori_loop(2, NQB, body, 0)
        op_b_tail()
        ln2(NQB - 1)

        @pl.when(layer == 1)
        def _():
            out_copy(NQB - 2).start()
            out_copy(NQB - 1).start()

    def moe(layer):
        rm = rmax_ref[:, 0:1]
        ri = ridx_ref[:, 0:1]
        gm = jnp.max(rm, axis=0, keepdims=True)
        idx = jnp.min(jnp.where(rm == gm, ri, BIG))
        b16 = pl.multiple_of((idx // 16) * 16, 16)
        x1c = x1_b[pl.ds(b16, 16), :].astype(F32)
        h2c = _rnd(_ln(x1c))
        hb = h2c.astype(BF16)
        g = _rnd(jnp.dot(hb, wg[...], preferred_element_type=F32))
        u = _rnd(jnp.dot(hb, wu[...], preferred_element_type=F32))
        g = _rnd(g * _rnd(jax.nn.sigmoid(g)))
        act = (g * u).astype(BF16)
        y = _rnd(jnp.dot(act, wd[...], preferred_element_type=F32))
        y = _rnd(y * _rnd(jax.nn.sigmoid(gm)))
        x2n = x1c + _rnd(h2c + y)

        @pl.when(layer == 1)
        def _():
            for b in range(NQB):
                out_copy(b).wait()

        cur = xbuf[pl.ds(b16, 16), :].astype(F32)
        sel = lax.broadcasted_iota(I32, (16, D), 0) == (idx - b16)
        xbuf[pl.ds(b16, 16), :] = jnp.where(sel, x2n, cur).astype(BF16)

        @pl.when(layer == 1)
        def _():
            cp = pltpu.make_async_copy(xbuf.at[pl.ds(b16, 16), :],
                                       out_hbm.at[pl.ds(b16, 16), :], sem_o.at[1])
            cp.start()
            cp.wait()

    def layer_body(layer, carry):
        phase_a()

        @pl.when(layer == 0)
        def _():
            w_copies[1].wait()

        phase_b(layer)

        @pl.when(layer == 0)
        def _():
            for c in w_copies[2:]:
                c.wait()

        moe(layer)
        return carry

    lax.fori_loop(0, 2, layer_body, 0)


@jax.jit
def pallas_interleave_layers__sliding_block__moe_arch_mod__prompt_kernel(
    A_x: jax.Array,
    A_wqkv: jax.Array,
    A_wo: jax.Array,
    B_x: jax.Array,
    B_w_r: jax.Array,
    B_w_gate: jax.Array,
    B_w_up: jax.Array,
    B_w_down: jax.Array,
):
    del B_x
    hbm = pl.BlockSpec(memory_space=pl.ANY)
    scratch = [
        pltpu.VMEM((S, D), BF16),
        pltpu.VMEM((S // 2, D), U32),
        pltpu.VMEM(((S + MB) // 2, D), U32),
        pltpu.VMEM((S // 2, D), U32),
        pltpu.VMEM((S // 2, D), U32),
        pltpu.VMEM((D // 2, S), U32),
        pltpu.VMEM((D, 3 * D), BF16),
        pltpu.VMEM((D // 2, D), U32),
        pltpu.VMEM((D, D), BF16),
        pltpu.VMEM((D, FF), BF16),
        pltpu.VMEM((D, FF), BF16),
        pltpu.VMEM((FF, D), BF16),
        pltpu.VMEM((4, 256, 128), F32),
        pltpu.VMEM((4, 256, 128), F32),
        pltpu.VMEM((128, 512), U32),
        pltpu.VMEM((128, 512), U32),
        pltpu.VMEM((128, 512), U32),
        pltpu.VMEM((256, 256), U32),
        pltpu.VMEM((QB, D), F32),
        pltpu.VMEM((QB, D), F32),
        pltpu.VMEM((8, 128), F32),
        pltpu.VMEM((8, 128), I32),
        pltpu.SMEM((4,), I32),
        pltpu.SemaphoreType.DMA((NMB,)),
        pltpu.SemaphoreType.DMA((5,)),
        pltpu.SemaphoreType.DMA((2,)),
    ]
    out = pl.pallas_call(
        _kernel,
        out_shape=jax.ShapeDtypeStruct((S, D), BF16),
        in_specs=[hbm, hbm, hbm, pl.BlockSpec(memory_space=pltpu.VMEM), hbm, hbm, hbm],
        out_specs=hbm,
        scratch_shapes=scratch,
        compiler_params=pltpu.CompilerParams(vmem_limit_bytes=110 * 1024 * 1024),
        name="swa_moe_fused",
    )(A_x.reshape(S, D), A_wqkv, A_wo, B_w_r.reshape(1, D), B_w_gate, B_w_up, B_w_down)
    return out.reshape(1, S, D)
```

```python
import math

import jax
import jax.numpy as jnp
from jax import lax
import jax.experimental.pallas as pl
import jax.experimental.pallas.tpu as pltpu

S = 2048
D = 1024
NH = 32
DH = 32
WIN = 256
FF = 3584
QB = 128
NQB = S // QB
MB = 256
NMB = S // MB
EPS = 1e-5
QSCALE = (DH ** -0.5) * math.log2(math.e)
NEG = -1e30
BIG = 2 ** 30
L_LO = 2.0 ** -64
L_HI = 2.0 ** 64
F_MAX = 3.0e38

F32 = jnp.float32
BF16 = jnp.bfloat16
U32 = jnp.uint32
I32 = jnp.int32

NT = (((1,), (1,)), ((), ()))
TN = (((0,), (0,)), ((), ()))


def _rnd(v):
    return v.astype(BF16).astype(F32)


def _ln(xf):
    m = jnp.mean(xf, axis=-1, keepdims=True)
    xc = xf - m
    v = jnp.mean(xc * xc, axis=-1, keepdims=True)
    return xc * lax.rsqrt(v + EPS)


def _mo(v, m):
    return v if isinstance(v, int) else pl.multiple_of(v, m)


def _kernel(x_hbm, wqkv_hbm, wo_hbm, wr_ref, wg_hbm, wu_hbm, wd_hbm, out_hbm,
            xbuf, x1_u, h_u, qt_u, k_u, vt_u, wqkv, wqvt_u, wo, wg, wu, wd,
            p0, p1, p2, ot_u, ysum, rmax_ref, ridx_ref, zs, flag,
            sem_x, sem_w, sem_o):
    x1_b = x1_u.bitcast(BF16)
    h_b = h_u.bitcast(BF16)
    qt_b = qt_u.bitcast(BF16)
    k_b = k_u.bitcast(BF16)
    vt_b = vt_u.bitcast(BF16)
    wqvt_b = wqvt_u.bitcast(BF16)
    ot_b = ot_u.bitcast(BF16)
    pbufs_u = (p0, p1, p2)
    pbufs_b = tuple(p.bitcast(BF16) for p in pbufs_u)

    def x_copy(j):
        return pltpu.make_async_copy(x_hbm.at[pl.ds(j * MB, MB), :],
                                     xbuf.at[pl.ds(j * MB, MB), :], sem_x.at[j])

    def wqkv_copy(t):
        return pltpu.make_async_copy(wqkv_hbm.at[:, pl.ds(t * D, D)],
                                     wqkv.at[:, pl.ds(t * D, D)], sem_w.at[t])

    w_copies = [
        pltpu.make_async_copy(wo_hbm, wo, sem_w.at[3]),
        pltpu.make_async_copy(wg_hbm, wg, sem_w.at[4]),
        pltpu.make_async_copy(wu_hbm, wu, sem_w.at[5]),
        pltpu.make_async_copy(wd_hbm, wd, sem_w.at[6]),
    ]
    wqkv_copy(0).start()
    wqkv_copy(2).start()
    x_copy(0).start()
    wqkv_copy(1).start()
    for j in range(1, NMB):
        x_copy(j).start()

    for t in range(4):
        zs[t] = 0

    eye = (lax.broadcasted_iota(I32, (128, 128), 0)
           == lax.broadcasted_iota(I32, (128, 128), 1)).astype(F32).astype(BF16)

    def transpose_w(src_col0, dst_row0):
        for t in range(D // 128):
            w_t = wqkv[:, src_col0 + 128 * t:src_col0 + 128 * (t + 1)]
            wqvt_b[dst_row0 + 128 * t:dst_row0 + 128 * (t + 1), :] = lax.dot_general(
                eye, w_t, NT, preferred_element_type=F32).astype(BF16)

    wqkv_copy(0).wait()
    transpose_w(0, 0)
    wqkv_copy(2).wait()
    transpose_w(2 * D, D)
    wqkv_copy(1).wait()
    for j in range(NMB):
        x_copy(j).wait()
    for c in w_copies:
        c.start()

    def ln1(src_row0, dst_row0):
        src = xbuf.at[pl.ds(src_row0, MB), :]
        dst = h_b.at[pl.ds(dst_row0, MB), :]
        for c in range(MB // 64):
            xf = src[64 * c:64 * (c + 1), :].astype(F32)
            dst[64 * c:64 * (c + 1), :] = _ln(xf).astype(BF16)

    def proj(base):
        h = h_b[pl.ds(base, MB), :]
        k = jnp.dot(h, wqkv[:, D:2 * D], preferred_element_type=F32)
        k_b[pl.ds(base, MB), :] = k.astype(BF16)
        qv = lax.dot_general(wqvt_b[...], h, NT, preferred_element_type=F32)
        qt_b[:, pl.ds(base, MB)] = (qv[0:D] * QSCALE).astype(BF16)
        vt_b[:, pl.ds(base, MB)] = qv[D:2 * D].astype(BF16)

    def phase_a():
        ln1(0, 0)

        def body(j, carry):
            base = pl.multiple_of(j * MB, MB)
            nxt = pl.multiple_of(jnp.minimum(j + 1, NMB - 1) * MB, MB)
            proj(base)
            ln1(nxt, base + MB)
            return carry

        lax.fori_loop(0, NMB, body, 0)

    def ot_view(i):
        par = (i % 2) * 256
        return ot_b.at[:, pl.ds(_mo(par, 256), 256)]

    def attention(i, nkb, between):
        zst = zs[0]
        zld = zs[1]
        zl2 = zs[2]
        r0 = _mo(i * QB, QB)
        lane = lax.broadcasted_iota(I32, (QB, QB), 1)
        row = lax.broadcasted_iota(I32, (QB, QB), 0)
        newmask = row <= lane
        l2 = lax.broadcasted_iota(I32, (QB // 2, QB), 1)
        r2 = lax.broadcasted_iota(I32, (QB // 2, QB), 0) * 2
        pm_new = (jnp.where(r2 <= l2, U32(0xFFFF), U32(0))
                  | jnp.where(r2 + 1 <= l2, U32(0xFFFF0000), U32(0)))
        nrow = 128 if nkb == 1 else 256
        k0 = 128 * (nkb - 1)
        qw = qt_b.at[:, pl.ds(r0, QB)]
        kw = k_b.at[pl.ds(r0 - k0, k0 + QB), :]
        vw = vt_b.at[:, pl.ds(r0 - k0, k0 + QB)]
        ow = ot_view(i)
        p_st = [p.at[zst] for p in pbufs_b]
        p_ld = [p.at[zld] for p in pbufs_u]
        p_l2 = [p.at[zl2] for p in pbufs_u]
        zero32 = jnp.zeros((32, QB), BF16)
        good = [None]

        def qk(g):
            cs = slice(128 * g, 128 * (g + 1))
            ws = []
            for j in range(4):
                h = 4 * g + j
                ws.append(jnp.concatenate(
                    [zero32] * j + [qw[32 * h:32 * (h + 1), :]] + [zero32] * (3 - j), axis=0))
            w = jnp.concatenate(ws, axis=1)
            parts = []
            if nkb == 3:
                for c in range(8):
                    parts.append(kw[16 * c:16 * c + 16, cs])
                    parts.append(kw[256 + 16 * c:256 + 16 * c + 16, cs])
            else:
                parts.append(kw[k0:k0 + 128, cs])
            if nkb >= 2:
                parts.append(kw[k0 - 128:k0, cs])
            kk = jnp.concatenate(parts, axis=0)
            st = jnp.dot(kk, w, preferred_element_type=F32)
            pref = p_st[g % 3]
            for j in range(4):
                s = st[:, 128 * j:128 * (j + 1)]
                ls = slice(128 * j, 128 * (j + 1))
                for c in range(8):
                    nm = newmask[16 * c:16 * c + 16]
                    if nkb == 3:
                        f = jnp.where(nm, s[32 * c + 16:32 * c + 32], s[32 * c:32 * c + 16])
                    else:
                        f = jnp.where(nm, s[16 * c:16 * c + 16], NEG)
                    pref[16 * c:16 * c + 16, ls] = jnp.exp2(f).astype(BF16)
                if nkb >= 2:
                    o = 256 if nkb == 3 else 128
                    for c in range(8):
                        pref[128 + 16 * c:128 + 16 * c + 16, ls] = jnp.exp2(
                            s[o + 16 * c:o + 16 * c + 16]).astype(BF16)

        def pv(g, j):
            h = 4 * g + j
            pref = p_ld[g % 3]
            ls = slice(128 * j, 128 * (j + 1))
            pf = pref[0:64, ls]
            if nkb == 3:
                pnew = pf & pm_new
                p = jnp.concatenate([pf ^ pnew, pref[64:128, ls], pnew], axis=0)
            elif nkb == 2:
                p = jnp.concatenate([pref[64:128, ls], pf], axis=0)
            else:
                p = pf
            vt = vw[32 * h:32 * (h + 1), :]
            ot = jnp.dot(vt, pltpu.bitcast(p, BF16), preferred_element_type=F32)
            pp = p_l2[g % 3][0:nrow // 2, ls]
            x = (pltpu.bitcast(pp & U32(0xFFFF0000), F32)
                 + pltpu.bitcast(pp << 16, F32)).reshape(nrow // 16, 8, 128)
            while x.shape[0] > 1:
                n = x.shape[0] // 2
                x = x[:n] + x[n:]
            l = jnp.sum(x[0], axis=0, keepdims=True)
            am = jnp.max(jnp.abs(ot).reshape(4, 8, 128), axis=0)
            ok = (l >= L_LO) & (l <= L_HI) & (am <= F_MAX)
            good[0] = ok if good[0] is None else (good[0] & ok)
            o = (ot * (1.0 / l)).astype(BF16)
            ow[32 * (h % 16):32 * (h % 16) + 32, 128 * (h // 16):128 * (h // 16) + 128] = o

        for s in range(10):
            if s < 8:
                qk(s)
            if s >= 2:
                for j in range(4):
                    pv(s - 2, j)
        between()
        flag[0] = jnp.min(jnp.where(good[0], 1, 0))

    def attention_safe(i):
        r0 = _mo(i * QB, QB)
        start = pl.multiple_of(jnp.maximum(i - 2, 0) * QB, QB)
        qw = qt_b.at[:, pl.ds(r0, QB)]
        kw = k_b.at[pl.ds(start, 3 * QB), :]
        vw = vt_b.at[:, pl.ds(start, 3 * QB)]
        ow = ot_view(i)
        key = lax.broadcasted_iota(I32, (3 * QB, QB), 0) + start
        qry = lax.broadcasted_iota(I32, (3 * QB, QB), 1) + r0
        valid = (qry - key >= 0) & (qry - key < WIN)
        drow = lax.broadcasted_iota(I32, (128, QB), 0)

        def head(h, carry):
            g0 = pl.multiple_of((h // 4) * 128, 128)
            j0 = (h % 4) * 32
            q4 = qw[pl.ds(g0, 128), :].astype(F32)
            w = jnp.where((drow >= j0) & (drow < j0 + 32), q4, 0.0).astype(BF16)
            s = jnp.dot(kw[:, pl.ds(g0, 128)], w, preferred_element_type=F32)
            s = jnp.where(valid, s, NEG)
            m = jnp.max(s, axis=0, keepdims=True)
            p = jnp.exp2(s - m).astype(BF16)
            l = jnp.sum(p.astype(F32), axis=0, keepdims=True)
            vt = vw[pl.ds(pl.multiple_of(h * 32, 32), 32), :]
            o = jnp.dot(vt, p, preferred_element_type=F32) * (1.0 / l)
            ow[pl.ds(pl.multiple_of((h % 16) * 32, 32), 32),
               pl.ds(pl.multiple_of((h // 16) * 128, 128), 128)] = o.astype(BF16)
            return carry

        lax.fori_loop(0, NH, head, 0)

    def check(i):
        @pl.when(flag[0] == 0)
        def _():
            attention_safe(i)

    def out_proj(b):
        ow = ot_view(b)
        o = jnp.concatenate([ow[:, 0:128], ow[:, 128:256]], axis=0)
        ysum[...] = lax.dot_general(o, wo[...], TN, preferred_element_type=F32)

    def ln2(b):
        rb = _mo(b * QB, QB)
        wr = wr_ref[...].astype(F32)
        CH = 32
        xw = xbuf.at[pl.ds(rb, QB), :]
        x1w = x1_b.at[pl.ds(rb, QB), :]
        bm = None
        bi = None
        sub = lax.broadcasted_iota(I32, (8, 1), 0)
        for c in range(QB // CH):
            a = _rnd(ysum[CH * c:CH * (c + 1), :])
            x0 = xw[CH * c:CH * (c + 1), :].astype(F32)
            x1h = (x0 + a).astype(BF16)
            x1w[CH * c:CH * (c + 1), :] = x1h
            x1 = x1h.astype(F32)
            h2 = _rnd(_ln(x1))
            xw[CH * c:CH * (c + 1), :] = (x1 + h2).astype(BF16)
            r = _rnd(jnp.sum(h2 * wr, axis=-1, keepdims=True))
            for t in range(CH // 8):
                rt = r[8 * t:8 * t + 8]
                it = sub + (rb + CH * c + 8 * t)
                if bm is None:
                    bm, bi = rt, it
                else:
                    better = rt > bm
                    bm = jnp.where(better, rt, bm)
                    bi = jnp.where(better, it, bi)
        om = rmax_ref[:, 0:1]
        oi = ridx_ref[:, 0:1]
        better = bm > om
        rmax_ref[:, 0:1] = jnp.where(better, bm, om)
        ridx_ref[:, 0:1] = jnp.where(better, bi, oi)

    def out_copy(b):
        return pltpu.make_async_copy(xbuf.at[pl.ds(b * QB, QB), :],
                                     out_hbm.at[pl.ds(b * QB, QB), :], sem_o.at[0])

    def phase_b(layer):
        rmax_ref[...] = jnp.full(rmax_ref.shape, -jnp.inf, F32)
        ridx_ref[...] = jnp.zeros(ridx_ref.shape, I32)
        attention(0, 1, lambda: None)
        check(0)
        attention(1, 2, lambda: out_proj(0))

        def body(i, carry):
            check(i - 1)

            @pl.when(jnp.logical_and(layer == 1, i >= 3))
            def _():
                out_copy(i - 3).start()

            ln2(i - 2)
            attention(i, 3, lambda: out_proj(i - 1))
            return carry

        lax.fori_loop(2, NQB, body, 0)
        check(NQB - 1)
        ln2(NQB - 2)
        out_proj(NQB - 1)
        ln2(NQB - 1)

        @pl.when(layer == 1)
        def _():
            for b in range(NQB - 3, NQB):
                out_copy(b).start()

    def moe(layer):
        rm = rmax_ref[:, 0:1]
        ri = ridx_ref[:, 0:1]
        gm = jnp.max(rm, axis=0, keepdims=True)
        idx = jnp.min(jnp.where(rm == gm, ri, BIG))
        b16 = pl.multiple_of((idx // 16) * 16, 16)
        x1c = x1_b[pl.ds(b16, 16), :].astype(F32)
        h2c = _rnd(_ln(x1c))
        hb = h2c.astype(BF16)
        g = _rnd(jnp.dot(hb, wg[...], preferred_element_type=F32))
        u = _rnd(jnp.dot(hb, wu[...], preferred_element_type=F32))
        g = _rnd(g * _rnd(jax.nn.sigmoid(g)))
        act = (g * u).astype(BF16)
        y = _rnd(jnp.dot(act, wd[...], preferred_element_type=F32))
        y = _rnd(y * _rnd(jax.nn.sigmoid(gm)))
        x2n = x1c + _rnd(h2c + y)

        @pl.when(layer == 1)
        def _():
            for b in range(NQB):
                out_copy(b).wait()

        cur = xbuf[pl.ds(b16, 16), :].astype(F32)
        sel = lax.broadcasted_iota(I32, (16, D), 0) == (idx - b16)
        xbuf[pl.ds(b16, 16), :] = jnp.where(sel, x2n, cur).astype(BF16)

        @pl.when(layer == 1)
        def _():
            cp = pltpu.make_async_copy(xbuf.at[pl.ds(b16, 16), :],
                                       out_hbm.at[pl.ds(b16, 16), :], sem_o.at[1])
            cp.start()
            cp.wait()

    def layer_body(layer, carry):
        phase_a()

        @pl.when(layer == 0)
        def _():
            w_copies[0].wait()

        phase_b(layer)

        @pl.when(layer == 0)
        def _():
            for c in w_copies[1:]:
                c.wait()

        moe(layer)
        return carry

    lax.fori_loop(0, 2, layer_body, 0)


@jax.jit
def pallas_interleave_layers__sliding_block__moe_arch_mod__prompt_kernel(
    A_x: jax.Array,
    A_wqkv: jax.Array,
    A_wo: jax.Array,
    B_x: jax.Array,
    B_w_r: jax.Array,
    B_w_gate: jax.Array,
    B_w_up: jax.Array,
    B_w_down: jax.Array,
):
    del B_x
    hbm = pl.BlockSpec(memory_space=pl.ANY)
    scratch = [
        pltpu.VMEM((S, D), BF16),
        pltpu.VMEM((S // 2, D), U32),
        pltpu.VMEM(((S + MB) // 2, D), U32),
        pltpu.VMEM((D // 2, S), U32),
        pltpu.VMEM((S // 2, D), U32),
        pltpu.VMEM((D // 2, S), U32),
        pltpu.VMEM((D, 3 * D), BF16),
        pltpu.VMEM((D, D), U32),
        pltpu.VMEM((D, D), BF16),
        pltpu.VMEM((D, FF), BF16),
        pltpu.VMEM((D, FF), BF16),
        pltpu.VMEM((FF, D), BF16),
        pltpu.VMEM((1, 128, 512), U32),
        pltpu.VMEM((1, 128, 512), U32),
        pltpu.VMEM((1, 128, 512), U32),
        pltpu.VMEM((256, 512), U32),
        pltpu.VMEM((QB, D), F32),
        pltpu.VMEM((8, 128), F32),
        pltpu.VMEM((8, 128), I32),
        pltpu.SMEM((4,), I32),
        pltpu.SMEM((1,), I32),
        pltpu.SemaphoreType.DMA((NMB,)),
        pltpu.SemaphoreType.DMA((7,)),
        pltpu.SemaphoreType.DMA((2,)),
    ]
    out = pl.pallas_call(
        _kernel,
        out_shape=jax.ShapeDtypeStruct((S, D), BF16),
        in_specs=[hbm, hbm, hbm, pl.BlockSpec(memory_space=pltpu.VMEM), hbm, hbm, hbm],
        out_specs=hbm,
        scratch_shapes=scratch,
        compiler_params=pltpu.CompilerParams(vmem_limit_bytes=110 * 1024 * 1024),
        name="swa_moe_fused",
    )(A_x.reshape(S, D), A_wqkv, A_wo, B_w_r.reshape(1, D), B_w_gate, B_w_up, B_w_down)
    return out.reshape(1, S, D)
```

```python
import math

import jax
import jax.numpy as jnp
from jax import lax
import jax.experimental.pallas as pl
import jax.experimental.pallas.tpu as pltpu

S = 2048
D = 1024
NH = 32
DH = 32
WIN = 256
FF = 3584
QB = 128
NQB = S // QB
MB = 256
NMB = S // MB
EPS = 1e-5
QSCALE = (DH ** -0.5) * math.log2(math.e)
NEG = -1e30
BIG = 2 ** 30
L_LO = 2.0 ** -64
L_HI = 2.0 ** 64
F_MAX = 3.0e38

F32 = jnp.float32
BF16 = jnp.bfloat16
U32 = jnp.uint32
I32 = jnp.int32

NT = (((1,), (1,)), ((), ()))
TN = (((0,), (0,)), ((), ()))


def _rnd(v):
    return v.astype(BF16).astype(F32)


def _ln(xf):
    m = jnp.mean(xf, axis=-1, keepdims=True)
    xc = xf - m
    v = jnp.mean(xc * xc, axis=-1, keepdims=True)
    return xc * lax.rsqrt(v + EPS)


def _mo(v, m):
    return v if isinstance(v, int) else pl.multiple_of(v, m)


def _kernel(x_hbm, wqkv_hbm, wo_hbm, wr_ref, wg_hbm, wu_hbm, wd_hbm, out_hbm,
            xn_u, xres_u, x1_u, h0_u, h1_u, qt_u, k_u, vt_u,
            wqkv_u, wqvt_u, wo_u, wg_u, wu_u, wd_u,
            p0, p1, p2, ota_u, otb_u, y0, y1, bmax_ref, bidx_ref, zs, flag,
            sem_x, sem_w, sem_o):
    xn = xn_u.bitcast(BF16)
    xres = xres_u.bitcast(BF16)
    x1_b = x1_u.bitcast(BF16)
    hbufs = (h0_u.bitcast(BF16), h1_u.bitcast(BF16))
    qt_b = qt_u.bitcast(BF16)
    k_b = k_u.bitcast(BF16)
    vt_b = vt_u.bitcast(BF16)
    wqkv = wqkv_u.bitcast(BF16)
    wqvt = wqvt_u.bitcast(BF16)
    wo = wo_u.bitcast(BF16)
    wg = wg_u.bitcast(BF16)
    wu = wu_u.bitcast(BF16)
    wd = wd_u.bitcast(BF16)
    otbufs = (ota_u.bitcast(BF16), otb_u.bitcast(BF16))
    ybufs = (y0, y1)
    pbufs_u = (p0, p1, p2)
    pbufs_b = tuple(p.bitcast(BF16) for p in pbufs_u)

    def x_copy(j):
        return pltpu.make_async_copy(x_hbm.at[pl.ds(j * MB, MB), :],
                                     xn.at[pl.ds(j * MB, MB), :], sem_x.at[j])

    def wqkv_copy(t):
        return pltpu.make_async_copy(wqkv_hbm.at[:, pl.ds(t * D, D)],
                                     wqkv.at[:, pl.ds(t * D, D)], sem_w.at[t])

    w_copies = [
        pltpu.make_async_copy(wo_hbm, wo, sem_w.at[3]),
        pltpu.make_async_copy(wg_hbm, wg, sem_w.at[4]),
        pltpu.make_async_copy(wu_hbm, wu, sem_w.at[5]),
        pltpu.make_async_copy(wd_hbm, wd, sem_w.at[6]),
    ]
    wqkv_copy(0).start()
    wqkv_copy(2).start()
    x_copy(0).start()
    wqkv_copy(1).start()
    for j in range(1, NMB):
        x_copy(j).start()

    for t in range(4):
        zs[t] = 0

    eye = (lax.broadcasted_iota(I32, (128, 128), 0)
           == lax.broadcasted_iota(I32, (128, 128), 1)).astype(F32).astype(BF16)

    def transpose_w(src_col0, dst_row0):
        for t in range(D // 128):
            w_t = wqkv[:, src_col0 + 128 * t:src_col0 + 128 * (t + 1)]
            wqvt[dst_row0 + 128 * t:dst_row0 + 128 * (t + 1), :] = lax.dot_general(
                eye, w_t, NT, preferred_element_type=F32).astype(BF16)

    wqkv_copy(0).wait()
    transpose_w(0, 0)
    wqkv_copy(2).wait()
    transpose_w(2 * D, D)
    wqkv_copy(1).wait()
    for j in range(NMB):
        x_copy(j).wait()
    for c in w_copies:
        c.start()

    def ln1(row0, dst):
        src = xn.at[pl.ds(row0, MB), :]
        res = xres.at[pl.ds(row0, MB), :]
        for c in range(MB // 64):
            xb = src[64 * c:64 * (c + 1), :]
            res[64 * c:64 * (c + 1), :] = xb
            dst[64 * c:64 * (c + 1), :] = _ln(xb.astype(F32)).astype(BF16)

    def proj(base, hsrc):
        h = hsrc[...]
        k = jnp.dot(h, wqkv[:, D:2 * D], preferred_element_type=F32)
        k_b[pl.ds(base, MB), :] = k.astype(BF16)
        qv = lax.dot_general(wqvt[...], h, NT, preferred_element_type=F32)
        qt_b[:, pl.ds(base, MB)] = (qv[0:D] * QSCALE).astype(BF16)
        vt_b[:, pl.ds(base, MB)] = qv[D:2 * D].astype(BF16)

    def phase_a():
        ln1(0, hbufs[0])

        def body(t, carry):
            b0 = pl.multiple_of(2 * t * MB, MB)
            b1 = pl.multiple_of(b0 + MB, MB)
            b2 = pl.multiple_of(jnp.minimum(2 * t + 2, NMB - 1) * MB, MB)
            proj(b0, hbufs[0])
            ln1(b1, hbufs[1])
            proj(b1, hbufs[1])
            ln1(b2, hbufs[0])
            return carry

        lax.fori_loop(0, NMB // 2, body, 0)

    def attention(blocks):
        zst = zs[0]
        zld = zs[1]
        zl2 = zs[2]
        lane = lax.broadcasted_iota(I32, (QB, QB), 1)
        row = lax.broadcasted_iota(I32, (QB, QB), 0)
        newmask = row <= lane
        l2 = lax.broadcasted_iota(I32, (QB // 2, QB), 1)
        r2 = lax.broadcasted_iota(I32, (QB // 2, QB), 0) * 2
        pm_new = (jnp.where(r2 <= l2, U32(0xFFFF), U32(0))
                  | jnp.where(r2 + 1 <= l2, U32(0xFFFF0000), U32(0)))
        p_st = [p.at[zst] for p in pbufs_b]
        p_ld = [p.at[zld] for p in pbufs_u]
        p_l2 = [p.at[zl2] for p in pbufs_u]
        zero32 = jnp.zeros((32, QB), BF16)
        good = [None] * len(blocks)
        views = []
        for (i, nkb) in blocks:
            r0 = _mo(i * QB, QB)
            k0 = 128 * (nkb - 1)
            views.append((qt_b.at[:, pl.ds(r0, QB)],
                          k_b.at[pl.ds(r0 - k0, k0 + QB), :],
                          vt_b.at[:, pl.ds(r0 - k0, k0 + QB)]))

        def qk(n, g, slot):
            nkb = blocks[n][1]
            k0 = 128 * (nkb - 1)
            qw, kw, _ = views[n]
            cs = slice(128 * g, 128 * (g + 1))
            ws = []
            for j in range(4):
                h = 4 * g + j
                ws.append(jnp.concatenate(
                    [zero32] * j + [qw[32 * h:32 * (h + 1), :]] + [zero32] * (3 - j), axis=0))
            w = jnp.concatenate(ws, axis=1)
            parts = []
            if nkb == 3:
                for c in range(8):
                    parts.append(kw[16 * c:16 * c + 16, cs])
                    parts.append(kw[256 + 16 * c:256 + 16 * c + 16, cs])
            else:
                parts.append(kw[k0:k0 + 128, cs])
            if nkb >= 2:
                parts.append(kw[k0 - 128:k0, cs])
            kk = jnp.concatenate(parts, axis=0)
            st = jnp.dot(kk, w, preferred_element_type=F32)
            pref = p_st[slot]
            for j in range(4):
                s = st[:, 128 * j:128 * (j + 1)]
                ls = slice(128 * j, 128 * (j + 1))
                for c in range(8):
                    nm = newmask[16 * c:16 * c + 16]
                    if nkb == 3:
                        f = jnp.where(nm, s[32 * c + 16:32 * c + 32], s[32 * c:32 * c + 16])
                    else:
                        f = jnp.where(nm, s[16 * c:16 * c + 16], NEG)
                    pref[16 * c:16 * c + 16, ls] = jnp.exp2(f).astype(BF16)
                if nkb >= 2:
                    o = 256 if nkb == 3 else 128
                    for c in range(8):
                        pref[128 + 16 * c:128 + 16 * c + 16, ls] = jnp.exp2(
                            s[o + 16 * c:o + 16 * c + 16]).astype(BF16)

        def pv(n, g, j, slot):
            nkb = blocks[n][1]
            nrow = 128 if nkb == 1 else 256
            vw = views[n][2]
            h = 4 * g + j
            pref = p_ld[slot]
            ls = slice(128 * j, 128 * (j + 1))
            pf = pref[0:64, ls]
            if nkb == 3:
                pnew = pf & pm_new
                p = jnp.concatenate([pf ^ pnew, pref[64:128, ls], pnew], axis=0)
            elif nkb == 2:
                p = jnp.concatenate([pref[64:128, ls], pf], axis=0)
            else:
                p = pf
            vt = vw[32 * h:32 * (h + 1), :]
            ot = jnp.dot(vt, pltpu.bitcast(p, BF16), preferred_element_type=F32)
            pp = p_l2[slot][0:nrow // 2, ls]
            x = (pltpu.bitcast(pp & U32(0xFFFF0000), F32)
                 + pltpu.bitcast(pp << 16, F32)).reshape(nrow // 16, 8, 128)
            while x.shape[0] > 1:
                m = x.shape[0] // 2
                x = x[:m] + x[m:]
            l = jnp.sum(x[0], axis=0, keepdims=True)
            am = jnp.max(jnp.abs(ot).reshape(4, 8, 128), axis=0)
            ok = (l >= L_LO) & (l <= L_HI) & (am <= F_MAX)
            good[n] = ok if good[n] is None else (good[n] & ok)
            o = (ot * (1.0 / l)).astype(BF16)
            otbufs[n][32 * (h % 16):32 * (h % 16) + 32,
                      128 * (h // 16):128 * (h // 16) + 128] = o

        seq = [(n, g) for n in range(len(blocks)) for g in range(8)]
        for s in range(len(seq) + 2):
            if s < len(seq):
                qk(seq[s][0], seq[s][1], s % 3)
            if s >= 2:
                for j in range(4):
                    pv(seq[s - 2][0], seq[s - 2][1], j, (s - 2) % 3)
        for n in range(len(blocks)):
            flag[n] = jnp.min(jnp.where(good[n], 1, 0))

    def attention_safe(i, ow):
        r0 = _mo(i * QB, QB)
        start = pl.multiple_of(jnp.maximum(i - 2, 0) * QB, QB)
        qw = qt_b.at[:, pl.ds(r0, QB)]
        kw = k_b.at[pl.ds(start, 3 * QB), :]
        vw = vt_b.at[:, pl.ds(start, 3 * QB)]
        key = lax.broadcasted_iota(I32, (3 * QB, QB), 0) + start
        qry = lax.broadcasted_iota(I32, (3 * QB, QB), 1) + r0
        valid = (qry - key >= 0) & (qry - key < WIN)
        drow = lax.broadcasted_iota(I32, (128, QB), 0)

        def head(h, carry):
            g0 = pl.multiple_of((h // 4) * 128, 128)
            j0 = (h % 4) * 32
            q4 = qw[pl.ds(g0, 128), :].astype(F32)
            w = jnp.where((drow >= j0) & (drow < j0 + 32), q4, 0.0).astype(BF16)
            s = jnp.dot(kw[:, pl.ds(g0, 128)], w, preferred_element_type=F32)
            s = jnp.where(valid, s, NEG)
            m = jnp.max(s, axis=0, keepdims=True)
            p = jnp.exp2(s - m).astype(BF16)
            l = jnp.sum(p.astype(F32), axis=0, keepdims=True)
            vt = vw[pl.ds(pl.multiple_of(h * 32, 32), 32), :]
            o = jnp.dot(vt, p, preferred_element_type=F32) * (1.0 / l)
            ow[pl.ds(pl.multiple_of((h % 16) * 32, 32), 32),
               pl.ds(pl.multiple_of((h // 16) * 128, 128), 128)] = o.astype(BF16)
            return carry

        lax.fori_loop(0, NH, head, 0)

    def out_proj(n):
        ow = otbufs[n]
        o = jnp.concatenate([ow[:, 0:128], ow[:, 128:256]], axis=0)
        ybufs[n][zs[0]] = lax.dot_general(o, wo[...], TN, preferred_element_type=F32)

    def ln2(b, n, CH=16, NCHAIN=2):
        rb = _mo(b * QB, QB)
        wr = wr_ref[...].astype(F32)
        x1w = x1_b.at[pl.ds(rb, QB), :]
        x2w = xn.at[pl.ds(rb, QB), :]
        bm = None
        bi = None
        sub = lax.broadcasted_iota(I32, (8, 1), 0)
        toks = []
        for c in range(QB // CH):
            z = toks[c - NCHAIN] if c >= NCHAIN else 0
            yw = ybufs[n].at[zs[1] + z]
            xw = xres.at[pl.ds(pl.multiple_of(rb + z * 16, 16), QB), :]
            x1 = xw[CH * c:CH * (c + 1), :].astype(F32) + yw[CH * c:CH * (c + 1), :]
            x1w[CH * c:CH * (c + 1), :] = x1.astype(BF16)
            h2 = _ln(x1)
            x2w[CH * c:CH * (c + 1), :] = (x1 + h2).astype(BF16)
            r = _rnd(jnp.sum(h2 * wr, axis=-1, keepdims=True))
            ru = lax.bitcast_convert_type(r, I32)
            toks.append(jnp.max(lax.shift_right_logical(lax.shift_right_logical(ru, 16), 16)))
            for t in range(CH // 8):
                rt = r[8 * t:8 * t + 8]
                it = sub + (rb + CH * c + 8 * t)
                if bm is None:
                    bm, bi = rt, it
                else:
                    better = rt > bm
                    bm = jnp.where(better, rt, bm)
                    bi = jnp.where(better, it, bi)
        bmax_ref[b] = jnp.broadcast_to(bm, (8, 128))
        bidx_ref[b] = jnp.broadcast_to(bi, (8, 128))

    def checks(i0):
        @pl.when(flag[0] == 0)
        def _():
            attention_safe(i0, otbufs[0])
            out_proj(0)
            ln2(i0, 0, NCHAIN=8)

        @pl.when(flag[1] == 0)
        def _():
            attention_safe(i0 + 1, otbufs[1])
            out_proj(1)

    def out_copy(b):
        return pltpu.make_async_copy(xn.at[pl.ds(b * QB, QB), :],
                                     out_hbm.at[pl.ds(b * QB, QB), :], sem_o.at[0])

    def phase_b(layer):
        attention([(0, 1), (1, 2)])
        out_proj(0)
        ln2(0, 0)
        out_proj(1)

        def body(t, carry):
            i0 = 2 * t
            checks(i0 - 2)

            @pl.when(layer == 1)
            def _():
                out_copy(i0 - 2).start()

            @pl.when(jnp.logical_and(layer == 1, t >= 2))
            def _():
                out_copy(i0 - 3).start()

            attention([(i0, 3), (i0 + 1, 3)])
            ln2(i0 - 1, 1)
            out_proj(0)
            ln2(i0, 0)
            out_proj(1)
            return carry

        lax.fori_loop(1, NQB // 2, body, 0)
        checks(NQB - 2)
        ln2(NQB - 1, 1, NCHAIN=8)

        @pl.when(layer == 1)
        def _():
            for b in range(NQB - 3, NQB):
                out_copy(b).start()

    def moe(layer):
        rm = bmax_ref[:, :, 0:1]
        ri = bidx_ref[:, :, 0:1]
        gm = jnp.max(jnp.max(rm, axis=0), axis=0, keepdims=True)
        idx = jnp.min(jnp.where(rm == gm, ri, BIG))
        b16 = pl.multiple_of((idx // 16) * 16, 16)
        x1c = x1_b[pl.ds(b16, 16), :].astype(F32)
        h2c = _rnd(_ln(x1c))
        hb = h2c.astype(BF16)
        g = _rnd(jnp.dot(hb, wg[...], preferred_element_type=F32))
        u = _rnd(jnp.dot(hb, wu[...], preferred_element_type=F32))
        g = _rnd(g * _rnd(jax.nn.sigmoid(g)))
        act = (g * u).astype(BF16)
        y = _rnd(jnp.dot(act, wd[...], preferred_element_type=F32))
        y = _rnd(y * _rnd(jax.nn.sigmoid(gm)))
        x2n = x1c + _rnd(h2c + y)

        @pl.when(layer == 1)
        def _():
            for b in range(NQB):
                out_copy(b).wait()

        cur = xn[pl.ds(b16, 16), :].astype(F32)
        sel = lax.broadcasted_iota(I32, (16, D), 0) == (idx - b16)
        xn[pl.ds(b16, 16), :] = jnp.where(sel, x2n, cur).astype(BF16)

        @pl.when(layer == 1)
        def _():
            cp = pltpu.make_async_copy(xn.at[pl.ds(b16, 16), :],
                                       out_hbm.at[pl.ds(b16, 16), :], sem_o.at[1])
            cp.start()
            cp.wait()

    def layer_body(layer, carry):
        phase_a()

        @pl.when(layer == 0)
        def _():
            w_copies[0].wait()

        phase_b(layer)

        @pl.when(layer == 0)
        def _():
            for c in w_copies[1:]:
                c.wait()

        moe(layer)
        return carry

    lax.fori_loop(0, 2, layer_body, 0)


@jax.jit
def pallas_interleave_layers__sliding_block__moe_arch_mod__prompt_kernel(
    A_x: jax.Array,
    A_wqkv: jax.Array,
    A_wo: jax.Array,
    B_x: jax.Array,
    B_w_r: jax.Array,
    B_w_gate: jax.Array,
    B_w_up: jax.Array,
    B_w_down: jax.Array,
):
    del B_x
    hbm = pl.BlockSpec(memory_space=pl.ANY)
    scratch = [
        pltpu.VMEM((S // 2, D), U32),
        pltpu.VMEM((S // 2, D), U32),
        pltpu.VMEM((S // 2, D), U32),
        pltpu.VMEM((MB // 2, D), U32),
        pltpu.VMEM((MB // 2, D), U32),
        pltpu.VMEM((D // 2, S), U32),
        pltpu.VMEM((S // 2, D), U32),
        pltpu.VMEM((D // 2, S), U32),
        pltpu.VMEM((D // 2, 3 * D), U32),
        pltpu.VMEM((D, D), U32),
        pltpu.VMEM((D // 2, D), U32),
        pltpu.VMEM((D // 2, FF), U32),
        pltpu.VMEM((D // 2, FF), U32),
        pltpu.VMEM((FF // 2, D), U32),
        pltpu.VMEM((1, 128, 512), U32),
        pltpu.VMEM((1, 128, 512), U32),
        pltpu.VMEM((1, 128, 512), U32),
        pltpu.VMEM((256, 256), U32),
        pltpu.VMEM((256, 256), U32),
        pltpu.VMEM((1, QB, D), F32),
        pltpu.VMEM((1, QB, D), F32),
        pltpu.VMEM((NQB, 8, 128), F32),
        pltpu.VMEM((NQB, 8, 128), I32),
        pltpu.SMEM((4,), I32),
        pltpu.SMEM((2,), I32),
        pltpu.SemaphoreType.DMA((NMB,)),
        pltpu.SemaphoreType.DMA((7,)),
        pltpu.SemaphoreType.DMA((2,)),
    ]
    out = pl.pallas_call(
        _kernel,
        out_shape=jax.ShapeDtypeStruct((S, D), BF16),
        in_specs=[hbm, hbm, hbm, pl.BlockSpec(memory_space=pltpu.VMEM), hbm, hbm, hbm],
        out_specs=hbm,
        scratch_shapes=scratch,
        compiler_params=pltpu.CompilerParams(vmem_limit_bytes=110 * 1024 * 1024),
        name="swa_moe_fused",
    )(A_x.reshape(S, D), A_wqkv, A_wo, B_w_r.reshape(1, D), B_w_gate, B_w_up, B_w_down)
    return out.reshape(1, S, D)
```

```python
import math

import jax
import jax.numpy as jnp
from jax import lax
import jax.experimental.pallas as pl
import jax.experimental.pallas.tpu as pltpu

S = 2048
D = 1024
NH = 32
DH = 32
WIN = 256
FF = 3584
QB = 128
NQB = S // QB
MB = 256
NMB = S // MB
EPS = 1e-5
QSCALE = (DH ** -0.5) * math.log2(math.e)
NEG = -1e30
BIG = 2 ** 30
L_LO = 2.0 ** -64
L_HI = 2.0 ** 64
F_MAX = 3.0e38

F32 = jnp.float32
BF16 = jnp.bfloat16
U32 = jnp.uint32
I32 = jnp.int32

NT = (((1,), (1,)), ((), ()))
TN = (((0,), (0,)), ((), ()))


def _rnd(v):
    return v.astype(BF16).astype(F32)


def _ln(xf):
    m = jnp.mean(xf, axis=-1, keepdims=True)
    xc = xf - m
    v = jnp.mean(xc * xc, axis=-1, keepdims=True)
    return xc * lax.rsqrt(v + EPS)


def _mo(v, m):
    return v if isinstance(v, int) else pl.multiple_of(v, m)


def _kernel(x_hbm, wqkv_hbm, wo_hbm, wr_ref, wg_hbm, wu_hbm, wd_hbm, out_hbm,
            xn_u, xres_u, x1_u, h0_u, h1_u, qt_u, k_u, vt_u,
            wqkv_u, wqvt_u, wo_u, wg_u, wu_u, wd_u,
            p0, p1, p2, ota_u, otb_u, y0, y1, bmax_ref, bidx_ref, zs, flag,
            sem_x, sem_w, sem_o):
    xn = xn_u.bitcast(BF16)
    xres = xres_u.bitcast(BF16)
    x1_b = x1_u.bitcast(BF16)
    hbufs = (h0_u.bitcast(BF16), h1_u.bitcast(BF16))
    qt_b = qt_u.bitcast(BF16)
    k_b = k_u.bitcast(BF16)
    vt_b = vt_u.bitcast(BF16)
    wqkv = wqkv_u.bitcast(BF16)
    wqvt = wqvt_u.bitcast(BF16)
    wo = wo_u.bitcast(BF16)
    wg = wg_u.bitcast(BF16)
    wu = wu_u.bitcast(BF16)
    wd = wd_u.bitcast(BF16)
    otbufs = (ota_u.bitcast(BF16), otb_u.bitcast(BF16))
    ybufs = (y0, y1)
    pbufs_u = (p0, p1, p2)
    pbufs_b = tuple(p.bitcast(BF16) for p in pbufs_u)

    def x_copy(j):
        return pltpu.make_async_copy(x_hbm.at[pl.ds(j * MB, MB), :],
                                     xn.at[pl.ds(j * MB, MB), :], sem_x.at[j])

    def wqkv_copy(t):
        return pltpu.make_async_copy(wqkv_hbm.at[:, pl.ds(t * D, D)],
                                     wqkv.at[:, pl.ds(t * D, D)], sem_w.at[t])

    w_copies = [
        pltpu.make_async_copy(wo_hbm, wo, sem_w.at[3]),
        pltpu.make_async_copy(wg_hbm, wg, sem_w.at[4]),
        pltpu.make_async_copy(wu_hbm, wu, sem_w.at[5]),
        pltpu.make_async_copy(wd_hbm, wd, sem_w.at[6]),
    ]
    wqkv_copy(0).start()
    x_copy(0).start()
    wqkv_copy(2).start()
    x_copy(1).start()
    x_copy(2).start()
    wqkv_copy(1).start()
    for j in range(3, NMB):
        x_copy(j).start()

    for t in range(4):
        zs[t] = 0

    eye = (lax.broadcasted_iota(I32, (128, 128), 0)
           == lax.broadcasted_iota(I32, (128, 128), 1)).astype(F32).astype(BF16)

    def transpose_w(src_col0, dst_row0):
        for t in range(D // 128):
            w_t = wqkv[:, src_col0 + 128 * t:src_col0 + 128 * (t + 1)]
            wqvt[dst_row0 + 128 * t:dst_row0 + 128 * (t + 1), :] = lax.dot_general(
                eye, w_t, NT, preferred_element_type=F32).astype(BF16)

    def ln1(row0, dst):
        src = xn.at[pl.ds(row0, MB), :]
        res = xres.at[pl.ds(row0, MB), :]
        for c in range(MB // 64):
            xb = src[64 * c:64 * (c + 1), :]
            res[64 * c:64 * (c + 1), :] = xb
            dst[64 * c:64 * (c + 1), :] = _ln(xb.astype(F32)).astype(BF16)

    def proj(base, hsrc):
        h = hsrc[...]
        qv = lax.dot_general(wqvt[...], h, NT, preferred_element_type=F32)
        qt_b[:, pl.ds(base, MB)] = (qv[0:D] * QSCALE).astype(BF16)
        vt_b[:, pl.ds(base, MB)] = qv[D:2 * D].astype(BF16)
        k = jnp.dot(h, wqkv[:, D:2 * D], preferred_element_type=F32)
        k_b[pl.ds(base, MB), :] = k.astype(BF16)

    def phase_a(layer):
        def body(t, carry):
            @pl.when(jnp.logical_and(layer == 0, t >= 1))
            def _():
                x_copy(2 * t + 1).wait()

            @pl.when(jnp.logical_and(layer == 0, jnp.logical_and(t >= 1, t < NMB // 2 - 1)))
            def _():
                x_copy(2 * t + 2).wait()

            b0 = pl.multiple_of(2 * t * MB, MB)
            b1 = pl.multiple_of(b0 + MB, MB)
            b2 = pl.multiple_of(jnp.minimum(2 * t + 2, NMB - 1) * MB, MB)
            proj(b0, hbufs[0])
            ln1(b1, hbufs[1])
            proj(b1, hbufs[1])
            ln1(b2, hbufs[0])
            return carry

        lax.fori_loop(0, NMB // 2, body, 0)

    wqkv_copy(0).wait()
    transpose_w(0, 0)
    x_copy(0).wait()
    ln1(0, hbufs[0])
    wqkv_copy(2).wait()
    transpose_w(2 * D, D)
    x_copy(1).wait()
    x_copy(2).wait()
    wqkv_copy(1).wait()
    for c in w_copies:
        c.start()

    def attention(blocks):
        zst = zs[0]
        zld = zs[1]
        zl2 = zs[2]
        lane = lax.broadcasted_iota(I32, (QB, QB), 1)
        row = lax.broadcasted_iota(I32, (QB, QB), 0)
        newmask = row <= lane
        l2 = lax.broadcasted_iota(I32, (QB // 2, QB), 1)
        r2 = lax.broadcasted_iota(I32, (QB // 2, QB), 0) * 2
        pm_new = (jnp.where(r2 <= l2, U32(0xFFFF), U32(0))
                  | jnp.where(r2 + 1 <= l2, U32(0xFFFF0000), U32(0)))
        p_st = [p.at[zst] for p in pbufs_b]
        p_ld = [p.at[zld] for p in pbufs_u]
        p_l2 = [p.at[zl2] for p in pbufs_u]
        zero32 = jnp.zeros((32, QB), BF16)
        good = [None] * len(blocks)
        views = []
        for (i, nkb) in blocks:
            r0 = _mo(i * QB, QB)
            k0 = 128 * (nkb - 1)
            views.append((qt_b.at[:, pl.ds(r0, QB)],
                          k_b.at[pl.ds(r0 - k0, k0 + QB), :],
                          vt_b.at[:, pl.ds(r0 - k0, k0 + QB)]))

        def qk(n, g, slot):
            nkb = blocks[n][1]
            k0 = 128 * (nkb - 1)
            qw, kw, _ = views[n]
            cs = slice(128 * g, 128 * (g + 1))
            ws = []
            for j in range(4):
                h = 4 * g + j
                ws.append(jnp.concatenate(
                    [zero32] * j + [qw[32 * h:32 * (h + 1), :]] + [zero32] * (3 - j), axis=0))
            w = jnp.concatenate(ws, axis=1)
            parts = []
            if nkb == 3:
                for c in range(8):
                    parts.append(kw[16 * c:16 * c + 16, cs])
                    parts.append(kw[256 + 16 * c:256 + 16 * c + 16, cs])
            else:
                parts.append(kw[k0:k0 + 128, cs])
            if nkb >= 2:
                parts.append(kw[k0 - 128:k0, cs])
            kk = jnp.concatenate(parts, axis=0)
            st = jnp.dot(kk, w, preferred_element_type=F32)
            pref = p_st[slot]
            for j in range(4):
                s = st[:, 128 * j:128 * (j + 1)]
                ls = slice(128 * j, 128 * (j + 1))
                for c in range(8):
                    nm = newmask[16 * c:16 * c + 16]
                    if nkb == 3:
                        f = jnp.where(nm, s[32 * c + 16:32 * c + 32], s[32 * c:32 * c + 16])
                    else:
                        f = jnp.where(nm, s[16 * c:16 * c + 16], NEG)
                    pref[16 * c:16 * c + 16, ls] = jnp.exp2(f).astype(BF16)
                if nkb >= 2:
                    o = 256 if nkb == 3 else 128
                    for c in range(8):
                        pref[128 + 16 * c:128 + 16 * c + 16, ls] = jnp.exp2(
                            s[o + 16 * c:o + 16 * c + 16]).astype(BF16)

        def pv(n, g, j, slot):
            nkb = blocks[n][1]
            nrow = 128 if nkb == 1 else 256
            vw = views[n][2]
            h = 4 * g + j
            pref = p_ld[slot]
            ls = slice(128 * j, 128 * (j + 1))
            pf = pref[0:64, ls]
            if nkb == 3:
                pnew = pf & pm_new
                p = jnp.concatenate([pf ^ pnew, pref[64:128, ls], pnew], axis=0)
            elif nkb == 2:
                p = jnp.concatenate([pref[64:128, ls], pf], axis=0)
            else:
                p = pf
            vt = vw[32 * h:32 * (h + 1), :]
            ot = jnp.dot(vt, pltpu.bitcast(p, BF16), preferred_element_type=F32)
            pp = p_l2[slot][0:nrow // 2, ls]
            x = (pltpu.bitcast(pp & U32(0xFFFF0000), F32)
                 + pltpu.bitcast(pp << 16, F32)).reshape(nrow // 16, 8, 128)
            while x.shape[0] > 1:
                m = x.shape[0] // 2
                x = x[:m] + x[m:]
            l = jnp.sum(x[0], axis=0, keepdims=True)
            am = jnp.max(jnp.abs(ot).reshape(4, 8, 128), axis=0)
            ok = (l >= L_LO) & (l <= L_HI) & (am <= F_MAX)
            good[n] = ok if good[n] is None else (good[n] & ok)
            o = (ot * (1.0 / l)).astype(BF16)
            otbufs[n][32 * (h % 16):32 * (h % 16) + 32,
                      128 * (h // 16):128 * (h // 16) + 128] = o

        seq = [(n, g) for n in range(len(blocks)) for g in range(8)]
        for s in range(len(seq) + 2):
            if s < len(seq):
                qk(seq[s][0], seq[s][1], s % 3)
            if s >= 2:
                for j in range(4):
                    pv(seq[s - 2][0], seq[s - 2][1], j, (s - 2) % 3)
        for n in range(len(blocks)):
            flag[n] = jnp.min(jnp.where(good[n], 1, 0))

    def attention_safe(i, ow):
        r0 = _mo(i * QB, QB)
        start = pl.multiple_of(jnp.maximum(i - 2, 0) * QB, QB)
        qw = qt_b.at[:, pl.ds(r0, QB)]
        kw = k_b.at[pl.ds(start, 3 * QB), :]
        vw = vt_b.at[:, pl.ds(start, 3 * QB)]
        key = lax.broadcasted_iota(I32, (3 * QB, QB), 0) + start
        qry = lax.broadcasted_iota(I32, (3 * QB, QB), 1) + r0
        valid = (qry - key >= 0) & (qry - key < WIN)
        drow = lax.broadcasted_iota(I32, (128, QB), 0)

        def head(h, carry):
            g0 = pl.multiple_of((h // 4) * 128, 128)
            j0 = (h % 4) * 32
            q4 = qw[pl.ds(g0, 128), :].astype(F32)
            w = jnp.where((drow >= j0) & (drow < j0 + 32), q4, 0.0).astype(BF16)
            s = jnp.dot(kw[:, pl.ds(g0, 128)], w, preferred_element_type=F32)
            s = jnp.where(valid, s, NEG)
            m = jnp.max(s, axis=0, keepdims=True)
            p = jnp.exp2(s - m).astype(BF16)
            l = jnp.sum(p.astype(F32), axis=0, keepdims=True)
            vt = vw[pl.ds(pl.multiple_of(h * 32, 32), 32), :]
            o = jnp.dot(vt, p, preferred_element_type=F32) * (1.0 / l)
            ow[pl.ds(pl.multiple_of((h % 16) * 32, 32), 32),
               pl.ds(pl.multiple_of((h // 16) * 128, 128), 128)] = o.astype(BF16)
            return carry

        lax.fori_loop(0, NH, head, 0)

    def out_proj(n):
        ow = otbufs[n]
        o = jnp.concatenate([ow[:, 0:128], ow[:, 128:256]], axis=0)
        ybufs[n][zs[0]] = lax.dot_general(o, wo[...], TN, preferred_element_type=F32)

    def ln2(b, n, CH=16, NCHAIN=2):
        rb = _mo(b * QB, QB)
        wr = wr_ref[...].astype(F32)
        x1w = x1_b.at[pl.ds(rb, QB), :]
        x2w = xn.at[pl.ds(rb, QB), :]
        bm = None
        bi = None
        sub = lax.broadcasted_iota(I32, (8, 1), 0)
        toks = []
        for c in range(QB // CH):
            z = toks[c - NCHAIN] if c >= NCHAIN else 0
            yw = ybufs[n].at[zs[1] + z]
            xw = xres.at[pl.ds(pl.multiple_of(rb + z * 16, 16), QB), :]
            x1 = xw[CH * c:CH * (c + 1), :].astype(F32) + yw[CH * c:CH * (c + 1), :]
            x1w[CH * c:CH * (c + 1), :] = x1.astype(BF16)
            h2 = _ln(x1)
            x2w[CH * c:CH * (c + 1), :] = (x1 + h2).astype(BF16)
            r = _rnd(jnp.sum(h2 * wr, axis=-1, keepdims=True))
            ru = lax.bitcast_convert_type(r, I32)
            toks.append(jnp.max(lax.shift_right_logical(lax.shift_right_logical(ru, 16), 16)))
            for t in range(CH // 8):
                rt = r[8 * t:8 * t + 8]
                it = sub + (rb + CH * c + 8 * t)
                if bm is None:
                    bm, bi = rt, it
                else:
                    better = rt > bm
                    bm = jnp.where(better, rt, bm)
                    bi = jnp.where(better, it, bi)
        bmax_ref[b] = jnp.broadcast_to(bm, (8, 128))
        bidx_ref[b] = jnp.broadcast_to(bi, (8, 128))

    def checks(i0):
        @pl.when(flag[0] == 0)
        def _():
            attention_safe(i0, otbufs[0])
            out_proj(0)
            ln2(i0, 0, NCHAIN=8)

        @pl.when(flag[1] == 0)
        def _():
            attention_safe(i0 + 1, otbufs[1])
            out_proj(1)

    def out_copy(b):
        return pltpu.make_async_copy(xn.at[pl.ds(b * QB, QB), :],
                                     out_hbm.at[pl.ds(b * QB, QB), :], sem_o.at[0])

    def phase_b(layer):
        attention([(0, 1), (1, 2)])
        out_proj(0)
        ln2(0, 0)
        out_proj(1)

        def body(t, carry):
            i0 = 2 * t
            checks(i0 - 2)

            @pl.when(layer == 1)
            def _():
                out_copy(i0 - 2).start()

            @pl.when(jnp.logical_and(layer == 1, t >= 2))
            def _():
                out_copy(i0 - 3).start()

            attention([(i0, 3), (i0 + 1, 3)])
            ln2(i0 - 1, 1)
            out_proj(0)
            ln2(i0, 0)
            out_proj(1)
            return carry

        lax.fori_loop(1, NQB // 2, body, 0)
        checks(NQB - 2)
        ln2(NQB - 1, 1, NCHAIN=8)

        @pl.when(layer == 1)
        def _():
            for b in range(NQB - 3, NQB):
                out_copy(b).start()

    def moe(layer):
        rm = bmax_ref[:, :, 0:1]
        ri = bidx_ref[:, :, 0:1]
        gm = jnp.max(jnp.max(rm, axis=0), axis=0, keepdims=True)
        idx = jnp.min(jnp.where(rm == gm, ri, BIG))
        b16 = pl.multiple_of((idx // 16) * 16, 16)
        x1c = x1_b[pl.ds(b16, 16), :].astype(F32)
        h2c = _rnd(_ln(x1c))
        hb = h2c.astype(BF16)
        g = _rnd(jnp.dot(hb, wg[...], preferred_element_type=F32))
        u = _rnd(jnp.dot(hb, wu[...], preferred_element_type=F32))
        g = _rnd(g * _rnd(jax.nn.sigmoid(g)))
        act = (g * u).astype(BF16)
        y = _rnd(jnp.dot(act, wd[...], preferred_element_type=F32))
        y = _rnd(y * _rnd(jax.nn.sigmoid(gm)))
        x2n = x1c + _rnd(h2c + y)

        @pl.when(layer == 1)
        def _():
            for b in range(NQB):
                out_copy(b).wait()

        cur = xn[pl.ds(b16, 16), :].astype(F32)
        sel = lax.broadcasted_iota(I32, (16, D), 0) == (idx - b16)
        xn[pl.ds(b16, 16), :] = jnp.where(sel, x2n, cur).astype(BF16)

        @pl.when(layer == 1)
        def _():
            cp = pltpu.make_async_copy(xn.at[pl.ds(b16, 16), :],
                                       out_hbm.at[pl.ds(b16, 16), :], sem_o.at[1])
            cp.start()
            cp.wait()

    def layer_body(layer, carry):
        phase_a(layer)

        @pl.when(layer == 0)
        def _():
            w_copies[0].wait()

        phase_b(layer)

        @pl.when(layer == 0)
        def _():
            for c in w_copies[1:]:
                c.wait()

        moe(layer)

        @pl.when(layer == 0)
        def _():
            ln1(0, hbufs[0])

        return carry

    lax.fori_loop(0, 2, layer_body, 0)


@jax.jit
def pallas_interleave_layers__sliding_block__moe_arch_mod__prompt_kernel(
    A_x: jax.Array,
    A_wqkv: jax.Array,
    A_wo: jax.Array,
    B_x: jax.Array,
    B_w_r: jax.Array,
    B_w_gate: jax.Array,
    B_w_up: jax.Array,
    B_w_down: jax.Array,
):
    del B_x
    hbm = pl.BlockSpec(memory_space=pl.ANY)
    scratch = [
        pltpu.VMEM((S // 2, D), U32),
        pltpu.VMEM((S // 2, D), U32),
        pltpu.VMEM((S // 2, D), U32),
        pltpu.VMEM((MB // 2, D), U32),
        pltpu.VMEM((MB // 2, D), U32),
        pltpu.VMEM((D // 2, S), U32),
        pltpu.VMEM((S // 2, D), U32),
        pltpu.VMEM((D // 2, S), U32),
        pltpu.VMEM((D // 2, 3 * D), U32),
        pltpu.VMEM((D, D), U32),
        pltpu.VMEM((D // 2, D), U32),
        pltpu.VMEM((D // 2, FF), U32),
        pltpu.VMEM((D // 2, FF), U32),
        pltpu.VMEM((FF // 2, D), U32),
        pltpu.VMEM((1, 128, 512), U32),
        pltpu.VMEM((1, 128, 512), U32),
        pltpu.VMEM((1, 128, 512), U32),
        pltpu.VMEM((256, 256), U32),
        pltpu.VMEM((256, 256), U32),
        pltpu.VMEM((1, QB, D), F32),
        pltpu.VMEM((1, QB, D), F32),
        pltpu.VMEM((NQB, 8, 128), F32),
        pltpu.VMEM((NQB, 8, 128), I32),
        pltpu.SMEM((4,), I32),
        pltpu.SMEM((2,), I32),
        pltpu.SemaphoreType.DMA((NMB,)),
        pltpu.SemaphoreType.DMA((7,)),
        pltpu.SemaphoreType.DMA((2,)),
    ]
    out = pl.pallas_call(
        _kernel,
        out_shape=jax.ShapeDtypeStruct((S, D), BF16),
        in_specs=[hbm, hbm, hbm, pl.BlockSpec(memory_space=pltpu.VMEM), hbm, hbm, hbm],
        out_specs=hbm,
        scratch_shapes=scratch,
        compiler_params=pltpu.CompilerParams(vmem_limit_bytes=110 * 1024 * 1024),
        name="swa_moe_fused",
    )(A_x.reshape(S, D), A_wqkv, A_wo, B_w_r.reshape(1, D), B_w_gate, B_w_up, B_w_down)
    return out.reshape(1, S, D)
```

```python
import math

import jax
import jax.numpy as jnp
from jax import lax
import jax.experimental.pallas as pl
import jax.experimental.pallas.tpu as pltpu

S = 2048
D = 1024
NH = 32
DH = 32
WIN = 256
FF = 3584
QB = 128
NQB = S // QB
MB = 256
NMB = S // MB
EPS = 1e-5
QSCALE = (DH ** -0.5) * math.log2(math.e)
NEG = -1e30
BIG = 2 ** 30
L_LO = 2.0 ** -64
L_HI = 2.0 ** 64
F_MAX = 3.0e38

F32 = jnp.float32
BF16 = jnp.bfloat16
U32 = jnp.uint32
I32 = jnp.int32

NT = (((1,), (1,)), ((), ()))
TN = (((0,), (0,)), ((), ()))


def _rnd(v):
    return v.astype(BF16).astype(F32)


def _ln(xf):
    m = jnp.mean(xf, axis=-1, keepdims=True)
    xc = xf - m
    v = jnp.mean(xc * xc, axis=-1, keepdims=True)
    return xc * lax.rsqrt(v + EPS)


def _mo(v, m):
    return v if isinstance(v, int) else pl.multiple_of(v, m)


def _kernel(x_hbm, wqkv_hbm, wo_hbm, wr_ref, wg_hbm, wu_hbm, wd_hbm, out_hbm,
            xn_u, xres_u, x1_u, h0_u, h1_u, qt_u, k_u, vt_u,
            wqkv_u, wqvt_u, wo_u, wg_u, wu_u, wd_u,
            p0, p1, p2, ot_u, ysum, bmax_ref, bidx_ref, zs, flag,
            sem_x, sem_w, sem_o):
    xn = xn_u.bitcast(BF16)
    xres = xres_u.bitcast(BF16)
    x1_b = x1_u.bitcast(BF16)
    hbufs = (h0_u.bitcast(BF16), h1_u.bitcast(BF16))
    qt_b = qt_u.bitcast(BF16)
    k_b = k_u.bitcast(BF16)
    vt_b = vt_u.bitcast(BF16)
    wqkv = wqkv_u.bitcast(BF16)
    wqvt = wqvt_u.bitcast(BF16)
    wo = wo_u.bitcast(BF16)
    wg = wg_u.bitcast(BF16)
    wu = wu_u.bitcast(BF16)
    wd = wd_u.bitcast(BF16)
    ot_b = ot_u.bitcast(BF16)
    otbufs = (ot_b.at[0], ot_b.at[1])
    pbufs_u = (p0, p1, p2)
    pbufs_b = tuple(p.bitcast(BF16) for p in pbufs_u)

    def x_copy(j):
        return pltpu.make_async_copy(x_hbm.at[pl.ds(j * MB, MB), :],
                                     xn.at[pl.ds(j * MB, MB), :], sem_x.at[j])

    def wqkv_copy(t):
        return pltpu.make_async_copy(wqkv_hbm.at[:, pl.ds(t * D, D)],
                                     wqkv.at[:, pl.ds(t * D, D)], sem_w.at[t])

    w_copies = [
        pltpu.make_async_copy(wo_hbm, wo, sem_w.at[3]),
        pltpu.make_async_copy(wg_hbm, wg, sem_w.at[4]),
        pltpu.make_async_copy(wu_hbm, wu, sem_w.at[5]),
        pltpu.make_async_copy(wd_hbm, wd, sem_w.at[6]),
    ]
    wqkv_copy(0).start()
    x_copy(0).start()
    wqkv_copy(2).start()
    x_copy(1).start()
    x_copy(2).start()
    wqkv_copy(1).start()
    for j in range(3, NMB):
        x_copy(j).start()

    for t in range(4):
        zs[t] = 0

    eye = (lax.broadcasted_iota(I32, (128, 128), 0)
           == lax.broadcasted_iota(I32, (128, 128), 1)).astype(F32).astype(BF16)

    def transpose_w(src_col0, dst_row0, tiles):
        for t in tiles:
            w_t = wqkv[:, src_col0 + 128 * t:src_col0 + 128 * (t + 1)]
            wqvt[dst_row0 + 128 * t:dst_row0 + 128 * (t + 1), :] = lax.dot_general(
                eye, w_t, NT, preferred_element_type=F32).astype(BF16)

    def ln1(row0, dst):
        src = xn.at[pl.ds(row0, MB), :]
        res = xres.at[pl.ds(row0, MB), :]
        for c in range(MB // 64):
            xb = src[64 * c:64 * (c + 1), :]
            res[64 * c:64 * (c + 1), :] = xb
            dst[64 * c:64 * (c + 1), :] = _ln(xb.astype(F32)).astype(BF16)

    def proj_q(base, hsrc):
        q = lax.dot_general(wqvt[0:D, :], hsrc[...], NT, preferred_element_type=F32)
        qt_b[:, pl.ds(base, MB)] = (q * QSCALE).astype(BF16)

    def proj_v(base, hsrc):
        v = lax.dot_general(wqvt[D:2 * D, :], hsrc[...], NT, preferred_element_type=F32)
        vt_b[:, pl.ds(base, MB)] = v.astype(BF16)

    def proj_qv(base, hsrc):
        qv = lax.dot_general(wqvt[...], hsrc[...], NT, preferred_element_type=F32)
        qt_b[:, pl.ds(base, MB)] = (qv[0:D] * QSCALE).astype(BF16)
        vt_b[:, pl.ds(base, MB)] = qv[D:2 * D].astype(BF16)

    def proj_k(base, hsrc):
        k = jnp.dot(hsrc[...], wqkv[:, D:2 * D], preferred_element_type=F32)
        k_b[pl.ds(base, MB), :] = k.astype(BF16)

    def phase_a(layer):
        def body(t, carry):
            first = jnp.logical_and(layer == 0, t == 0)

            @pl.when(first)
            def _():
                x_copy(1).wait()
                x_copy(2).wait()
                wqkv_copy(1).wait()
                for c in w_copies:
                    c.start()

            @pl.when(jnp.logical_and(layer == 0, t >= 1))
            def _():
                x_copy(2 * t + 1).wait()

            @pl.when(jnp.logical_and(layer == 0, jnp.logical_and(t >= 1, t < NMB // 2 - 1)))
            def _():
                x_copy(2 * t + 2).wait()

            b0 = pl.multiple_of(2 * t * MB, MB)
            b1 = pl.multiple_of(b0 + MB, MB)
            b2 = pl.multiple_of(jnp.minimum(2 * t + 2, NMB - 1) * MB, MB)

            @pl.when(jnp.logical_not(first))
            def _():
                proj_qv(b0, hbufs[0])

            proj_k(b0, hbufs[0])
            ln1(b1, hbufs[1])
            proj_qv(b1, hbufs[1])
            proj_k(b1, hbufs[1])
            ln1(b2, hbufs[0])
            return carry

        lax.fori_loop(0, NMB // 2, body, 0)

    wqkv_copy(0).wait()
    transpose_w(0, 0, range(0, 4))
    x_copy(0).wait()
    transpose_w(0, 0, range(4, 8))
    ln1(0, hbufs[0])
    proj_q(0, hbufs[0])
    wqkv_copy(2).wait()
    transpose_w(2 * D, D, range(8))
    proj_v(0, hbufs[0])

    def attention(blocks):
        zst = zs[0]
        zld = zs[1]
        zl2 = zs[2]
        lane = lax.broadcasted_iota(I32, (QB, QB), 1)
        row = lax.broadcasted_iota(I32, (QB, QB), 0)
        newmask = row <= lane
        l2 = lax.broadcasted_iota(I32, (QB // 2, QB), 1)
        r2 = lax.broadcasted_iota(I32, (QB // 2, QB), 0) * 2
        pm_new = (jnp.where(r2 <= l2, U32(0xFFFF), U32(0))
                  | jnp.where(r2 + 1 <= l2, U32(0xFFFF0000), U32(0)))
        p_st = [p.at[zst] for p in pbufs_b]
        p_ld = [p.at[zld] for p in pbufs_u]
        p_l2 = [p.at[zl2] for p in pbufs_u]
        zero32 = jnp.zeros((32, QB), BF16)
        good = [None] * len(blocks)
        views = []
        for (i, nkb) in blocks:
            r0 = _mo(i * QB, QB)
            k0 = 128 * (nkb - 1)
            views.append((qt_b.at[:, pl.ds(r0, QB)],
                          k_b.at[pl.ds(r0 - k0, k0 + QB), :],
                          vt_b.at[:, pl.ds(r0 - k0, k0 + QB)]))

        def qk(n, g, slot):
            nkb = blocks[n][1]
            k0 = 128 * (nkb - 1)
            qw, kw, _ = views[n]
            cs = slice(128 * g, 128 * (g + 1))
            ws = []
            for j in range(4):
                h = 4 * g + j
                ws.append(jnp.concatenate(
                    [zero32] * j + [qw[32 * h:32 * (h + 1), :]] + [zero32] * (3 - j), axis=0))
            w = jnp.concatenate(ws, axis=1)
            parts = []
            if nkb == 3:
                for c in range(8):
                    parts.append(kw[16 * c:16 * c + 16, cs])
                    parts.append(kw[256 + 16 * c:256 + 16 * c + 16, cs])
            else:
                parts.append(kw[k0:k0 + 128, cs])
            if nkb >= 2:
                parts.append(kw[k0 - 128:k0, cs])
            kk = jnp.concatenate(parts, axis=0)
            st = jnp.dot(kk, w, preferred_element_type=F32)
            pref = p_st[slot]
            for j in range(4):
                s = st[:, 128 * j:128 * (j + 1)]
                ls = slice(128 * j, 128 * (j + 1))
                for c in range(8):
                    nm = newmask[16 * c:16 * c + 16]
                    if nkb == 3:
                        f = jnp.where(nm, s[32 * c + 16:32 * c + 32], s[32 * c:32 * c + 16])
                    else:
                        f = jnp.where(nm, s[16 * c:16 * c + 16], NEG)
                    pref[16 * c:16 * c + 16, ls] = jnp.exp2(f).astype(BF16)
                if nkb >= 2:
                    o = 256 if nkb == 3 else 128
                    for c in range(8):
                        pref[128 + 16 * c:128 + 16 * c + 16, ls] = jnp.exp2(
                            s[o + 16 * c:o + 16 * c + 16]).astype(BF16)

        def pv(n, g, j, slot):
            nkb = blocks[n][1]
            nrow = 128 if nkb == 1 else 256
            vw = views[n][2]
            h = 4 * g + j
            pref = p_ld[slot]
            ls = slice(128 * j, 128 * (j + 1))
            pf = pref[0:64, ls]
            if nkb == 3:
                pnew = pf & pm_new
                p = jnp.concatenate([pf ^ pnew, pref[64:128, ls], pnew], axis=0)
            elif nkb == 2:
                p = jnp.concatenate([pref[64:128, ls], pf], axis=0)
            else:
                p = pf
            vt = vw[32 * h:32 * (h + 1), :]
            ot = jnp.dot(vt, pltpu.bitcast(p, BF16), preferred_element_type=F32)
            pp = p_l2[slot][0:nrow // 2, ls]
            x = (pltpu.bitcast(pp & U32(0xFFFF0000), F32)
                 + pltpu.bitcast(pp << 16, F32)).reshape(nrow // 16, 8, 128)
            while x.shape[0] > 1:
                m = x.shape[0] // 2
                x = x[:m] + x[m:]
            l = jnp.sum(x[0], axis=0, keepdims=True)
            am = jnp.max(jnp.abs(ot).reshape(4, 8, 128), axis=0)
            ok = (l >= L_LO) & (l <= L_HI) & (am <= F_MAX)
            good[n] = ok if good[n] is None else (good[n] & ok)
            o = (ot * (1.0 / l)).astype(BF16)
            otbufs[n][32 * (h % 16):32 * (h % 16) + 32,
                      128 * (h // 16):128 * (h // 16) + 128] = o

        l64 = lax.broadcasted_iota(I32, (16, QB), 1)
        lo16 = l64 < 64
        lo8 = lax.broadcasted_iota(I32, (8, QB), 1) < 64
        lo1 = lax.broadcasted_iota(I32, (1, QB), 1) < 64
        t64 = lax.broadcasted_iota(I32, (64, QB), 0)
        s64 = lax.broadcasted_iota(I32, (64, QB), 1) & 63
        new64 = t64 <= s64
        r32 = lax.broadcasted_iota(I32, (32, QB), 0) * 2
        c32 = lax.broadcasted_iota(I32, (32, QB), 1)
        lo32 = c32 < 64
        pn64 = (jnp.where(r32 <= (c32 & 63), U32(0xFFFF), U32(0))
                | jnp.where(r32 + 1 <= (c32 & 63), U32(0xFFFF0000), U32(0)))
        po64 = ~pn64
        zu = U32(0)

        def qk2(n, g, slot):
            qw, kw, _ = views[n]
            cs = slice(128 * g, 128 * (g + 1))
            pref = p_st[slot]
            for a in range(2):
                he = 4 * g + 2 * a
                xe = pltpu.bitcast(qw[32 * he:32 * he + 32, :], U32)
                xo = pltpu.roll(pltpu.bitcast(qw[32 * he + 32:32 * he + 64, :], U32), 64, 1)
                for u in range(2):
                    me = lo16 if u == 0 else jnp.logical_not(lo16)
                    wt = pltpu.bitcast(jnp.concatenate(
                        [jnp.where(me, xe, zu), jnp.where(me, zu, xo)], axis=0), BF16)
                    w = jnp.concatenate([zero32] * (2 * a) + [wt] + [zero32] * (2 - 2 * a), axis=0)
                    parts = []
                    for c in range(4):
                        parts.append(kw[64 * u + 16 * c:64 * u + 16 * c + 16, cs])
                        parts.append(kw[64 * u + 256 + 16 * c:64 * u + 256 + 16 * c + 16, cs])
                    parts.append(kw[64 * u + 64:64 * u + 256, cs])
                    s = jnp.dot(jnp.concatenate(parts, axis=0), w, preferred_element_type=F32)
                    ls = slice(128 * (2 * a + u), 128 * (2 * a + u + 1))
                    for c in range(4):
                        f = jnp.where(new64[16 * c:16 * c + 16], s[32 * c + 16:32 * c + 32],
                                      s[32 * c:32 * c + 16])
                        pref[16 * c:16 * c + 16, ls] = jnp.exp2(f).astype(BF16)
                    for c in range(12):
                        pref[64 + 16 * c:64 + 16 * c + 16, ls] = jnp.exp2(
                            s[128 + 16 * c:128 + 16 * c + 16]).astype(BF16)

        def colsum(pp):
            x = (pltpu.bitcast(pp & U32(0xFFFF0000), F32)
                 + pltpu.bitcast(pp << 16, F32)).reshape(pp.shape[0] // 8, 8, 128)
            while x.shape[0] > 1:
                m = x.shape[0] // 2
                x = x[:m] + x[m:]
            return jnp.sum(x[0], axis=0, keepdims=True)

        def pv2(n, g, a, slot):
            vw = views[n][2]
            pref = p_ld[slot]
            c0 = slice(128 * (2 * a), 128 * (2 * a + 1))
            c1 = slice(128 * (2 * a + 1), 128 * (2 * a + 2))
            f0 = pref[0:32, c0]
            f1 = pref[0:32, c1]
            n0 = f0 & pn64
            o0 = f0 ^ n0
            n1 = f1 & pn64
            o1 = f1 ^ n1
            m0 = [pref[32 + 32 * b:64 + 32 * b, c0] for b in range(3)]
            m1 = [pref[32 + 32 * b:64 + 32 * b, c1] for b in range(3)]
            l0 = colsum(p_l2[slot][:, c0])
            l1 = colsum(p_l2[slot][:, c1])
            for e in range(2):
                h = 4 * g + 2 * a + e
                if e == 0:
                    tiles = [jnp.where(lo32, o0, zu), jnp.where(lo32, m0[0], o1),
                             jnp.where(lo32, m0[1], m1[0]), jnp.where(lo32, m0[2], m1[1]),
                             jnp.where(lo32, n0, m1[2]), jnp.where(lo32, zu, n1)]
                    l = jnp.where(lo1, l0, l1)
                else:
                    tiles = [jnp.where(lo32, zu, o0), jnp.where(lo32, o1, m0[0]),
                             jnp.where(lo32, m1[0], m0[1]), jnp.where(lo32, m1[1], m0[2]),
                             jnp.where(lo32, m1[2], n0), jnp.where(lo32, n1, zu)]
                    l = jnp.where(lo1, l1, l0)
                p = pltpu.bitcast(jnp.concatenate(tiles, axis=0), BF16)
                ot = jnp.dot(vw[32 * h:32 * (h + 1), :], p, preferred_element_type=F32)
                am = jnp.max(jnp.abs(ot).reshape(4, 8, 128), axis=0)
                ok = (l >= L_LO) & (l <= L_HI) & (am <= F_MAX)
                good[n] = ok if good[n] is None else (good[n] & ok)
                o = ot * (1.0 / l)
                if e == 1:
                    o = pltpu.roll(o, 64, 1)
                otbufs[n][32 * (h % 16):32 * (h % 16) + 32,
                          128 * (h // 16):128 * (h // 16) + 128] = o.astype(BF16)

        seq = [(n, g) for n in range(len(blocks)) for g in range(8)]
        for s in range(len(seq) + 2):
            if s < len(seq):
                n, g = seq[s]
                (qk2 if blocks[n][1] == 3 else qk)(n, g, s % 3)
            if s >= 2:
                n, g = seq[s - 2]
                if blocks[n][1] == 3:
                    for a in range(2):
                        pv2(n, g, a, (s - 2) % 3)
                else:
                    for j in range(4):
                        pv(n, g, j, (s - 2) % 3)
        for n in range(len(blocks)):
            flag[n] = jnp.min(jnp.where(good[n], 1, 0))

    def attention_safe(i, ow):
        r0 = _mo(i * QB, QB)
        start = pl.multiple_of(jnp.maximum(i - 2, 0) * QB, QB)
        qw = qt_b.at[:, pl.ds(r0, QB)]
        kw = k_b.at[pl.ds(start, 3 * QB), :]
        vw = vt_b.at[:, pl.ds(start, 3 * QB)]
        key = lax.broadcasted_iota(I32, (3 * QB, QB), 0) + start
        qry = lax.broadcasted_iota(I32, (3 * QB, QB), 1) + r0
        valid = (qry - key >= 0) & (qry - key < WIN)
        drow = lax.broadcasted_iota(I32, (128, QB), 0)

        def head(h, carry):
            g0 = pl.multiple_of((h // 4) * 128, 128)
            j0 = (h % 4) * 32
            q4 = qw[pl.ds(g0, 128), :].astype(F32)
            w = jnp.where((drow >= j0) & (drow < j0 + 32), q4, 0.0).astype(BF16)
            s = jnp.dot(kw[:, pl.ds(g0, 128)], w, preferred_element_type=F32)
            s = jnp.where(valid, s, NEG)
            m = jnp.max(s, axis=0, keepdims=True)
            p = jnp.exp2(s - m).astype(BF16)
            l = jnp.sum(p.astype(F32), axis=0, keepdims=True)
            vt = vw[pl.ds(pl.multiple_of(h * 32, 32), 32), :]
            o = jnp.dot(vt, p, preferred_element_type=F32) * (1.0 / l)
            ow[pl.ds(pl.multiple_of((h % 16) * 32, 32), 32),
               pl.ds(pl.multiple_of((h // 16) * 128, 128), 128)] = o.astype(BF16)
            return carry

        lax.fori_loop(0, NH, head, 0)

    def out_proj(n, slot=None):
        ow = ot_b.at[n]
        o = jnp.concatenate([ow[:, 0:128], ow[:, 128:256]], axis=0)
        ysum[n if slot is None else slot] = lax.dot_general(
            o, wo[...], TN, preferred_element_type=F32)

    def ln2(b, n, CH=16, NCHAIN=2):
        rb = _mo(b * QB, QB)
        wr = wr_ref[...].astype(F32)
        x1w = x1_b.at[pl.ds(rb, QB), :]
        x2w = xn.at[pl.ds(rb, QB), :]
        bm = None
        bi = None
        sub = lax.broadcasted_iota(I32, (8, 1), 0)
        toks = []
        for c in range(QB // CH):
            z = toks[c - NCHAIN] if c >= NCHAIN else 0
            yw = ysum.at[n + zs[1] + z]
            xw = xres.at[pl.ds(pl.multiple_of(rb + z * 16, 16), QB), :]
            x1 = xw[CH * c:CH * (c + 1), :].astype(F32) + yw[CH * c:CH * (c + 1), :]
            x1w[CH * c:CH * (c + 1), :] = x1.astype(BF16)
            h2 = _ln(x1)
            x2w[CH * c:CH * (c + 1), :] = (x1 + h2).astype(BF16)
            r = _rnd(jnp.sum(h2 * wr, axis=-1, keepdims=True))
            ru = lax.bitcast_convert_type(r, I32)
            toks.append(jnp.max(lax.shift_right_logical(lax.shift_right_logical(ru, 16), 16)))
            for t in range(CH // 8):
                rt = r[8 * t:8 * t + 8]
                it = sub + (rb + CH * c + 8 * t)
                if bm is None:
                    bm, bi = rt, it
                else:
                    better = rt > bm
                    bm = jnp.where(better, rt, bm)
                    bi = jnp.where(better, it, bi)
        bmax_ref[b] = jnp.broadcast_to(bm, (8, 128))
        bidx_ref[b] = jnp.broadcast_to(bi, (8, 128))

    def checks(i0):
        def one(n, carry):
            @pl.when(flag[n] == 0)
            def _():
                attention_safe(i0 + n, ot_b.at[n])
                out_proj(n)

                @pl.when(n == 0)
                def _():
                    ln2(i0, 0, NCHAIN=8)
            return carry

        @pl.when(flag[0] + flag[1] < 2)
        def _():
            lax.fori_loop(0, 2, one, 0)

    def out_copy(b):
        return pltpu.make_async_copy(xn.at[pl.ds(b * QB, QB), :],
                                     out_hbm.at[pl.ds(b * QB, QB), :], sem_o.at[0])

    def phase_b(layer):
        attention([(0, 1), (1, 2)])
        out_proj(0, zs[0])
        ln2(0, 0)
        out_proj(1)

        def body(t, carry):
            i0 = 2 * t
            checks(i0 - 2)

            @pl.when(layer == 1)
            def _():
                out_copy(i0 - 2).start()

            @pl.when(jnp.logical_and(layer == 1, t >= 2))
            def _():
                out_copy(i0 - 3).start()

            @pl.when(t < NQB // 2)
            def _():
                attention([(i0, 3), (i0 + 1, 3)])
                ln2(i0 - 1, 1)
                out_proj(0, zs[0])
                ln2(i0, 0)
                out_proj(1)
            return carry

        lax.fori_loop(1, NQB // 2 + 1, body, 0)
        ln2(NQB - 1, 1, NCHAIN=8)

        @pl.when(layer == 1)
        def _():
            out_copy(NQB - 1).start()

    def moe(layer):
        rm = bmax_ref[:, :, 0:1]
        ri = bidx_ref[:, :, 0:1]
        gm = jnp.max(jnp.max(rm, axis=0), axis=0, keepdims=True)
        idx = jnp.min(jnp.where(rm == gm, ri, BIG))
        b16 = pl.multiple_of((idx // 16) * 16, 16)
        x1c = x1_b[pl.ds(b16, 16), :].astype(F32)
        h2c = _rnd(_ln(x1c))
        hb = h2c.astype(BF16)
        g = _rnd(jnp.dot(hb, wg[...], preferred_element_type=F32))
        u = _rnd(jnp.dot(hb, wu[...], preferred_element_type=F32))
        g = _rnd(g * _rnd(jax.nn.sigmoid(g)))
        act = (g * u).astype(BF16)
        y = _rnd(jnp.dot(act, wd[...], preferred_element_type=F32))
        y = _rnd(y * _rnd(jax.nn.sigmoid(gm)))
        x2n = x1c + _rnd(h2c + y)

        @pl.when(layer == 1)
        def _():
            for b in range(NQB):
                out_copy(b).wait()

        cur = xn[pl.ds(b16, 16), :].astype(F32)
        sel = lax.broadcasted_iota(I32, (16, D), 0) == (idx - b16)
        xn[pl.ds(b16, 16), :] = jnp.where(sel, x2n, cur).astype(BF16)

        @pl.when(layer == 1)
        def _():
            cp = pltpu.make_async_copy(xn.at[pl.ds(b16, 16), :],
                                       out_hbm.at[pl.ds(b16, 16), :], sem_o.at[1])
            cp.start()
            cp.wait()

    def layer_body(layer, carry):
        phase_a(layer)

        @pl.when(layer == 0)
        def _():
            w_copies[0].wait()

        phase_b(layer)

        @pl.when(layer == 0)
        def _():
            for c in w_copies[1:]:
                c.wait()

        moe(layer)

        @pl.when(layer == 0)
        def _():
            ln1(0, hbufs[0])

        return carry

    lax.fori_loop(0, 2, layer_body, 0)


@jax.jit
def pallas_interleave_layers__sliding_block__moe_arch_mod__prompt_kernel(
    A_x: jax.Array,
    A_wqkv: jax.Array,
    A_wo: jax.Array,
    B_x: jax.Array,
    B_w_r: jax.Array,
    B_w_gate: jax.Array,
    B_w_up: jax.Array,
    B_w_down: jax.Array,
):
    del B_x
    hbm = pl.BlockSpec(memory_space=pl.ANY)
    scratch = [
        pltpu.VMEM((S // 2, D), U32),
        pltpu.VMEM((S // 2, D), U32),
        pltpu.VMEM((S // 2, D), U32),
        pltpu.VMEM((MB // 2, D), U32),
        pltpu.VMEM((MB // 2, D), U32),
        pltpu.VMEM((D // 2, S), U32),
        pltpu.VMEM((S // 2, D), U32),
        pltpu.VMEM((D // 2, S), U32),
        pltpu.VMEM((D // 2, 3 * D), U32),
        pltpu.VMEM((D, D), U32),
        pltpu.VMEM((D // 2, D), U32),
        pltpu.VMEM((D // 2, FF), U32),
        pltpu.VMEM((D // 2, FF), U32),
        pltpu.VMEM((FF // 2, D), U32),
        pltpu.VMEM((1, 128, 512), U32),
        pltpu.VMEM((1, 128, 512), U32),
        pltpu.VMEM((1, 128, 512), U32),
        pltpu.VMEM((2, 256, 256), U32),
        pltpu.VMEM((2, QB, D), F32),
        pltpu.VMEM((NQB, 8, 128), F32),
        pltpu.VMEM((NQB, 8, 128), I32),
        pltpu.SMEM((4,), I32),
        pltpu.SMEM((2,), I32),
        pltpu.SemaphoreType.DMA((NMB,)),
        pltpu.SemaphoreType.DMA((7,)),
        pltpu.SemaphoreType.DMA((2,)),
    ]
    out = pl.pallas_call(
        _kernel,
        out_shape=jax.ShapeDtypeStruct((S, D), BF16),
        in_specs=[hbm, hbm, hbm, pl.BlockSpec(memory_space=pltpu.VMEM), hbm, hbm, hbm],
        out_specs=hbm,
        scratch_shapes=scratch,
        compiler_params=pltpu.CompilerParams(vmem_limit_bytes=110 * 1024 * 1024),
        name="swa_moe_fused",
    )(A_x.reshape(S, D), A_wqkv, A_wo, B_w_r.reshape(1, D), B_w_gate, B_w_up, B_w_down)
    return out.reshape(1, S, D)
```

```python
import math

import jax
import jax.numpy as jnp
from jax import lax
import jax.experimental.pallas as pl
import jax.experimental.pallas.tpu as pltpu

S = 2048
D = 1024
NH = 32
DH = 32
WIN = 256
FF = 3584
QB = 128
NQB = S // QB
MB = 256
NMB = S // MB
EPS = 1e-5
QSCALE = (DH ** -0.5) * math.log2(math.e)
NEG = -1e30
BIG = 2 ** 30
L_LO = 2.0 ** -64
L_HI = 2.0 ** 64
F_MAX = 3.0e38

F32 = jnp.float32
BF16 = jnp.bfloat16
U32 = jnp.uint32
I32 = jnp.int32

NT = (((1,), (1,)), ((), ()))
TN = (((0,), (0,)), ((), ()))


def _rnd(v):
    return v.astype(BF16).astype(F32)


def _ln(xf):
    m = jnp.mean(xf, axis=-1, keepdims=True)
    xc = xf - m
    v = jnp.mean(xc * xc, axis=-1, keepdims=True)
    return xc * lax.rsqrt(v + EPS)


def _ln_stats(xf):
    m = jnp.sum(xf, axis=-1, keepdims=True) * (1.0 / D)
    v = jnp.sum(xf * xf, axis=-1, keepdims=True) * (1.0 / D) - m * m
    return m, lax.rsqrt(jnp.maximum(v, 0.0) + EPS)


def _mo(v, m):
    return v if isinstance(v, int) else pl.multiple_of(v, m)


def _kernel(x_hbm, wqkv_hbm, wo_hbm, wr_ref, wg_hbm, wu_hbm, wd_hbm, out_hbm,
            xn_u, xres_u, x1_u, h0_u, h1_u, qt_u, k_u, vt_u,
            wqkv_u, wqvt_u, wo_u, wg_u, wu_u, wd_u,
            p0, p1, p2, ot_u, ysum, bmax_ref, bidx_ref, zs, flag,
            sem_x, sem_w, sem_o):
    xn = xn_u.bitcast(BF16)
    xres = xres_u.bitcast(BF16)
    x1_b = x1_u.bitcast(BF16)
    hbufs = (h0_u.bitcast(BF16), h1_u.bitcast(BF16))
    qt_b = qt_u.bitcast(BF16)
    k_b = k_u.bitcast(BF16)
    vt_b = vt_u.bitcast(BF16)
    wqkv = wqkv_u.bitcast(BF16)
    wqvt = wqvt_u.bitcast(BF16)
    wo = wo_u.bitcast(BF16)
    wg = wg_u.bitcast(BF16)
    wu = wu_u.bitcast(BF16)
    wd = wd_u.bitcast(BF16)
    ot_b = ot_u.bitcast(BF16)
    otbufs = (ot_b.at[0], ot_b.at[1])
    pbufs_u = (p0, p1, p2)
    pbufs_b = tuple(p.bitcast(BF16) for p in pbufs_u)

    def x_copy(j):
        return pltpu.make_async_copy(x_hbm.at[pl.ds(j * MB, MB), :],
                                     xn.at[pl.ds(j * MB, MB), :], sem_x.at[j])

    def wqkv_copy(t):
        return pltpu.make_async_copy(wqkv_hbm.at[:, pl.ds(t * D, D)],
                                     wqkv.at[:, pl.ds(t * D, D)], sem_w.at[t])

    w_copies = [
        pltpu.make_async_copy(wo_hbm, wo, sem_w.at[3]),
        pltpu.make_async_copy(wg_hbm, wg, sem_w.at[4]),
        pltpu.make_async_copy(wu_hbm, wu, sem_w.at[5]),
        pltpu.make_async_copy(wd_hbm, wd, sem_w.at[6]),
    ]
    wqkv_copy(0).start()
    x_copy(0).start()
    wqkv_copy(2).start()
    x_copy(1).start()
    x_copy(2).start()
    wqkv_copy(1).start()
    for j in range(3, NMB):
        x_copy(j).start()

    for t in range(4):
        zs[t] = 0

    eye = (lax.broadcasted_iota(I32, (128, 128), 0)
           == lax.broadcasted_iota(I32, (128, 128), 1)).astype(F32).astype(BF16)

    def transpose_w(src_col0, dst_row0, tiles):
        for t in tiles:
            w_t = wqkv[:, src_col0 + 128 * t:src_col0 + 128 * (t + 1)]
            wqvt[dst_row0 + 128 * t:dst_row0 + 128 * (t + 1), :] = lax.dot_general(
                eye, w_t, NT, preferred_element_type=F32).astype(BF16)

    def ln1(row0, dst):
        src = xn.at[pl.ds(row0, MB), :]
        res = xres.at[pl.ds(row0, MB), :]
        for c in range(MB // 64):
            xb = src[64 * c:64 * (c + 1), :]
            res[64 * c:64 * (c + 1), :] = xb
            dst[64 * c:64 * (c + 1), :] = _ln(xb.astype(F32)).astype(BF16)

    def proj_q(base, hsrc):
        q = lax.dot_general(wqvt[0:D, :], hsrc[...], NT, preferred_element_type=F32)
        qt_b[:, pl.ds(base, MB)] = (q * QSCALE).astype(BF16)

    def proj_v(base, hsrc):
        v = lax.dot_general(wqvt[D:2 * D, :], hsrc[...], NT, preferred_element_type=F32)
        vt_b[:, pl.ds(base, MB)] = v.astype(BF16)

    def proj_qv(base, hsrc):
        qv = lax.dot_general(wqvt[...], hsrc[...], NT, preferred_element_type=F32)
        qt_b[:, pl.ds(base, MB)] = (qv[0:D] * QSCALE).astype(BF16)
        vt_b[:, pl.ds(base, MB)] = qv[D:2 * D].astype(BF16)

    def proj_k(base, hsrc):
        k = jnp.dot(hsrc[...], wqkv[:, D:2 * D], preferred_element_type=F32)
        k_b[pl.ds(base, MB), :] = k.astype(BF16)

    def phase_a(layer):
        def body(t, carry):
            first = jnp.logical_and(layer == 0, t == 0)

            @pl.when(first)
            def _():
                x_copy(1).wait()
                x_copy(2).wait()
                wqkv_copy(1).wait()
                for c in w_copies:
                    c.start()

            @pl.when(jnp.logical_and(layer == 0, t >= 1))
            def _():
                x_copy(2 * t + 1).wait()

            @pl.when(jnp.logical_and(layer == 0, jnp.logical_and(t >= 1, t < NMB // 2 - 1)))
            def _():
                x_copy(2 * t + 2).wait()

            b0 = pl.multiple_of(2 * t * MB, MB)
            b1 = pl.multiple_of(b0 + MB, MB)
            b2 = pl.multiple_of(jnp.minimum(2 * t + 2, NMB - 1) * MB, MB)

            @pl.when(jnp.logical_not(first))
            def _():
                proj_qv(b0, hbufs[0])

            proj_k(b0, hbufs[0])
            ln1(b1, hbufs[1])
            proj_qv(b1, hbufs[1])
            proj_k(b1, hbufs[1])
            ln1(b2, hbufs[0])
            return carry

        lax.fori_loop(0, NMB // 2, body, 0)

    wqkv_copy(0).wait()
    transpose_w(0, 0, range(0, 4))
    x_copy(0).wait()
    transpose_w(0, 0, range(4, 8))
    ln1(0, hbufs[0])
    proj_q(0, hbufs[0])
    wqkv_copy(2).wait()
    transpose_w(2 * D, D, range(8))
    proj_v(0, hbufs[0])

    def attention(blocks):
        zst = zs[0]
        zld = zs[1]
        zl2 = zs[2]
        lane = lax.broadcasted_iota(I32, (QB, QB), 1)
        row = lax.broadcasted_iota(I32, (QB, QB), 0)
        newmask = row <= lane
        l2 = lax.broadcasted_iota(I32, (QB // 2, QB), 1)
        r2 = lax.broadcasted_iota(I32, (QB // 2, QB), 0) * 2
        pm_new = (jnp.where(r2 <= l2, U32(0xFFFF), U32(0))
                  | jnp.where(r2 + 1 <= l2, U32(0xFFFF0000), U32(0)))
        p_st = [p.at[zst] for p in pbufs_b]
        p_ld = [p.at[zld] for p in pbufs_u]
        p_l2 = [p.at[zl2] for p in pbufs_u]
        zero32 = jnp.zeros((32, QB), BF16)
        good = [None] * len(blocks)
        views = []
        for (i, nkb) in blocks:
            r0 = _mo(i * QB, QB)
            k0 = 128 * (nkb - 1)
            views.append((qt_b.at[:, pl.ds(r0, QB)],
                          k_b.at[pl.ds(r0 - k0, k0 + QB), :],
                          vt_b.at[:, pl.ds(r0 - k0, k0 + QB)]))

        def qk(n, g, slot):
            nkb = blocks[n][1]
            k0 = 128 * (nkb - 1)
            qw, kw, _ = views[n]
            cs = slice(128 * g, 128 * (g + 1))
            ws = []
            for j in range(4):
                h = 4 * g + j
                ws.append(jnp.concatenate(
                    [zero32] * j + [qw[32 * h:32 * (h + 1), :]] + [zero32] * (3 - j), axis=0))
            w = jnp.concatenate(ws, axis=1)
            parts = []
            if nkb == 3:
                for c in range(8):
                    parts.append(kw[16 * c:16 * c + 16, cs])
                    parts.append(kw[256 + 16 * c:256 + 16 * c + 16, cs])
            else:
                parts.append(kw[k0:k0 + 128, cs])
            if nkb >= 2:
                parts.append(kw[k0 - 128:k0, cs])
            kk = jnp.concatenate(parts, axis=0)
            st = jnp.dot(kk, w, preferred_element_type=F32)
            pref = p_st[slot]
            for j in range(4):
                s = st[:, 128 * j:128 * (j + 1)]
                ls = slice(128 * j, 128 * (j + 1))
                for c in range(8):
                    nm = newmask[16 * c:16 * c + 16]
                    if nkb == 3:
                        f = jnp.where(nm, s[32 * c + 16:32 * c + 32], s[32 * c:32 * c + 16])
                    else:
                        f = jnp.where(nm, s[16 * c:16 * c + 16], NEG)
                    pref[16 * c:16 * c + 16, ls] = jnp.exp2(f).astype(BF16)
                if nkb >= 2:
                    o = 256 if nkb == 3 else 128
                    for c in range(8):
                        pref[128 + 16 * c:128 + 16 * c + 16, ls] = jnp.exp2(
                            s[o + 16 * c:o + 16 * c + 16]).astype(BF16)

        def pv(n, g, j, slot):
            nkb = blocks[n][1]
            nrow = 128 if nkb == 1 else 256
            vw = views[n][2]
            h = 4 * g + j
            pref = p_ld[slot]
            ls = slice(128 * j, 128 * (j + 1))
            pf = pref[0:64, ls]
            if nkb == 3:
                pnew = pf & pm_new
                p = jnp.concatenate([pf ^ pnew, pref[64:128, ls], pnew], axis=0)
            elif nkb == 2:
                p = jnp.concatenate([pref[64:128, ls], pf], axis=0)
            else:
                p = pf
            vt = vw[32 * h:32 * (h + 1), :]
            ot = jnp.dot(vt, pltpu.bitcast(p, BF16), preferred_element_type=F32)
            pp = p_l2[slot][0:nrow // 2, ls]
            x = (pltpu.bitcast(pp & U32(0xFFFF0000), F32)
                 + pltpu.bitcast(pp << 16, F32)).reshape(nrow // 16, 8, 128)
            while x.shape[0] > 1:
                m = x.shape[0] // 2
                x = x[:m] + x[m:]
            l = jnp.sum(x[0], axis=0, keepdims=True)
            am = jnp.max(jnp.abs(ot).reshape(4, 8, 128), axis=0)
            ok = (l >= L_LO) & (l <= L_HI) & (am <= F_MAX)
            good[n] = ok if good[n] is None else (good[n] & ok)
            o = (ot * (1.0 / l)).astype(BF16)
            otbufs[n][32 * (h % 16):32 * (h % 16) + 32,
                      128 * (h // 16):128 * (h // 16) + 128] = o

        l64 = lax.broadcasted_iota(I32, (16, QB), 1)
        lo16 = l64 < 64
        lo8 = lax.broadcasted_iota(I32, (8, QB), 1) < 64
        lo1 = lax.broadcasted_iota(I32, (1, QB), 1) < 64
        t64 = lax.broadcasted_iota(I32, (64, QB), 0)
        s64 = lax.broadcasted_iota(I32, (64, QB), 1) & 63
        new64 = t64 <= s64
        r32 = lax.broadcasted_iota(I32, (32, QB), 0) * 2
        c32 = lax.broadcasted_iota(I32, (32, QB), 1)
        lo32 = c32 < 64
        pn64 = (jnp.where(r32 <= (c32 & 63), U32(0xFFFF), U32(0))
                | jnp.where(r32 + 1 <= (c32 & 63), U32(0xFFFF0000), U32(0)))
        po64 = ~pn64
        zu = U32(0)

        def qk2(n, g, slot):
            qw, kw, _ = views[n]
            cs = slice(128 * g, 128 * (g + 1))
            pref = p_st[slot]
            for a in range(2):
                he = 4 * g + 2 * a
                xe = pltpu.bitcast(qw[32 * he:32 * he + 32, :], U32)
                xo = pltpu.roll(pltpu.bitcast(qw[32 * he + 32:32 * he + 64, :], U32), 64, 1)
                for u in range(2):
                    me = lo16 if u == 0 else jnp.logical_not(lo16)
                    wt = pltpu.bitcast(jnp.concatenate(
                        [jnp.where(me, xe, zu), jnp.where(me, zu, xo)], axis=0), BF16)
                    w = jnp.concatenate([zero32] * (2 * a) + [wt] + [zero32] * (2 - 2 * a), axis=0)
                    parts = []
                    for c in range(4):
                        parts.append(kw[64 * u + 16 * c:64 * u + 16 * c + 16, cs])
                        parts.append(kw[64 * u + 256 + 16 * c:64 * u + 256 + 16 * c + 16, cs])
                    parts.append(kw[64 * u + 64:64 * u + 256, cs])
                    s = jnp.dot(jnp.concatenate(parts, axis=0), w, preferred_element_type=F32)
                    ls = slice(128 * (2 * a + u), 128 * (2 * a + u + 1))
                    for c in range(4):
                        f = jnp.where(new64[16 * c:16 * c + 16], s[32 * c + 16:32 * c + 32],
                                      s[32 * c:32 * c + 16])
                        pref[16 * c:16 * c + 16, ls] = jnp.exp2(f).astype(BF16)
                    for c in range(12):
                        pref[64 + 16 * c:64 + 16 * c + 16, ls] = jnp.exp2(
                            s[128 + 16 * c:128 + 16 * c + 16]).astype(BF16)

        def colsum(pp):
            x = (pltpu.bitcast(pp & U32(0xFFFF0000), F32)
                 + pltpu.bitcast(pp << 16, F32)).reshape(pp.shape[0] // 8, 8, 128)
            while x.shape[0] > 1:
                m = x.shape[0] // 2
                x = x[:m] + x[m:]
            return jnp.sum(x[0], axis=0, keepdims=True)

        def pv2(n, g, a, slot):
            vw = views[n][2]
            pref = p_ld[slot]
            c0 = slice(128 * (2 * a), 128 * (2 * a + 1))
            c1 = slice(128 * (2 * a + 1), 128 * (2 * a + 2))
            f0 = pref[0:32, c0]
            f1 = pref[0:32, c1]
            n0 = f0 & pn64
            o0 = f0 ^ n0
            n1 = f1 & pn64
            o1 = f1 ^ n1
            m0 = [pref[32 + 32 * b:64 + 32 * b, c0] for b in range(3)]
            m1 = [pref[32 + 32 * b:64 + 32 * b, c1] for b in range(3)]
            l0 = colsum(p_l2[slot][:, c0])
            l1 = colsum(p_l2[slot][:, c1])
            for e in range(2):
                h = 4 * g + 2 * a + e
                if e == 0:
                    tiles = [jnp.where(lo32, o0, zu), jnp.where(lo32, m0[0], o1),
                             jnp.where(lo32, m0[1], m1[0]), jnp.where(lo32, m0[2], m1[1]),
                             jnp.where(lo32, n0, m1[2]), jnp.where(lo32, zu, n1)]
                    l = jnp.where(lo1, l0, l1)
                else:
                    tiles = [jnp.where(lo32, zu, o0), jnp.where(lo32, o1, m0[0]),
                             jnp.where(lo32, m1[0], m0[1]), jnp.where(lo32, m1[1], m0[2]),
                             jnp.where(lo32, m1[2], n0), jnp.where(lo32, n1, zu)]
                    l = jnp.where(lo1, l1, l0)
                p = pltpu.bitcast(jnp.concatenate(tiles, axis=0), BF16)
                ot = jnp.dot(vw[32 * h:32 * (h + 1), :], p, preferred_element_type=F32)
                am = jnp.max(jnp.abs(ot).reshape(4, 8, 128), axis=0)
                ok = (l >= L_LO) & (l <= L_HI) & (am <= F_MAX)
                good[n] = ok if good[n] is None else (good[n] & ok)
                o = ot * (1.0 / l)
                if e == 1:
                    o = pltpu.roll(o, 64, 1)
                otbufs[n][32 * (h % 16):32 * (h % 16) + 32,
                          128 * (h // 16):128 * (h // 16) + 128] = o.astype(BF16)

        seq = [(n, g) for n in range(len(blocks)) for g in range(8)]
        for s in range(len(seq) + 2):
            if s < len(seq):
                n, g = seq[s]
                (qk2 if blocks[n][1] == 3 else qk)(n, g, s % 3)
            if s >= 2:
                n, g = seq[s - 2]
                if blocks[n][1] == 3:
                    for a in range(2):
                        pv2(n, g, a, (s - 2) % 3)
                else:
                    for j in range(4):
                        pv(n, g, j, (s - 2) % 3)
        for n in range(len(blocks)):
            flag[n] = jnp.min(jnp.where(good[n], 1, 0))

    def attention_safe(i, ow):
        r0 = _mo(i * QB, QB)
        start = pl.multiple_of(jnp.maximum(i - 2, 0) * QB, QB)
        qw = qt_b.at[:, pl.ds(r0, QB)]
        kw = k_b.at[pl.ds(start, 3 * QB), :]
        vw = vt_b.at[:, pl.ds(start, 3 * QB)]
        key = lax.broadcasted_iota(I32, (3 * QB, QB), 0) + start
        qry = lax.broadcasted_iota(I32, (3 * QB, QB), 1) + r0
        valid = (qry - key >= 0) & (qry - key < WIN)
        drow = lax.broadcasted_iota(I32, (128, QB), 0)

        def head(h, carry):
            g0 = pl.multiple_of((h // 4) * 128, 128)
            j0 = (h % 4) * 32
            q4 = qw[pl.ds(g0, 128), :].astype(F32)
            w = jnp.where((drow >= j0) & (drow < j0 + 32), q4, 0.0).astype(BF16)
            s = jnp.dot(kw[:, pl.ds(g0, 128)], w, preferred_element_type=F32)
            s = jnp.where(valid, s, NEG)
            m = jnp.max(s, axis=0, keepdims=True)
            p = jnp.exp2(s - m).astype(BF16)
            l = jnp.sum(p.astype(F32), axis=0, keepdims=True)
            vt = vw[pl.ds(pl.multiple_of(h * 32, 32), 32), :]
            o = jnp.dot(vt, p, preferred_element_type=F32) * (1.0 / l)
            ow[pl.ds(pl.multiple_of((h % 16) * 32, 32), 32),
               pl.ds(pl.multiple_of((h // 16) * 128, 128), 128)] = o.astype(BF16)
            return carry

        lax.fori_loop(0, NH, head, 0)

    def out_proj(n, slot=None):
        ow = ot_b.at[n]
        o = jnp.concatenate([ow[:, 0:128], ow[:, 128:256]], axis=0)
        ysum[n if slot is None else slot] = lax.dot_general(
            o, wo[...], TN, preferred_element_type=F32)

    def ln2(b, n, CH=16, NCHAIN=2):
        rb = _mo(b * QB, QB)
        wr = wr_ref[...].astype(F32).reshape(1, D)
        wsum = jnp.sum(wr, axis=-1, keepdims=True)
        x1w = x1_b.at[pl.ds(rb, QB), :]
        x2w = xn.at[pl.ds(rb, QB), :]
        bm = None
        bi = None
        sub = lax.broadcasted_iota(I32, (8, 1), 0)
        toks = []
        for c in range(QB // CH):
            z = toks[c - NCHAIN] if c >= NCHAIN else 0
            yw = ysum.at[n + zs[1] + z]
            xw = xres.at[pl.ds(pl.multiple_of(rb + z * 16, 16), QB), :]
            x1 = xw[CH * c:CH * (c + 1), :].astype(F32) + yw[CH * c:CH * (c + 1), :]
            x1w[CH * c:CH * (c + 1), :] = x1.astype(BF16)
            m, rs = _ln_stats(x1)
            x2w[CH * c:CH * (c + 1), :] = (x1 * (1.0 + rs) - m * rs).astype(BF16)
            r = _rnd(rs * (jnp.sum(x1 * wr, axis=-1, keepdims=True) - m * wsum))
            ru = lax.bitcast_convert_type(r, I32)
            toks.append(jnp.max(lax.shift_right_logical(lax.shift_right_logical(ru, 16), 16)))
            for t in range(CH // 8):
                rt = r[8 * t:8 * t + 8]
                it = sub + (rb + CH * c + 8 * t)
                if bm is None:
                    bm, bi = rt, it
                else:
                    better = rt > bm
                    bm = jnp.where(better, rt, bm)
                    bi = jnp.where(better, it, bi)
        bmax_ref[b] = jnp.broadcast_to(bm, (8, 128))
        bidx_ref[b] = jnp.broadcast_to(bi, (8, 128))

    def checks(i0):
        def one(n, carry):
            @pl.when(flag[n] == 0)
            def _():
                attention_safe(i0 + n, ot_b.at[n])
                out_proj(n)

                @pl.when(n == 0)
                def _():
                    ln2(i0, 0, NCHAIN=8)
            return carry

        @pl.when(flag[0] + flag[1] < 2)
        def _():
            lax.fori_loop(0, 2, one, 0)

    def out_copy(b):
        return pltpu.make_async_copy(xn.at[pl.ds(b * QB, QB), :],
                                     out_hbm.at[pl.ds(b * QB, QB), :], sem_o.at[0])

    def phase_b(layer):
        attention([(0, 1), (1, 2)])
        out_proj(0, zs[0])
        ln2(0, 0)
        out_proj(1)

        def body(t, carry):
            i0 = 2 * t
            checks(i0 - 2)

            @pl.when(layer == 1)
            def _():
                out_copy(i0 - 2).start()

            @pl.when(jnp.logical_and(layer == 1, t >= 2))
            def _():
                out_copy(i0 - 3).start()

            @pl.when(t < NQB // 2)
            def _():
                attention([(i0, 3), (i0 + 1, 3)])
                ln2(i0 - 1, 1)
                out_proj(0, zs[0])
                ln2(i0, 0)
                out_proj(1)
            return carry

        lax.fori_loop(1, NQB // 2 + 1, body, 0)
        ln2(NQB - 1, 1, NCHAIN=8)

        @pl.when(layer == 1)
        def _():
            out_copy(NQB - 1).start()

    def moe(layer):
        rm = bmax_ref[:, :, 0:1]
        ri = bidx_ref[:, :, 0:1]
        gm = jnp.max(jnp.max(rm, axis=0), axis=0, keepdims=True)
        idx = jnp.min(jnp.where(rm == gm, ri, BIG))
        b16 = pl.multiple_of((idx // 16) * 16, 16)
        x1c = x1_b[pl.ds(b16, 16), :].astype(F32)
        h2c = _rnd(_ln(x1c))
        hb = h2c.astype(BF16)
        g = _rnd(jnp.dot(hb, wg[...], preferred_element_type=F32))
        u = _rnd(jnp.dot(hb, wu[...], preferred_element_type=F32))
        g = _rnd(g * _rnd(jax.nn.sigmoid(g)))
        act = (g * u).astype(BF16)
        y = _rnd(jnp.dot(act, wd[...], preferred_element_type=F32))
        y = _rnd(y * _rnd(jax.nn.sigmoid(gm)))
        x2n = x1c + _rnd(h2c + y)

        @pl.when(layer == 1)
        def _():
            for b in range(NQB):
                out_copy(b).wait()

        cur = xn[pl.ds(b16, 16), :].astype(F32)
        sel = lax.broadcasted_iota(I32, (16, D), 0) == (idx - b16)
        xn[pl.ds(b16, 16), :] = jnp.where(sel, x2n, cur).astype(BF16)

        @pl.when(layer == 1)
        def _():
            cp = pltpu.make_async_copy(xn.at[pl.ds(b16, 16), :],
                                       out_hbm.at[pl.ds(b16, 16), :], sem_o.at[1])
            cp.start()
            cp.wait()

    def layer_body(layer, carry):
        phase_a(layer)

        @pl.when(layer == 0)
        def _():
            w_copies[0].wait()

        phase_b(layer)

        @pl.when(layer == 0)
        def _():
            for c in w_copies[1:]:
                c.wait()

        moe(layer)

        @pl.when(layer == 0)
        def _():
            ln1(0, hbufs[0])

        return carry

    lax.fori_loop(0, 2, layer_body, 0)


@jax.jit
def pallas_interleave_layers__sliding_block__moe_arch_mod__prompt_kernel(
    A_x: jax.Array,
    A_wqkv: jax.Array,
    A_wo: jax.Array,
    B_x: jax.Array,
    B_w_r: jax.Array,
    B_w_gate: jax.Array,
    B_w_up: jax.Array,
    B_w_down: jax.Array,
):
    del B_x
    hbm = pl.BlockSpec(memory_space=pl.ANY)
    scratch = [
        pltpu.VMEM((S // 2, D), U32),
        pltpu.VMEM((S // 2, D), U32),
        pltpu.VMEM((S // 2, D), U32),
        pltpu.VMEM((MB // 2, D), U32),
        pltpu.VMEM((MB // 2, D), U32),
        pltpu.VMEM((D // 2, S), U32),
        pltpu.VMEM((S // 2, D), U32),
        pltpu.VMEM((D // 2, S), U32),
        pltpu.VMEM((D // 2, 3 * D), U32),
        pltpu.VMEM((D, D), U32),
        pltpu.VMEM((D // 2, D), U32),
        pltpu.VMEM((D // 2, FF), U32),
        pltpu.VMEM((D // 2, FF), U32),
        pltpu.VMEM((FF // 2, D), U32),
        pltpu.VMEM((1, 128, 512), U32),
        pltpu.VMEM((1, 128, 512), U32),
        pltpu.VMEM((1, 128, 512), U32),
        pltpu.VMEM((2, 256, 256), U32),
        pltpu.VMEM((2, QB, D), F32),
        pltpu.VMEM((NQB, 8, 128), F32),
        pltpu.VMEM((NQB, 8, 128), I32),
        pltpu.SMEM((4,), I32),
        pltpu.SMEM((2,), I32),
        pltpu.SemaphoreType.DMA((NMB,)),
        pltpu.SemaphoreType.DMA((7,)),
        pltpu.SemaphoreType.DMA((2,)),
    ]
    out = pl.pallas_call(
        _kernel,
        out_shape=jax.ShapeDtypeStruct((S, D), BF16),
        in_specs=[hbm, hbm, hbm, pl.BlockSpec(memory_space=pltpu.VMEM), hbm, hbm, hbm],
        out_specs=hbm,
        scratch_shapes=scratch,
        compiler_params=pltpu.CompilerParams(vmem_limit_bytes=110 * 1024 * 1024),
        name="swa_moe_fused",
    )(A_x.reshape(S, D), A_wqkv, A_wo, B_w_r, B_w_gate, B_w_up, B_w_down)
    return out.reshape(1, S, D)
```

```python
import math

import jax
import jax.numpy as jnp
from jax import lax
import jax.experimental.pallas as pl
import jax.experimental.pallas.tpu as pltpu

S = 2048
D = 1024
NH = 32
DH = 32
WIN = 256
FF = 3584
QB = 128
NQB = S // QB
MB = 256
NMB = S // MB
EPS = 1e-5
QSCALE = (DH ** -0.5) * math.log2(math.e)
NEG = -1e30
BIG = 2 ** 30
L_LO = 2.0 ** -64
L_HI = 2.0 ** 64
F_MAX = 3.0e38

F32 = jnp.float32
BF16 = jnp.bfloat16
U32 = jnp.uint32
I32 = jnp.int32

NT = (((1,), (1,)), ((), ()))
TN = (((0,), (0,)), ((), ()))


def _rnd(v):
    return v.astype(BF16).astype(F32)


def _ln(xf):
    m = jnp.mean(xf, axis=-1, keepdims=True)
    xc = xf - m
    v = jnp.mean(xc * xc, axis=-1, keepdims=True)
    return xc * lax.rsqrt(v + EPS)


def _ln_stats(xf):
    m = jnp.sum(xf, axis=-1, keepdims=True) * (1.0 / D)
    v = jnp.sum(xf * xf, axis=-1, keepdims=True) * (1.0 / D) - m * m
    return m, lax.rsqrt(jnp.maximum(v, 0.0) + EPS)


def _mo(v, m):
    return v if isinstance(v, int) else pl.multiple_of(v, m)


def _kernel(x_hbm, wqkv_hbm, wo_hbm, wr_ref, wg_hbm, wu_hbm, wd_hbm, out_hbm,
            xn_u, x1_u, h0_u, h1_u, qt_u, k_u, vt_u,
            wqkv_u, wqvt_u, wo_u, wg_u, wu_u, wd_u,
            p0, p1, p2, ot_u, bmax_ref, bidx_ref, zs, flag,
            sem_x, sem_w, sem_o):
    xn = xn_u.bitcast(BF16)
    x1_b = x1_u.bitcast(BF16)
    hbufs = (h0_u.bitcast(BF16), h1_u.bitcast(BF16))
    qt_b = qt_u.bitcast(BF16)
    k_b = k_u.bitcast(BF16)
    vt_b = vt_u.bitcast(BF16)
    wqkv = wqkv_u.bitcast(BF16)
    wqvt = wqvt_u.bitcast(BF16)
    wo = wo_u.bitcast(BF16)
    wg = wg_u.bitcast(BF16)
    wu = wu_u.bitcast(BF16)
    wd = wd_u.bitcast(BF16)
    ot_b = ot_u.bitcast(BF16)
    otbufs = (ot_b.at[0], ot_b.at[1])
    pbufs_u = (p0, p1, p2)
    pbufs_b = tuple(p.bitcast(BF16) for p in pbufs_u)

    def x_copy(j):
        return pltpu.make_async_copy(x_hbm.at[pl.ds(j * MB, MB), :],
                                     xn.at[pl.ds(j * MB, MB), :], sem_x.at[j])

    def wqkv_copy(t):
        return pltpu.make_async_copy(wqkv_hbm.at[:, pl.ds(t * D, D)],
                                     wqkv.at[:, pl.ds(t * D, D)], sem_w.at[t])

    w_copies = [
        pltpu.make_async_copy(wo_hbm, wo, sem_w.at[3]),
        pltpu.make_async_copy(wg_hbm, wg, sem_w.at[4]),
        pltpu.make_async_copy(wu_hbm, wu, sem_w.at[5]),
        pltpu.make_async_copy(wd_hbm, wd, sem_w.at[6]),
    ]
    wqkv_copy(0).start()
    x_copy(0).start()
    wqkv_copy(2).start()
    x_copy(1).start()
    x_copy(2).start()
    wqkv_copy(1).start()
    for j in range(3, NMB):
        x_copy(j).start()

    for t in range(4):
        zs[t] = 0

    eye = (lax.broadcasted_iota(I32, (128, 128), 0)
           == lax.broadcasted_iota(I32, (128, 128), 1)).astype(F32).astype(BF16)

    def transpose_w(src_col0, dst_row0, tiles):
        for t in tiles:
            w_t = wqkv[:, src_col0 + 128 * t:src_col0 + 128 * (t + 1)]
            wqvt[dst_row0 + 128 * t:dst_row0 + 128 * (t + 1), :] = lax.dot_general(
                eye, w_t, NT, preferred_element_type=F32).astype(BF16)

    def ln1(row0, dst):
        src = xn.at[pl.ds(row0, MB), :]
        for c in range(MB // 64):
            xf = src[64 * c:64 * (c + 1), :].astype(F32)
            dst[64 * c:64 * (c + 1), :] = _ln(xf).astype(BF16)

    def proj_q(base, hsrc):
        q = lax.dot_general(wqvt[0:D, :], hsrc[...], NT, preferred_element_type=F32)
        qt_b[:, pl.ds(base, MB)] = (q * QSCALE).astype(BF16)

    def proj_v(base, hsrc):
        v = lax.dot_general(wqvt[D:2 * D, :], hsrc[...], NT, preferred_element_type=F32)
        vt_b[:, pl.ds(base, MB)] = v.astype(BF16)

    def proj_qv(base, hsrc):
        qv = lax.dot_general(wqvt[...], hsrc[...], NT, preferred_element_type=F32)
        qt_b[:, pl.ds(base, MB)] = (qv[0:D] * QSCALE).astype(BF16)
        vt_b[:, pl.ds(base, MB)] = qv[D:2 * D].astype(BF16)

    def proj_k(base, hsrc):
        k = jnp.dot(hsrc[...], wqkv[:, D:2 * D], preferred_element_type=F32)
        k_b[pl.ds(base, MB), :] = k.astype(BF16)

    def phase_a(layer):
        def body(t, carry):
            first = jnp.logical_and(layer == 0, t == 0)

            @pl.when(first)
            def _():
                x_copy(1).wait()
                x_copy(2).wait()
                wqkv_copy(1).wait()
                for c in w_copies:
                    c.start()

            @pl.when(jnp.logical_and(layer == 0, t >= 1))
            def _():
                x_copy(2 * t + 1).wait()

            @pl.when(jnp.logical_and(layer == 0, jnp.logical_and(t >= 1, t < NMB // 2 - 1)))
            def _():
                x_copy(2 * t + 2).wait()

            b0 = pl.multiple_of(2 * t * MB, MB)
            b1 = pl.multiple_of(b0 + MB, MB)
            b2 = pl.multiple_of(jnp.minimum(2 * t + 2, NMB - 1) * MB, MB)

            @pl.when(jnp.logical_not(first))
            def _():
                proj_qv(b0, hbufs[0])

            proj_k(b0, hbufs[0])
            ln1(b1, hbufs[1])
            proj_qv(b1, hbufs[1])
            proj_k(b1, hbufs[1])
            ln1(b2, hbufs[0])
            return carry

        lax.fori_loop(0, NMB // 2, body, 0)

    wqkv_copy(0).wait()
    transpose_w(0, 0, range(0, 4))
    x_copy(0).wait()
    transpose_w(0, 0, range(4, 8))
    ln1(0, hbufs[0])
    proj_q(0, hbufs[0])
    wqkv_copy(2).wait()
    transpose_w(2 * D, D, range(8))
    proj_v(0, hbufs[0])

    def attention(blocks):
        zst = zs[0]
        zld = zs[1]
        zl2 = zs[2]
        lane = lax.broadcasted_iota(I32, (QB, QB), 1)
        row = lax.broadcasted_iota(I32, (QB, QB), 0)
        newmask = row <= lane
        l2 = lax.broadcasted_iota(I32, (QB // 2, QB), 1)
        r2 = lax.broadcasted_iota(I32, (QB // 2, QB), 0) * 2
        pm_new = (jnp.where(r2 <= l2, U32(0xFFFF), U32(0))
                  | jnp.where(r2 + 1 <= l2, U32(0xFFFF0000), U32(0)))
        p_st = [p.at[zst] for p in pbufs_b]
        p_ld = [p.at[zld] for p in pbufs_u]
        p_l2 = [p.at[zl2] for p in pbufs_u]
        zero32 = jnp.zeros((32, QB), BF16)
        good = [None] * len(blocks)
        views = []
        for (i, nkb) in blocks:
            r0 = _mo(i * QB, QB)
            k0 = 128 * (nkb - 1)
            views.append((qt_b.at[:, pl.ds(r0, QB)],
                          k_b.at[pl.ds(r0 - k0, k0 + QB), :],
                          vt_b.at[:, pl.ds(r0 - k0, k0 + QB)]))

        def qk(n, g, slot):
            nkb = blocks[n][1]
            k0 = 128 * (nkb - 1)
            qw, kw, _ = views[n]
            cs = slice(128 * g, 128 * (g + 1))
            ws = []
            for j in range(4):
                h = 4 * g + j
                ws.append(jnp.concatenate(
                    [zero32] * j + [qw[32 * h:32 * (h + 1), :]] + [zero32] * (3 - j), axis=0))
            w = jnp.concatenate(ws, axis=1)
            parts = []
            if nkb == 3:
                for c in range(8):
                    parts.append(kw[16 * c:16 * c + 16, cs])
                    parts.append(kw[256 + 16 * c:256 + 16 * c + 16, cs])
            else:
                parts.append(kw[k0:k0 + 128, cs])
            if nkb >= 2:
                parts.append(kw[k0 - 128:k0, cs])
            kk = jnp.concatenate(parts, axis=0)
            st = jnp.dot(kk, w, preferred_element_type=F32)
            pref = p_st[slot]
            for j in range(4):
                s = st[:, 128 * j:128 * (j + 1)]
                ls = slice(128 * j, 128 * (j + 1))
                for c in range(8):
                    nm = newmask[16 * c:16 * c + 16]
                    if nkb == 3:
                        f = jnp.where(nm, s[32 * c + 16:32 * c + 32], s[32 * c:32 * c + 16])
                    else:
                        f = jnp.where(nm, s[16 * c:16 * c + 16], NEG)
                    pref[16 * c:16 * c + 16, ls] = jnp.exp2(f).astype(BF16)
                if nkb >= 2:
                    o = 256 if nkb == 3 else 128
                    for c in range(8):
                        pref[128 + 16 * c:128 + 16 * c + 16, ls] = jnp.exp2(
                            s[o + 16 * c:o + 16 * c + 16]).astype(BF16)

        def pv(n, g, j, slot):
            nkb = blocks[n][1]
            nrow = 128 if nkb == 1 else 256
            vw = views[n][2]
            h = 4 * g + j
            pref = p_ld[slot]
            ls = slice(128 * j, 128 * (j + 1))
            pf = pref[0:64, ls]
            if nkb == 3:
                pnew = pf & pm_new
                p = jnp.concatenate([pf ^ pnew, pref[64:128, ls], pnew], axis=0)
            elif nkb == 2:
                p = jnp.concatenate([pref[64:128, ls], pf], axis=0)
            else:
                p = pf
            vt = vw[32 * h:32 * (h + 1), :]
            ot = jnp.dot(vt, pltpu.bitcast(p, BF16), preferred_element_type=F32)
            pp = p_l2[slot][0:nrow // 2, ls]
            x = (pltpu.bitcast(pp & U32(0xFFFF0000), F32)
                 + pltpu.bitcast(pp << 16, F32)).reshape(nrow // 16, 8, 128)
            while x.shape[0] > 1:
                m = x.shape[0] // 2
                x = x[:m] + x[m:]
            l = jnp.sum(x[0], axis=0, keepdims=True)
            am = jnp.max(jnp.abs(ot).reshape(4, 8, 128), axis=0)
            ok = (l >= L_LO) & (l <= L_HI) & (am <= F_MAX)
            good[n] = ok if good[n] is None else (good[n] & ok)
            o = (ot * (1.0 / l)).astype(BF16)
            otbufs[n][32 * (h % 16):32 * (h % 16) + 32,
                      128 * (h // 16):128 * (h // 16) + 128] = o

        l64 = lax.broadcasted_iota(I32, (16, QB), 1)
        lo16 = l64 < 64
        lo8 = lax.broadcasted_iota(I32, (8, QB), 1) < 64
        lo1 = lax.broadcasted_iota(I32, (1, QB), 1) < 64
        t64 = lax.broadcasted_iota(I32, (64, QB), 0)
        s64 = lax.broadcasted_iota(I32, (64, QB), 1) & 63
        new64 = t64 <= s64
        r32 = lax.broadcasted_iota(I32, (32, QB), 0) * 2
        c32 = lax.broadcasted_iota(I32, (32, QB), 1)
        lo32 = c32 < 64
        pn64 = (jnp.where(r32 <= (c32 & 63), U32(0xFFFF), U32(0))
                | jnp.where(r32 + 1 <= (c32 & 63), U32(0xFFFF0000), U32(0)))
        po64 = ~pn64
        zu = U32(0)

        def qk2(n, g, slot):
            qw, kw, _ = views[n]
            cs = slice(128 * g, 128 * (g + 1))
            pref = p_st[slot]
            for a in range(2):
                he = 4 * g + 2 * a
                xe = pltpu.bitcast(qw[32 * he:32 * he + 32, :], U32)
                xo = pltpu.roll(pltpu.bitcast(qw[32 * he + 32:32 * he + 64, :], U32), 64, 1)
                for u in range(2):
                    me = lo16 if u == 0 else jnp.logical_not(lo16)
                    wt = pltpu.bitcast(jnp.concatenate(
                        [jnp.where(me, xe, zu), jnp.where(me, zu, xo)], axis=0), BF16)
                    w = jnp.concatenate([zero32] * (2 * a) + [wt] + [zero32] * (2 - 2 * a), axis=0)
                    parts = []
                    for c in range(4):
                        parts.append(kw[64 * u + 16 * c:64 * u + 16 * c + 16, cs])
                        parts.append(kw[64 * u + 256 + 16 * c:64 * u + 256 + 16 * c + 16, cs])
                    parts.append(kw[64 * u + 64:64 * u + 256, cs])
                    s = jnp.dot(jnp.concatenate(parts, axis=0), w, preferred_element_type=F32)
                    ls = slice(128 * (2 * a + u), 128 * (2 * a + u + 1))
                    for c in range(4):
                        f = jnp.where(new64[16 * c:16 * c + 16], s[32 * c + 16:32 * c + 32],
                                      s[32 * c:32 * c + 16])
                        pref[16 * c:16 * c + 16, ls] = jnp.exp2(f).astype(BF16)
                    for c in range(12):
                        pref[64 + 16 * c:64 + 16 * c + 16, ls] = jnp.exp2(
                            s[128 + 16 * c:128 + 16 * c + 16]).astype(BF16)

        def colsum(pp):
            x = (pltpu.bitcast(pp & U32(0xFFFF0000), F32)
                 + pltpu.bitcast(pp << 16, F32)).reshape(pp.shape[0] // 8, 8, 128)
            while x.shape[0] > 1:
                m = x.shape[0] // 2
                x = x[:m] + x[m:]
            return jnp.sum(x[0], axis=0, keepdims=True)

        def pv2(n, g, a, slot):
            vw = views[n][2]
            pref = p_ld[slot]
            c0 = slice(128 * (2 * a), 128 * (2 * a + 1))
            c1 = slice(128 * (2 * a + 1), 128 * (2 * a + 2))
            f0 = pref[0:32, c0]
            f1 = pref[0:32, c1]
            n0 = f0 & pn64
            o0 = f0 ^ n0
            n1 = f1 & pn64
            o1 = f1 ^ n1
            m0 = [pref[32 + 32 * b:64 + 32 * b, c0] for b in range(3)]
            m1 = [pref[32 + 32 * b:64 + 32 * b, c1] for b in range(3)]
            l0 = colsum(p_l2[slot][:, c0])
            l1 = colsum(p_l2[slot][:, c1])
            for e in range(2):
                h = 4 * g + 2 * a + e
                if e == 0:
                    tiles = [jnp.where(lo32, o0, zu), jnp.where(lo32, m0[0], o1),
                             jnp.where(lo32, m0[1], m1[0]), jnp.where(lo32, m0[2], m1[1]),
                             jnp.where(lo32, n0, m1[2]), jnp.where(lo32, zu, n1)]
                    l = jnp.where(lo1, l0, l1)
                else:
                    tiles = [jnp.where(lo32, zu, o0), jnp.where(lo32, o1, m0[0]),
                             jnp.where(lo32, m1[0], m0[1]), jnp.where(lo32, m1[1], m0[2]),
                             jnp.where(lo32, m1[2], n0), jnp.where(lo32, n1, zu)]
                    l = jnp.where(lo1, l1, l0)
                p = pltpu.bitcast(jnp.concatenate(tiles, axis=0), BF16)
                ot = jnp.dot(vw[32 * h:32 * (h + 1), :], p, preferred_element_type=F32)
                am = jnp.max(jnp.abs(ot).reshape(4, 8, 128), axis=0)
                ok = (l >= L_LO) & (l <= L_HI) & (am <= F_MAX)
                good[n] = ok if good[n] is None else (good[n] & ok)
                o = ot * (1.0 / l)
                if e == 1:
                    o = pltpu.roll(o, 64, 1)
                otbufs[n][32 * (h % 16):32 * (h % 16) + 32,
                          128 * (h // 16):128 * (h // 16) + 128] = o.astype(BF16)

        seq = [(n, g) for n in range(len(blocks)) for g in range(8)]
        for s in range(len(seq) + 2):
            if s < len(seq):
                n, g = seq[s]
                (qk2 if blocks[n][1] == 3 else qk)(n, g, s % 3)
            if s >= 2:
                n, g = seq[s - 2]
                if blocks[n][1] == 3:
                    for a in range(2):
                        pv2(n, g, a, (s - 2) % 3)
                else:
                    for j in range(4):
                        pv(n, g, j, (s - 2) % 3)
        for n in range(len(blocks)):
            flag[n] = jnp.min(jnp.where(good[n], 1, 0))

    def attention_safe(i, ow):
        r0 = _mo(i * QB, QB)
        start = pl.multiple_of(jnp.maximum(i - 2, 0) * QB, QB)
        qw = qt_b.at[:, pl.ds(r0, QB)]
        kw = k_b.at[pl.ds(start, 3 * QB), :]
        vw = vt_b.at[:, pl.ds(start, 3 * QB)]
        key = lax.broadcasted_iota(I32, (3 * QB, QB), 0) + start
        qry = lax.broadcasted_iota(I32, (3 * QB, QB), 1) + r0
        valid = (qry - key >= 0) & (qry - key < WIN)
        drow = lax.broadcasted_iota(I32, (128, QB), 0)

        def head(h, carry):
            g0 = pl.multiple_of((h // 4) * 128, 128)
            j0 = (h % 4) * 32
            q4 = qw[pl.ds(g0, 128), :].astype(F32)
            w = jnp.where((drow >= j0) & (drow < j0 + 32), q4, 0.0).astype(BF16)
            s = jnp.dot(kw[:, pl.ds(g0, 128)], w, preferred_element_type=F32)
            s = jnp.where(valid, s, NEG)
            m = jnp.max(s, axis=0, keepdims=True)
            p = jnp.exp2(s - m).astype(BF16)
            l = jnp.sum(p.astype(F32), axis=0, keepdims=True)
            vt = vw[pl.ds(pl.multiple_of(h * 32, 32), 32), :]
            o = jnp.dot(vt, p, preferred_element_type=F32) * (1.0 / l)
            ow[pl.ds(pl.multiple_of((h % 16) * 32, 32), 32),
               pl.ds(pl.multiple_of((h // 16) * 128, 128), 128)] = o.astype(BF16)
            return carry

        lax.fori_loop(0, NH, head, 0)

    def out_proj(n, xsrc, x1dst, z=0):
        ow = ot_b.at[n + z]
        o = jnp.concatenate([ow[:, 0:128], ow[:, 128:256]], axis=0)
        y = lax.dot_general(o, wo[...], TN, preferred_element_type=F32)
        x1dst[...] = (xsrc[...].astype(F32) + y).astype(BF16)

    def ln2(b, x1src, x2dst, CH=16, NCHAIN=2, z_in=0):
        rb = _mo(b * QB, QB)
        wr = wr_ref[...].astype(F32).reshape(1, D)
        wsum = jnp.sum(wr, axis=-1, keepdims=True)
        bm = None
        bi = None
        sub = lax.broadcasted_iota(I32, (8, 1), 0)
        toks = []
        for c in range(QB // CH):
            z = toks[c - NCHAIN] if c >= NCHAIN else z_in
            if isinstance(z, int):
                x1 = x1src[CH * c:CH * (c + 1), :].astype(F32)
            else:
                x1 = x1src[pl.ds(pl.multiple_of(CH * c + z * 16, 16), CH), :].astype(F32)
            m, rs = _ln_stats(x1)
            x2dst[CH * c:CH * (c + 1), :] = (x1 * (1.0 + rs) - m * rs).astype(BF16)
            r = _rnd(rs * (jnp.sum(x1 * wr, axis=-1, keepdims=True) - m * wsum))
            ru = lax.bitcast_convert_type(r, I32)
            toks.append(jnp.max(lax.shift_right_logical(lax.shift_right_logical(ru, 16), 16)))
            for t in range(CH // 8):
                rt = r[8 * t:8 * t + 8]
                it = sub + (rb + CH * c + 8 * t)
                if bm is None:
                    bm, bi = rt, it
                else:
                    better = rt > bm
                    bm = jnp.where(better, rt, bm)
                    bi = jnp.where(better, it, bi)
        bmax_ref[b] = jnp.broadcast_to(bm, (8, 128))
        bidx_ref[b] = jnp.broadcast_to(bi, (8, 128))
        tok = toks[-1]
        for k in range(2, min(NCHAIN, len(toks)) + 1):
            tok = tok + toks[-k]
        return tok

    def checks(i0):
        def one(n, carry):
            @pl.when(flag[n] == 0)
            def _():
                rb = pl.multiple_of((i0 + n) * QB, QB)
                attention_safe(i0 + n, ot_b.at[n])
                out_proj(n, xn.at[pl.ds(rb, QB), :], x1_b.at[pl.ds(rb, QB), :])
            return carry

        @pl.when(flag[0] + flag[1] < 2)
        def _():
            lax.fori_loop(0, 2, one, 0)

    def out_copy(b):
        return pltpu.make_async_copy(xn.at[pl.ds(b * QB, QB), :],
                                     out_hbm.at[pl.ds(b * QB, QB), :], sem_o.at[0])

    def phase_b(layer):
        attention([(0, 1), (1, 2)])
        out_proj(0, xn.at[0:QB, :], x1_b.at[0:QB, :])
        out_proj(1, xn.at[QB:2 * QB, :], x1_b.at[QB:2 * QB, :])

        def body(t, carry):
            i0 = 2 * t
            checks(i0 - 2)

            @pl.when(jnp.logical_and(layer == 1, t >= 2))
            def _():
                out_copy(i0 - 4).start()
                out_copy(i0 - 3).start()

            @pl.when(t < NQB // 2)
            def _():
                r2 = pl.multiple_of((i0 - 2) * QB, QB)
                xv = xn.at[pl.ds(r2, 4 * QB), :]
                x1v = x1_b.at[pl.ds(r2, 4 * QB), :]
                ln2(i0 - 2, x1v.at[0:QB, :], xv.at[0:QB, :])
                ln2(i0 - 1, x1v.at[QB:2 * QB, :], xv.at[QB:2 * QB, :])
                attention([(i0, 3), (i0 + 1, 3)])
                out_proj(0, xv.at[2 * QB:3 * QB, :], x1v.at[2 * QB:3 * QB, :])
                out_proj(1, xv.at[3 * QB:4 * QB, :], x1v.at[3 * QB:4 * QB, :])
            return carry

        lax.fori_loop(1, NQB // 2 + 1, body, 0)
        for b in (NQB - 2, NQB - 1):
            ln2(b, x1_b.at[b * QB:(b + 1) * QB, :], xn.at[b * QB:(b + 1) * QB, :], NCHAIN=8)

        @pl.when(layer == 1)
        def _():
            out_copy(NQB - 2).start()
            out_copy(NQB - 1).start()

    def moe(layer):
        rm = bmax_ref[:, :, 0:1]
        ri = bidx_ref[:, :, 0:1]
        gm = jnp.max(jnp.max(rm, axis=0), axis=0, keepdims=True)
        idx = jnp.min(jnp.where(rm == gm, ri, BIG))
        b16 = pl.multiple_of((idx // 16) * 16, 16)
        x1c = x1_b[pl.ds(b16, 16), :].astype(F32)
        h2c = _rnd(_ln(x1c))
        hb = h2c.astype(BF16)
        g = _rnd(jnp.dot(hb, wg[...], preferred_element_type=F32))
        u = _rnd(jnp.dot(hb, wu[...], preferred_element_type=F32))
        g = _rnd(g * _rnd(jax.nn.sigmoid(g)))
        act = (g * u).astype(BF16)
        y = _rnd(jnp.dot(act, wd[...], preferred_element_type=F32))
        y = _rnd(y * _rnd(jax.nn.sigmoid(gm)))
        x2n = x1c + _rnd(h2c + y)

        @pl.when(layer == 1)
        def _():
            for b in range(NQB):
                out_copy(b).wait()

        cur = xn[pl.ds(b16, 16), :].astype(F32)
        sel = lax.broadcasted_iota(I32, (16, D), 0) == (idx - b16)
        xn[pl.ds(b16, 16), :] = jnp.where(sel, x2n, cur).astype(BF16)

        @pl.when(layer == 1)
        def _():
            cp = pltpu.make_async_copy(xn.at[pl.ds(b16, 16), :],
                                       out_hbm.at[pl.ds(b16, 16), :], sem_o.at[1])
            cp.start()
            cp.wait()

    def layer_body(layer, carry):
        phase_a(layer)

        @pl.when(layer == 0)
        def _():
            w_copies[0].wait()

        phase_b(layer)

        @pl.when(layer == 0)
        def _():
            for c in w_copies[1:]:
                c.wait()

        moe(layer)

        @pl.when(layer == 0)
        def _():
            ln1(0, hbufs[0])

        return carry

    lax.fori_loop(0, 2, layer_body, 0)


@jax.jit
def pallas_interleave_layers__sliding_block__moe_arch_mod__prompt_kernel(
    A_x: jax.Array,
    A_wqkv: jax.Array,
    A_wo: jax.Array,
    B_x: jax.Array,
    B_w_r: jax.Array,
    B_w_gate: jax.Array,
    B_w_up: jax.Array,
    B_w_down: jax.Array,
):
    del B_x
    hbm = pl.BlockSpec(memory_space=pl.ANY)
    scratch = [
        pltpu.VMEM((S // 2, D), U32),
        pltpu.VMEM((S // 2, D), U32),
        pltpu.VMEM((MB // 2, D), U32),
        pltpu.VMEM((MB // 2, D), U32),
        pltpu.VMEM((D // 2, S), U32),
        pltpu.VMEM((S // 2, D), U32),
        pltpu.VMEM((D // 2, S), U32),
        pltpu.VMEM((D // 2, 3 * D), U32),
        pltpu.VMEM((D, D), U32),
        pltpu.VMEM((D // 2, D), U32),
        pltpu.VMEM((D // 2, FF), U32),
        pltpu.VMEM((D // 2, FF), U32),
        pltpu.VMEM((FF // 2, D), U32),
        pltpu.VMEM((1, 128, 512), U32),
        pltpu.VMEM((1, 128, 512), U32),
        pltpu.VMEM((1, 128, 512), U32),
        pltpu.VMEM((2, 256, 256), U32),
        pltpu.VMEM((NQB, 8, 128), F32),
        pltpu.VMEM((NQB, 8, 128), I32),
        pltpu.SMEM((4,), I32),
        pltpu.SMEM((2,), I32),
        pltpu.SemaphoreType.DMA((NMB,)),
        pltpu.SemaphoreType.DMA((7,)),
        pltpu.SemaphoreType.DMA((2,)),
    ]
    out = pl.pallas_call(
        _kernel,
        out_shape=jax.ShapeDtypeStruct((S, D), BF16),
        in_specs=[hbm, hbm, hbm, pl.BlockSpec(memory_space=pltpu.VMEM), hbm, hbm, hbm],
        out_specs=hbm,
        scratch_shapes=scratch,
        compiler_params=pltpu.CompilerParams(vmem_limit_bytes=110 * 1024 * 1024),
        name="swa_moe_fused",
    )(A_x.reshape(S, D), A_wqkv, A_wo, B_w_r, B_w_gate, B_w_up, B_w_down)
    return out.reshape(1, S, D)
```

```python
import math

import jax
import jax.numpy as jnp
from jax import lax
import jax.experimental.pallas as pl
import jax.experimental.pallas.tpu as pltpu

S = 2048
D = 1024
NH = 32
DH = 32
WIN = 256
FF = 3584
QB = 128
NQB = S // QB
MB = 256
NMB = S // MB
EPS = 1e-5
QSCALE = (DH ** -0.5) * math.log2(math.e)
NEG = -1e30
BIG = 2 ** 30
L_LO = 2.0 ** -64
L_HI = 2.0 ** 64
F_MAX = 3.0e38

F32 = jnp.float32
BF16 = jnp.bfloat16
U32 = jnp.uint32
I32 = jnp.int32

NT = (((1,), (1,)), ((), ()))
TN = (((0,), (0,)), ((), ()))


def _rnd(v):
    return v.astype(BF16).astype(F32)


def _ln(xf):
    m = jnp.mean(xf, axis=-1, keepdims=True)
    xc = xf - m
    v = jnp.mean(xc * xc, axis=-1, keepdims=True)
    return xc * lax.rsqrt(v + EPS)


def _ln_stats(xf):
    m = jnp.sum(xf, axis=-1, keepdims=True) * (1.0 / D)
    v = jnp.sum(xf * xf, axis=-1, keepdims=True) * (1.0 / D) - m * m
    return m, lax.rsqrt(jnp.maximum(v, 0.0) + EPS)


def _mo(v, m):
    return v if isinstance(v, int) else pl.multiple_of(v, m)


def _kernel(x_hbm, wqkv_hbm, wo_hbm, wr_ref, wg_hbm, wu_hbm, wd_hbm, out_hbm,
            xn_u, x1_u, h0_u, h1_u, qt_u, k_u, vt_u,
            wqkv_u, wqvt_u, wo_u, wg_u, wu_u, wd_u,
            p0, p1, p2, ot_u, bmax_ref, bidx_ref, zs, flag,
            sem_x, sem_w, sem_o):
    xn = xn_u.bitcast(BF16)
    x1_b = x1_u.bitcast(BF16)
    hbufs = (h0_u.bitcast(BF16), h1_u.bitcast(BF16))
    qt_b = qt_u.bitcast(BF16)
    k_b = k_u.bitcast(BF16)
    vt_b = vt_u.bitcast(BF16)
    wqkv = wqkv_u.bitcast(BF16)
    wqvt = wqvt_u.bitcast(BF16)
    wo = wo_u.bitcast(BF16)
    wg = wg_u.bitcast(BF16)
    wu = wu_u.bitcast(BF16)
    wd = wd_u.bitcast(BF16)
    ot_b = ot_u.bitcast(BF16)
    otbufs = (ot_b.at[0], ot_b.at[1])
    pbufs_u = (p0, p1, p2)
    pbufs_b = tuple(p.bitcast(BF16) for p in pbufs_u)

    def x_copy(j):
        return pltpu.make_async_copy(x_hbm.at[pl.ds(j * MB, MB), :],
                                     xn.at[pl.ds(j * MB, MB), :], sem_x.at[j])

    def wqkv_copy(c0, n, k):
        return pltpu.make_async_copy(wqkv_hbm.at[:, pl.ds(c0, n)],
                                     wqkv.at[:, pl.ds(c0, n)], sem_w.at[k])

    HD = D // 2
    wq_copies = [wqkv_copy(0, HD, 0), wqkv_copy(HD, HD, 1)]
    wv_copies = [wqkv_copy(2 * D, HD, 2), wqkv_copy(2 * D + HD, HD, 7)]
    wk_copy = wqkv_copy(D, D, 8)

    w_copies = [
        pltpu.make_async_copy(wo_hbm, wo, sem_w.at[3]),
        pltpu.make_async_copy(wg_hbm, wg, sem_w.at[4]),
        pltpu.make_async_copy(wu_hbm, wu, sem_w.at[5]),
        pltpu.make_async_copy(wd_hbm, wd, sem_w.at[6]),
    ]
    x_copy(0).start()
    wq_copies[0].start()
    wq_copies[1].start()
    wv_copies[0].start()
    wv_copies[1].start()
    x_copy(1).start()
    x_copy(2).start()
    wk_copy.start()
    for j in range(3, NMB):
        x_copy(j).start()

    for t in range(4):
        zs[t] = 0

    eye = (lax.broadcasted_iota(I32, (128, 128), 0)
           == lax.broadcasted_iota(I32, (128, 128), 1)).astype(F32).astype(BF16)

    def transpose_w(src_col0, dst_row0, tiles):
        for t in tiles:
            w_t = wqkv[:, src_col0 + 128 * t:src_col0 + 128 * (t + 1)]
            wqvt[dst_row0 + 128 * t:dst_row0 + 128 * (t + 1), :] = lax.dot_general(
                eye, w_t, NT, preferred_element_type=F32).astype(BF16)

    def ln1(row0, dst):
        src = xn.at[pl.ds(row0, MB), :]
        for c in range(MB // 64):
            xf = src[64 * c:64 * (c + 1), :].astype(F32)
            dst[64 * c:64 * (c + 1), :] = _ln(xf).astype(BF16)

    def proj_t(row0, n, base, hsrc):
        r = lax.dot_general(wqvt[row0:row0 + n, :], hsrc[...], NT, preferred_element_type=F32)
        if row0 < D:
            qt_b[row0:row0 + n, pl.ds(base, MB)] = (r * QSCALE).astype(BF16)
        else:
            vt_b[row0 - D:row0 - D + n, pl.ds(base, MB)] = r.astype(BF16)

    def proj_qv(base, hsrc):
        qv = lax.dot_general(wqvt[...], hsrc[...], NT, preferred_element_type=F32)
        qt_b[:, pl.ds(base, MB)] = (qv[0:D] * QSCALE).astype(BF16)
        vt_b[:, pl.ds(base, MB)] = qv[D:2 * D].astype(BF16)

    def proj_k(base, hsrc):
        k = jnp.dot(hsrc[...], wqkv[:, D:2 * D], preferred_element_type=F32)
        k_b[pl.ds(base, MB), :] = k.astype(BF16)

    def phase_a(layer):
        def body(t, carry):
            first = jnp.logical_and(layer == 0, t == 0)

            @pl.when(first)
            def _():
                x_copy(1).wait()
                x_copy(2).wait()
                wk_copy.wait()
                for c in w_copies:
                    c.start()

            @pl.when(jnp.logical_and(layer == 0, t >= 1))
            def _():
                x_copy(2 * t + 1).wait()

            @pl.when(jnp.logical_and(layer == 0, jnp.logical_and(t >= 1, t < NMB // 2 - 1)))
            def _():
                x_copy(2 * t + 2).wait()

            b0 = pl.multiple_of(2 * t * MB, MB)
            b1 = pl.multiple_of(b0 + MB, MB)
            b2 = pl.multiple_of(jnp.minimum(2 * t + 2, NMB - 1) * MB, MB)

            @pl.when(jnp.logical_not(first))
            def _():
                proj_qv(b0, hbufs[0])

            proj_k(b0, hbufs[0])
            ln1(b1, hbufs[1])
            proj_qv(b1, hbufs[1])
            proj_k(b1, hbufs[1])
            ln1(b2, hbufs[0])
            return carry

        lax.fori_loop(0, NMB // 2, body, 0)

    x_copy(0).wait()
    ln1(0, hbufs[0])
    for k in range(2):
        wq_copies[k].wait()
        transpose_w(k * HD, k * HD, range(4))
        proj_t(k * HD, HD, 0, hbufs[0])
    for k in range(2):
        wv_copies[k].wait()
        transpose_w(2 * D + k * HD, D + k * HD, range(4))
        proj_t(D + k * HD, HD, 0, hbufs[0])

    def attention(blocks):
        zst = zs[0]
        zld = zs[1]
        zl2 = zs[2]
        lane = lax.broadcasted_iota(I32, (QB, QB), 1)
        row = lax.broadcasted_iota(I32, (QB, QB), 0)
        newmask = row <= lane
        l2 = lax.broadcasted_iota(I32, (QB // 2, QB), 1)
        r2 = lax.broadcasted_iota(I32, (QB // 2, QB), 0) * 2
        pm_new = (jnp.where(r2 <= l2, U32(0xFFFF), U32(0))
                  | jnp.where(r2 + 1 <= l2, U32(0xFFFF0000), U32(0)))
        p_st = [p.at[zst] for p in pbufs_b]
        p_ld = [p.at[zld] for p in pbufs_u]
        p_l2 = [p.at[zl2] for p in pbufs_u]
        zero32 = jnp.zeros((32, QB), BF16)
        good = [None] * len(blocks)
        views = []
        for (i, nkb) in blocks:
            r0 = _mo(i * QB, QB)
            k0 = 128 * (nkb - 1)
            views.append((qt_b.at[:, pl.ds(r0, QB)],
                          k_b.at[pl.ds(r0 - k0, k0 + QB), :],
                          vt_b.at[:, pl.ds(r0 - k0, k0 + QB)]))

        def qk(n, g, slot):
            nkb = blocks[n][1]
            k0 = 128 * (nkb - 1)
            qw, kw, _ = views[n]
            cs = slice(128 * g, 128 * (g + 1))
            ws = []
            for j in range(4):
                h = 4 * g + j
                ws.append(jnp.concatenate(
                    [zero32] * j + [qw[32 * h:32 * (h + 1), :]] + [zero32] * (3 - j), axis=0))
            w = jnp.concatenate(ws, axis=1)
            parts = []
            if nkb == 3:
                for c in range(8):
                    parts.append(kw[16 * c:16 * c + 16, cs])
                    parts.append(kw[256 + 16 * c:256 + 16 * c + 16, cs])
            else:
                parts.append(kw[k0:k0 + 128, cs])
            if nkb >= 2:
                parts.append(kw[k0 - 128:k0, cs])
            kk = jnp.concatenate(parts, axis=0)
            st = jnp.dot(kk, w, preferred_element_type=F32)
            pref = p_st[slot]
            for j in range(4):
                s = st[:, 128 * j:128 * (j + 1)]
                ls = slice(128 * j, 128 * (j + 1))
                for c in range(8):
                    nm = newmask[16 * c:16 * c + 16]
                    if nkb == 3:
                        f = jnp.where(nm, s[32 * c + 16:32 * c + 32], s[32 * c:32 * c + 16])
                    else:
                        f = jnp.where(nm, s[16 * c:16 * c + 16], NEG)
                    pref[16 * c:16 * c + 16, ls] = jnp.exp2(f).astype(BF16)
                if nkb >= 2:
                    o = 256 if nkb == 3 else 128
                    for c in range(8):
                        pref[128 + 16 * c:128 + 16 * c + 16, ls] = jnp.exp2(
                            s[o + 16 * c:o + 16 * c + 16]).astype(BF16)

        def pv(n, g, j, slot):
            nkb = blocks[n][1]
            nrow = 128 if nkb == 1 else 256
            vw = views[n][2]
            h = 4 * g + j
            pref = p_ld[slot]
            ls = slice(128 * j, 128 * (j + 1))
            pf = pref[0:64, ls]
            if nkb == 3:
                pnew = pf & pm_new
                p = jnp.concatenate([pf ^ pnew, pref[64:128, ls], pnew], axis=0)
            elif nkb == 2:
                p = jnp.concatenate([pref[64:128, ls], pf], axis=0)
            else:
                p = pf
            vt = vw[32 * h:32 * (h + 1), :]
            ot = jnp.dot(vt, pltpu.bitcast(p, BF16), preferred_element_type=F32)
            pp = p_l2[slot][0:nrow // 2, ls]
            x = (pltpu.bitcast(pp & U32(0xFFFF0000), F32)
                 + pltpu.bitcast(pp << 16, F32)).reshape(nrow // 16, 8, 128)
            while x.shape[0] > 1:
                m = x.shape[0] // 2
                x = x[:m] + x[m:]
            l = jnp.sum(x[0], axis=0, keepdims=True)
            am = jnp.max(jnp.abs(ot).reshape(4, 8, 128), axis=0)
            ok = (l >= L_LO) & (l <= L_HI) & (am <= F_MAX)
            good[n] = ok if good[n] is None else (good[n] & ok)
            o = (ot * (1.0 / l)).astype(BF16)
            otbufs[n][32 * (h % 16):32 * (h % 16) + 32,
                      128 * (h // 16):128 * (h // 16) + 128] = o

        l64 = lax.broadcasted_iota(I32, (16, QB), 1)
        lo16 = l64 < 64
        lo8 = lax.broadcasted_iota(I32, (8, QB), 1) < 64
        lo1 = lax.broadcasted_iota(I32, (1, QB), 1) < 64
        t64 = lax.broadcasted_iota(I32, (64, QB), 0)
        s64 = lax.broadcasted_iota(I32, (64, QB), 1) & 63
        new64 = t64 <= s64
        r32 = lax.broadcasted_iota(I32, (32, QB), 0) * 2
        c32 = lax.broadcasted_iota(I32, (32, QB), 1)
        lo32 = c32 < 64
        pn64 = (jnp.where(r32 <= (c32 & 63), U32(0xFFFF), U32(0))
                | jnp.where(r32 + 1 <= (c32 & 63), U32(0xFFFF0000), U32(0)))
        po64 = ~pn64
        zu = U32(0)

        def qk2(n, g, slot):
            qw, kw, _ = views[n]
            cs = slice(128 * g, 128 * (g + 1))
            pref = p_st[slot]
            for a in range(2):
                he = 4 * g + 2 * a
                xe = pltpu.bitcast(qw[32 * he:32 * he + 32, :], U32)
                xo = pltpu.roll(pltpu.bitcast(qw[32 * he + 32:32 * he + 64, :], U32), 64, 1)
                for u in range(2):
                    me = lo16 if u == 0 else jnp.logical_not(lo16)
                    wt = pltpu.bitcast(jnp.concatenate(
                        [jnp.where(me, xe, zu), jnp.where(me, zu, xo)], axis=0), BF16)
                    w = jnp.concatenate([zero32] * (2 * a) + [wt] + [zero32] * (2 - 2 * a), axis=0)
                    parts = []
                    for c in range(4):
                        parts.append(kw[64 * u + 16 * c:64 * u + 16 * c + 16, cs])
                        parts.append(kw[64 * u + 256 + 16 * c:64 * u + 256 + 16 * c + 16, cs])
                    parts.append(kw[64 * u + 64:64 * u + 256, cs])
                    s = jnp.dot(jnp.concatenate(parts, axis=0), w, preferred_element_type=F32)
                    ls = slice(128 * (2 * a + u), 128 * (2 * a + u + 1))
                    for c in range(4):
                        f = jnp.where(new64[16 * c:16 * c + 16], s[32 * c + 16:32 * c + 32],
                                      s[32 * c:32 * c + 16])
                        pref[16 * c:16 * c + 16, ls] = jnp.exp2(f).astype(BF16)
                    for c in range(12):
                        pref[64 + 16 * c:64 + 16 * c + 16, ls] = jnp.exp2(
                            s[128 + 16 * c:128 + 16 * c + 16]).astype(BF16)

        def colsum(pp):
            x = (pltpu.bitcast(pp & U32(0xFFFF0000), F32)
                 + pltpu.bitcast(pp << 16, F32)).reshape(pp.shape[0] // 8, 8, 128)
            while x.shape[0] > 1:
                m = x.shape[0] // 2
                x = x[:m] + x[m:]
            return jnp.sum(x[0], axis=0, keepdims=True)

        def pv2(n, g, a, slot):
            vw = views[n][2]
            pref = p_ld[slot]
            c0 = slice(128 * (2 * a), 128 * (2 * a + 1))
            c1 = slice(128 * (2 * a + 1), 128 * (2 * a + 2))
            f0 = pref[0:32, c0]
            f1 = pref[0:32, c1]
            n0 = f0 & pn64
            o0 = f0 ^ n0
            n1 = f1 & pn64
            o1 = f1 ^ n1
            m0 = [pref[32 + 32 * b:64 + 32 * b, c0] for b in range(3)]
            m1 = [pref[32 + 32 * b:64 + 32 * b, c1] for b in range(3)]
            l0 = colsum(p_l2[slot][:, c0])
            l1 = colsum(p_l2[slot][:, c1])
            for e in range(2):
                h = 4 * g + 2 * a + e
                if e == 0:
                    tiles = [jnp.where(lo32, o0, zu), jnp.where(lo32, m0[0], o1),
                             jnp.where(lo32, m0[1], m1[0]), jnp.where(lo32, m0[2], m1[1]),
                             jnp.where(lo32, n0, m1[2]), jnp.where(lo32, zu, n1)]
                    l = jnp.where(lo1, l0, l1)
                else:
                    tiles = [jnp.where(lo32, zu, o0), jnp.where(lo32, o1, m0[0]),
                             jnp.where(lo32, m1[0], m0[1]), jnp.where(lo32, m1[1], m0[2]),
                             jnp.where(lo32, m1[2], n0), jnp.where(lo32, n1, zu)]
                    l = jnp.where(lo1, l1, l0)
                p = pltpu.bitcast(jnp.concatenate(tiles, axis=0), BF16)
                ot = jnp.dot(vw[32 * h:32 * (h + 1), :], p, preferred_element_type=F32)
                am = jnp.max(jnp.abs(ot).reshape(4, 8, 128), axis=0)
                ok = (l >= L_LO) & (l <= L_HI) & (am <= F_MAX)
                good[n] = ok if good[n] is None else (good[n] & ok)
                o = ot * (1.0 / l)
                if e == 1:
                    o = pltpu.roll(o, 64, 1)
                otbufs[n][32 * (h % 16):32 * (h % 16) + 32,
                          128 * (h // 16):128 * (h // 16) + 128] = o.astype(BF16)

        seq = [(n, g) for n in range(len(blocks)) for g in range(8)]
        for s in range(len(seq) + 2):
            if s < len(seq):
                n, g = seq[s]
                (qk2 if blocks[n][1] == 3 else qk)(n, g, s % 3)
            if s >= 2:
                n, g = seq[s - 2]
                if blocks[n][1] == 3:
                    for a in range(2):
                        pv2(n, g, a, (s - 2) % 3)
                else:
                    for j in range(4):
                        pv(n, g, j, (s - 2) % 3)
        for n in range(len(blocks)):
            flag[n] = jnp.min(jnp.where(good[n], 1, 0))

    def attention_safe(i, ow):
        r0 = _mo(i * QB, QB)
        start = pl.multiple_of(jnp.maximum(i - 2, 0) * QB, QB)
        qw = qt_b.at[:, pl.ds(r0, QB)]
        kw = k_b.at[pl.ds(start, 3 * QB), :]
        vw = vt_b.at[:, pl.ds(start, 3 * QB)]
        key = lax.broadcasted_iota(I32, (3 * QB, QB), 0) + start
        qry = lax.broadcasted_iota(I32, (3 * QB, QB), 1) + r0
        valid = (qry - key >= 0) & (qry - key < WIN)
        drow = lax.broadcasted_iota(I32, (128, QB), 0)

        def head(h, carry):
            g0 = pl.multiple_of((h // 4) * 128, 128)
            j0 = (h % 4) * 32
            q4 = qw[pl.ds(g0, 128), :].astype(F32)
            w = jnp.where((drow >= j0) & (drow < j0 + 32), q4, 0.0).astype(BF16)
            s = jnp.dot(kw[:, pl.ds(g0, 128)], w, preferred_element_type=F32)
            s = jnp.where(valid, s, NEG)
            m = jnp.max(s, axis=0, keepdims=True)
            p = jnp.exp2(s - m).astype(BF16)
            l = jnp.sum(p.astype(F32), axis=0, keepdims=True)
            vt = vw[pl.ds(pl.multiple_of(h * 32, 32), 32), :]
            o = jnp.dot(vt, p, preferred_element_type=F32) * (1.0 / l)
            ow[pl.ds(pl.multiple_of((h % 16) * 32, 32), 32),
               pl.ds(pl.multiple_of((h // 16) * 128, 128), 128)] = o.astype(BF16)
            return carry

        lax.fori_loop(0, NH, head, 0)

    def out_proj(n, xsrc, x1dst, z=0):
        ow = ot_b.at[n + z]
        o = jnp.concatenate([ow[:, 0:128], ow[:, 128:256]], axis=0)
        y = lax.dot_general(o, wo[...], TN, preferred_element_type=F32)
        x1dst[...] = (xsrc[...].astype(F32) + y).astype(BF16)

    def ln2(b, x1src, x2dst, CH=16, NCHAIN=8, z_in=0):
        rb = _mo(b * QB, QB)
        wr = wr_ref[...].astype(F32).reshape(1, D)
        wsum = jnp.sum(wr, axis=-1, keepdims=True)
        bm = None
        bi = None
        sub = lax.broadcasted_iota(I32, (8, 1), 0)
        toks = []
        for c in range(QB // CH):
            z = toks[c - NCHAIN] if c >= NCHAIN else z_in
            if isinstance(z, int):
                x1 = x1src[CH * c:CH * (c + 1), :].astype(F32)
            else:
                x1 = x1src[pl.ds(pl.multiple_of(CH * c + z * 16, 16), CH), :].astype(F32)
            m, rs = _ln_stats(x1)
            x2dst[CH * c:CH * (c + 1), :] = (x1 * (1.0 + rs) - m * rs).astype(BF16)
            r = _rnd(rs * (jnp.sum(x1 * wr, axis=-1, keepdims=True) - m * wsum))
            ru = lax.bitcast_convert_type(r, I32)
            toks.append(jnp.max(lax.shift_right_logical(lax.shift_right_logical(ru, 16), 16)))
            for t in range(CH // 8):
                rt = r[8 * t:8 * t + 8]
                it = sub + (rb + CH * c + 8 * t)
                if bm is None:
                    bm, bi = rt, it
                else:
                    better = rt > bm
                    bm = jnp.where(better, rt, bm)
                    bi = jnp.where(better, it, bi)
        bmax_ref[b] = jnp.broadcast_to(bm, (8, 128))
        bidx_ref[b] = jnp.broadcast_to(bi, (8, 128))
        tok = toks[-1]
        for k in range(2, min(NCHAIN, len(toks)) + 1):
            tok = tok + toks[-k]
        return tok

    def checks(i0):
        def one(n, carry):
            @pl.when(flag[n] == 0)
            def _():
                rb = pl.multiple_of((i0 + n) * QB, QB)
                attention_safe(i0 + n, ot_b.at[n])
                out_proj(n, xn.at[pl.ds(rb, QB), :], x1_b.at[pl.ds(rb, QB), :])
            return carry

        @pl.when(flag[0] + flag[1] < 2)
        def _():
            lax.fori_loop(0, 2, one, 0)

    def out_copy(b):
        return pltpu.make_async_copy(xn.at[pl.ds(b * QB, QB), :],
                                     out_hbm.at[pl.ds(b * QB, QB), :], sem_o.at[0])

    def phase_b(layer):
        attention([(0, 1), (1, 2)])
        out_proj(0, xn.at[0:QB, :], x1_b.at[0:QB, :])
        out_proj(1, xn.at[QB:2 * QB, :], x1_b.at[QB:2 * QB, :])

        def body(t, carry):
            i0 = 2 * t
            checks(i0 - 2)

            @pl.when(jnp.logical_and(layer == 1, t >= 2))
            def _():
                out_copy(i0 - 4).start()
                out_copy(i0 - 3).start()

            @pl.when(t < NQB // 2)
            def _():
                r2 = pl.multiple_of((i0 - 2) * QB, QB)
                xv = xn.at[pl.ds(r2, 4 * QB), :]
                x1v = x1_b.at[pl.ds(r2, 4 * QB), :]
                ln2(i0 - 2, x1v.at[0:QB, :], xv.at[0:QB, :])
                ln2(i0 - 1, x1v.at[QB:2 * QB, :], xv.at[QB:2 * QB, :])
                attention([(i0, 3), (i0 + 1, 3)])
                out_proj(0, xv.at[2 * QB:3 * QB, :], x1v.at[2 * QB:3 * QB, :])
                out_proj(1, xv.at[3 * QB:4 * QB, :], x1v.at[3 * QB:4 * QB, :])
            return carry

        lax.fori_loop(1, NQB // 2 + 1, body, 0)
        for b in (NQB - 2, NQB - 1):
            ln2(b, x1_b.at[b * QB:(b + 1) * QB, :], xn.at[b * QB:(b + 1) * QB, :], NCHAIN=8)

        @pl.when(layer == 1)
        def _():
            out_copy(NQB - 2).start()
            out_copy(NQB - 1).start()

    def moe(layer):
        rm = bmax_ref[:, :, 0:1]
        ri = bidx_ref[:, :, 0:1]
        gm = jnp.max(jnp.max(rm, axis=0), axis=0, keepdims=True)
        idx = jnp.min(jnp.where(rm == gm, ri, BIG))
        b16 = pl.multiple_of((idx // 16) * 16, 16)
        x1c = x1_b[pl.ds(b16, 16), :].astype(F32)
        h2c = _rnd(_ln(x1c))
        hb = h2c.astype(BF16)
        g = _rnd(jnp.dot(hb, wg[...], preferred_element_type=F32))
        u = _rnd(jnp.dot(hb, wu[...], preferred_element_type=F32))
        g = _rnd(g * _rnd(jax.nn.sigmoid(g)))
        act = (g * u).astype(BF16)
        y = _rnd(jnp.dot(act, wd[...], preferred_element_type=F32))
        y = _rnd(y * _rnd(jax.nn.sigmoid(gm)))
        x2n = x1c + _rnd(h2c + y)

        @pl.when(layer == 1)
        def _():
            for b in range(NQB):
                out_copy(b).wait()

        cur = xn[pl.ds(b16, 16), :].astype(F32)
        sel = lax.broadcasted_iota(I32, (16, D), 0) == (idx - b16)
        xn[pl.ds(b16, 16), :] = jnp.where(sel, x2n, cur).astype(BF16)

        @pl.when(layer == 1)
        def _():
            cp = pltpu.make_async_copy(xn.at[pl.ds(b16, 16), :],
                                       out_hbm.at[pl.ds(b16, 16), :], sem_o.at[1])
            cp.start()
            cp.wait()

    def layer_body(layer, carry):
        phase_a(layer)

        @pl.when(layer == 0)
        def _():
            w_copies[0].wait()

        phase_b(layer)

        @pl.when(layer == 0)
        def _():
            for c in w_copies[1:]:
                c.wait()

        moe(layer)

        @pl.when(layer == 0)
        def _():
            ln1(0, hbufs[0])

        return carry

    lax.fori_loop(0, 2, layer_body, 0)


@jax.jit
def pallas_interleave_layers__sliding_block__moe_arch_mod__prompt_kernel(
    A_x: jax.Array,
    A_wqkv: jax.Array,
    A_wo: jax.Array,
    B_x: jax.Array,
    B_w_r: jax.Array,
    B_w_gate: jax.Array,
    B_w_up: jax.Array,
    B_w_down: jax.Array,
):
    del B_x
    hbm = pl.BlockSpec(memory_space=pl.ANY)
    scratch = [
        pltpu.VMEM((S // 2, D), U32),
        pltpu.VMEM((S // 2, D), U32),
        pltpu.VMEM((MB // 2, D), U32),
        pltpu.VMEM((MB // 2, D), U32),
        pltpu.VMEM((D // 2, S), U32),
        pltpu.VMEM((S // 2, D), U32),
        pltpu.VMEM((D // 2, S), U32),
        pltpu.VMEM((D // 2, 3 * D), U32),
        pltpu.VMEM((D, D), U32),
        pltpu.VMEM((D // 2, D), U32),
        pltpu.VMEM((D // 2, FF), U32),
        pltpu.VMEM((D // 2, FF), U32),
        pltpu.VMEM((FF // 2, D), U32),
        pltpu.VMEM((1, 128, 512), U32),
        pltpu.VMEM((1, 128, 512), U32),
        pltpu.VMEM((1, 128, 512), U32),
        pltpu.VMEM((2, 256, 256), U32),
        pltpu.VMEM((NQB, 8, 128), F32),
        pltpu.VMEM((NQB, 8, 128), I32),
        pltpu.SMEM((4,), I32),
        pltpu.SMEM((2,), I32),
        pltpu.SemaphoreType.DMA((NMB,)),
        pltpu.SemaphoreType.DMA((9,)),
        pltpu.SemaphoreType.DMA((2,)),
    ]
    out = pl.pallas_call(
        _kernel,
        out_shape=jax.ShapeDtypeStruct((S, D), BF16),
        in_specs=[hbm, hbm, hbm, pl.BlockSpec(memory_space=pltpu.VMEM), hbm, hbm, hbm],
        out_specs=hbm,
        scratch_shapes=scratch,
        compiler_params=pltpu.CompilerParams(vmem_limit_bytes=110 * 1024 * 1024),
        name="swa_moe_fused",
    )(A_x.reshape(S, D), A_wqkv, A_wo, B_w_r, B_w_gate, B_w_up, B_w_down)
    return out.reshape(1, S, D)
```

```python
import math

import jax
import jax.numpy as jnp
from jax import lax
import jax.experimental.pallas as pl
import jax.experimental.pallas.tpu as pltpu

S = 2048
D = 1024
NH = 32
DH = 32
WIN = 256
FF = 3584
QB = 128
NQB = S // QB
MB = 256
NMB = S // MB
EPS = 1e-5
QSCALE = (DH ** -0.5) * math.log2(math.e)
NEG = -1e30
BIG = 2 ** 30
L_LO = 2.0 ** -64
L_HI = 2.0 ** 64
F_MAX = 3.0e38

F32 = jnp.float32
BF16 = jnp.bfloat16
U32 = jnp.uint32
I32 = jnp.int32

NT = (((1,), (1,)), ((), ()))
TN = (((0,), (0,)), ((), ()))


def _rnd(v):
    return v.astype(BF16).astype(F32)


def _ln(xf):
    m = jnp.mean(xf, axis=-1, keepdims=True)
    xc = xf - m
    v = jnp.mean(xc * xc, axis=-1, keepdims=True)
    return xc * lax.rsqrt(v + EPS)


def _ln_stats(xf):
    m = jnp.sum(xf, axis=-1, keepdims=True) * (1.0 / D)
    v = jnp.sum(xf * xf, axis=-1, keepdims=True) * (1.0 / D) - m * m
    return m, lax.rsqrt(jnp.maximum(v, 0.0) + EPS)


def _mo(v, m):
    return v if isinstance(v, int) else pl.multiple_of(v, m)


def _kernel(x_hbm, wqkv_hbm, wo_hbm, wr_ref, wg_hbm, wu_hbm, wd_hbm, out_hbm,
            xn_u, x1_u, h0_u, h1_u, qt_u, k_u, vt_u,
            wqkv_u, wqvt_u, wo_u, wg_u, wu_u, wd_u,
            p0, p1, p2, ot_u, bmax_ref, bidx_ref, zs, flag,
            sem_x, sem_w, sem_o):
    xn = xn_u.bitcast(BF16)
    x1_b = x1_u.bitcast(BF16)
    hbufs = (h0_u.bitcast(BF16), h1_u.bitcast(BF16))
    qt_b = qt_u.bitcast(BF16)
    k_b = k_u.bitcast(BF16)
    vt_b = vt_u.bitcast(BF16)
    wqkv = wqkv_u.bitcast(BF16)
    wqvt = wqvt_u.bitcast(BF16)
    wo = wo_u.bitcast(BF16)
    wg = wg_u.bitcast(BF16)
    wu = wu_u.bitcast(BF16)
    wd = wd_u.bitcast(BF16)
    ot_b = ot_u.bitcast(BF16)
    otbufs = (ot_b.at[0], ot_b.at[1])
    pbufs_u = (p0, p1, p2)
    pbufs_b = tuple(p.bitcast(BF16) for p in pbufs_u)

    def x_copy(j):
        return pltpu.make_async_copy(x_hbm.at[pl.ds(j * MB, MB), :],
                                     xn.at[pl.ds(j * MB, MB), :], sem_x.at[j])

    def wqkv_copy(c0, n, k):
        return pltpu.make_async_copy(wqkv_hbm.at[:, pl.ds(c0, n)],
                                     wqkv.at[:, pl.ds(c0, n)], sem_w.at[k])

    HD = D // 2
    wq_copies = [wqkv_copy(0, HD, 0), wqkv_copy(HD, HD, 1)]
    wv_copies = [wqkv_copy(2 * D, HD, 2), wqkv_copy(2 * D + HD, HD, 7)]
    wk_copy = wqkv_copy(D, D, 8)

    w_copies = [
        pltpu.make_async_copy(wo_hbm, wo, sem_w.at[3]),
        pltpu.make_async_copy(wg_hbm, wg, sem_w.at[4]),
        pltpu.make_async_copy(wu_hbm, wu, sem_w.at[5]),
        pltpu.make_async_copy(wd_hbm, wd, sem_w.at[6]),
    ]
    x_copy(0).start()
    wq_copies[0].start()
    wq_copies[1].start()
    wv_copies[0].start()
    wv_copies[1].start()
    x_copy(1).start()
    x_copy(2).start()
    wk_copy.start()
    for j in range(3, NMB):
        x_copy(j).start()

    for t in range(4):
        zs[t] = 0

    eye = (lax.broadcasted_iota(I32, (128, 128), 0)
           == lax.broadcasted_iota(I32, (128, 128), 1)).astype(F32).astype(BF16)

    def transpose_w(src_col0, dst_row0, tiles):
        for t in tiles:
            w_t = wqkv[:, src_col0 + 128 * t:src_col0 + 128 * (t + 1)]
            wqvt[dst_row0 + 128 * t:dst_row0 + 128 * (t + 1), :] = lax.dot_general(
                eye, w_t, NT, preferred_element_type=F32).astype(BF16)

    def ln1(row0, dst):
        src = xn.at[pl.ds(row0, MB), :]
        for c in range(MB // 64):
            xf = src[64 * c:64 * (c + 1), :].astype(F32)
            dst[64 * c:64 * (c + 1), :] = _ln(xf).astype(BF16)

    def proj_t(row0, n, base, hsrc):
        r = lax.dot_general(wqvt[row0:row0 + n, :], hsrc[...], NT, preferred_element_type=F32)
        if row0 < D:
            qt_b[row0:row0 + n, pl.ds(base, MB)] = (r * QSCALE).astype(BF16)
        else:
            vt_b[row0 - D:row0 - D + n, pl.ds(base, MB)] = r.astype(BF16)

    def proj_qv(base, hsrc):
        qv = lax.dot_general(wqvt[...], hsrc[...], NT, preferred_element_type=F32)
        qt_b[:, pl.ds(base, MB)] = (qv[0:D] * QSCALE).astype(BF16)
        vt_b[:, pl.ds(base, MB)] = qv[D:2 * D].astype(BF16)

    def proj_k(base, hsrc):
        k = jnp.dot(hsrc[...], wqkv[:, D:2 * D], preferred_element_type=F32)
        k_b[pl.ds(base, MB), :] = k.astype(BF16)

    def phase_a(layer):
        def body(t, carry):
            first = jnp.logical_and(layer == 0, t == 0)

            @pl.when(first)
            def _():
                x_copy(1).wait()
                x_copy(2).wait()
                wk_copy.wait()
                for c in w_copies:
                    c.start()

            @pl.when(jnp.logical_and(layer == 0, t >= 1))
            def _():
                x_copy(2 * t + 1).wait()

            @pl.when(jnp.logical_and(layer == 0, jnp.logical_and(t >= 1, t < NMB // 2 - 1)))
            def _():
                x_copy(2 * t + 2).wait()

            b0 = pl.multiple_of(2 * t * MB, MB)
            b1 = pl.multiple_of(b0 + MB, MB)
            b2 = pl.multiple_of(jnp.minimum(2 * t + 2, NMB - 1) * MB, MB)

            @pl.when(jnp.logical_not(first))
            def _():
                proj_qv(b0, hbufs[0])

            proj_k(b0, hbufs[0])
            ln1(b1, hbufs[1])
            proj_qv(b1, hbufs[1])
            proj_k(b1, hbufs[1])
            ln1(b2, hbufs[0])
            return carry

        lax.fori_loop(0, NMB // 2, body, 0)

    x_copy(0).wait()
    ln1(0, hbufs[0])
    for k in range(2):
        wq_copies[k].wait()
        transpose_w(k * HD, k * HD, range(4))
        proj_t(k * HD, HD, 0, hbufs[0])
    for k in range(2):
        wv_copies[k].wait()
        transpose_w(2 * D + k * HD, D + k * HD, range(4))
        proj_t(D + k * HD, HD, 0, hbufs[0])

    def attention(blocks):
        zst = zs[0]
        zld = zs[1]
        zl2 = zs[2]
        lane = lax.broadcasted_iota(I32, (QB, QB), 1)
        row = lax.broadcasted_iota(I32, (QB, QB), 0)
        newmask = row <= lane
        l2 = lax.broadcasted_iota(I32, (QB // 2, QB), 1)
        r2 = lax.broadcasted_iota(I32, (QB // 2, QB), 0) * 2
        pm_new = (jnp.where(r2 <= l2, U32(0xFFFF), U32(0))
                  | jnp.where(r2 + 1 <= l2, U32(0xFFFF0000), U32(0)))
        p_st = [p.at[zst] for p in pbufs_b]
        p_ld = [p.at[zld] for p in pbufs_u]
        p_l2 = [p.at[zl2] for p in pbufs_u]
        zero32 = jnp.zeros((32, QB), BF16)
        good = [None] * len(blocks)
        views = []
        for (i, nkb) in blocks:
            r0 = _mo(i * QB, QB)
            k0 = 128 * (nkb - 1)
            views.append((qt_b.at[:, pl.ds(r0, QB)],
                          k_b.at[pl.ds(r0 - k0, k0 + QB), :],
                          vt_b.at[:, pl.ds(r0 - k0, k0 + QB)]))

        def qk(n, g, slot):
            nkb = blocks[n][1]
            k0 = 128 * (nkb - 1)
            qw, kw, _ = views[n]
            cs = slice(128 * g, 128 * (g + 1))
            ws = []
            for j in range(4):
                h = 4 * g + j
                ws.append(jnp.concatenate(
                    [zero32] * j + [qw[32 * h:32 * (h + 1), :]] + [zero32] * (3 - j), axis=0))
            w = jnp.concatenate(ws, axis=1)
            parts = []
            if nkb == 3:
                for c in range(8):
                    parts.append(kw[16 * c:16 * c + 16, cs])
                    parts.append(kw[256 + 16 * c:256 + 16 * c + 16, cs])
            else:
                parts.append(kw[k0:k0 + 128, cs])
            if nkb >= 2:
                parts.append(kw[k0 - 128:k0, cs])
            kk = jnp.concatenate(parts, axis=0)
            st = jnp.dot(kk, w, preferred_element_type=F32)
            pref = p_st[slot]
            for j in range(4):
                s = st[:, 128 * j:128 * (j + 1)]
                ls = slice(128 * j, 128 * (j + 1))
                for c in range(8):
                    nm = newmask[16 * c:16 * c + 16]
                    if nkb == 3:
                        f = jnp.where(nm, s[32 * c + 16:32 * c + 32], s[32 * c:32 * c + 16])
                    else:
                        f = jnp.where(nm, s[16 * c:16 * c + 16], NEG)
                    pref[16 * c:16 * c + 16, ls] = jnp.exp2(f).astype(BF16)
                if nkb >= 2:
                    o = 256 if nkb == 3 else 128
                    for c in range(8):
                        pref[128 + 16 * c:128 + 16 * c + 16, ls] = jnp.exp2(
                            s[o + 16 * c:o + 16 * c + 16]).astype(BF16)

        def pv(n, g, j, slot):
            nkb = blocks[n][1]
            nrow = 128 if nkb == 1 else 256
            vw = views[n][2]
            h = 4 * g + j
            pref = p_ld[slot]
            ls = slice(128 * j, 128 * (j + 1))
            pf = pref[0:64, ls]
            if nkb == 3:
                pnew = pf & pm_new
                p = jnp.concatenate([pf ^ pnew, pref[64:128, ls], pnew], axis=0)
            elif nkb == 2:
                p = jnp.concatenate([pref[64:128, ls], pf], axis=0)
            else:
                p = pf
            vt = vw[32 * h:32 * (h + 1), :]
            ot = jnp.dot(vt, pltpu.bitcast(p, BF16), preferred_element_type=F32)
            pp = p_l2[slot][0:nrow // 2, ls]
            x = (pltpu.bitcast(pp & U32(0xFFFF0000), F32)
                 + pltpu.bitcast(pp << 16, F32)).reshape(nrow // 16, 8, 128)
            while x.shape[0] > 1:
                m = x.shape[0] // 2
                x = x[:m] + x[m:]
            l = jnp.sum(x[0], axis=0, keepdims=True)
            am = jnp.max(jnp.abs(ot).reshape(4, 8, 128), axis=0)
            ok = (l >= L_LO) & (l <= L_HI) & (am <= F_MAX)
            good[n] = ok if good[n] is None else (good[n] & ok)
            o = (ot * (1.0 / l)).astype(BF16)
            otbufs[n][32 * (h % 16):32 * (h % 16) + 32,
                      128 * (h // 16):128 * (h // 16) + 128] = o

        l64 = lax.broadcasted_iota(I32, (16, QB), 1)
        lo16 = l64 < 64
        lo8 = lax.broadcasted_iota(I32, (8, QB), 1) < 64
        lo1 = lax.broadcasted_iota(I32, (1, QB), 1) < 64
        t64 = lax.broadcasted_iota(I32, (64, QB), 0)
        s64 = lax.broadcasted_iota(I32, (64, QB), 1) & 63
        new64 = t64 <= s64
        r32 = lax.broadcasted_iota(I32, (32, QB), 0) * 2
        c32 = lax.broadcasted_iota(I32, (32, QB), 1)
        lo32 = c32 < 64
        pn64 = (jnp.where(r32 <= (c32 & 63), U32(0xFFFF), U32(0))
                | jnp.where(r32 + 1 <= (c32 & 63), U32(0xFFFF0000), U32(0)))
        po64 = ~pn64
        zu = U32(0)

        lsums = {}

        def qk2(n, g, slot):
            qw, kw, _ = views[n]
            cs = slice(128 * g, 128 * (g + 1))
            pref = p_st[slot]
            for a in range(2):
                he = 4 * g + 2 * a
                xe = pltpu.bitcast(qw[32 * he:32 * he + 32, :], U32)
                xo = pltpu.roll(pltpu.bitcast(qw[32 * he + 32:32 * he + 64, :], U32), 64, 1)
                for u in range(2):
                    me = lo16 if u == 0 else jnp.logical_not(lo16)
                    wt = pltpu.bitcast(jnp.concatenate(
                        [jnp.where(me, xe, zu), jnp.where(me, zu, xo)], axis=0), BF16)
                    w = jnp.concatenate([zero32] * (2 * a) + [wt] + [zero32] * (2 - 2 * a), axis=0)
                    parts = []
                    for c in range(4):
                        parts.append(kw[64 * u + 16 * c:64 * u + 16 * c + 16, cs])
                        parts.append(kw[64 * u + 256 + 16 * c:64 * u + 256 + 16 * c + 16, cs])
                    parts.append(kw[64 * u + 64:64 * u + 256, cs])
                    s = jnp.dot(jnp.concatenate(parts, axis=0), w, preferred_element_type=F32)
                    ls = slice(128 * (2 * a + u), 128 * (2 * a + u + 1))
                    acc = [None, None]

                    def put(row0, e, k):
                        pref[row0:row0 + 16, ls] = e.astype(BF16)
                        acc[k] = e if acc[k] is None else acc[k] + e

                    for c in range(4):
                        f = jnp.where(new64[16 * c:16 * c + 16], s[32 * c + 16:32 * c + 32],
                                      s[32 * c:32 * c + 16])
                        put(16 * c, jnp.exp2(f), c % 2)
                    for c in range(12):
                        put(64 + 16 * c, jnp.exp2(s[128 + 16 * c:128 + 16 * c + 16]), c % 2)
                    t = acc[0] + acc[1]
                    lsums[(slot, 2 * a + u)] = jnp.sum(t[0:8] + t[8:16], axis=0, keepdims=True)

        def colsum(pp):
            x = (pltpu.bitcast(pp & U32(0xFFFF0000), F32)
                 + pltpu.bitcast(pp << 16, F32)).reshape(pp.shape[0] // 8, 8, 128)
            while x.shape[0] > 1:
                m = x.shape[0] // 2
                x = x[:m] + x[m:]
            return jnp.sum(x[0], axis=0, keepdims=True)

        def pv2(n, g, a, slot):
            vw = views[n][2]
            pref = p_ld[slot]
            c0 = slice(128 * (2 * a), 128 * (2 * a + 1))
            c1 = slice(128 * (2 * a + 1), 128 * (2 * a + 2))
            f0 = pref[0:32, c0]
            f1 = pref[0:32, c1]
            n0 = f0 & pn64
            o0 = f0 ^ n0
            n1 = f1 & pn64
            o1 = f1 ^ n1
            m0 = [pref[32 + 32 * b:64 + 32 * b, c0] for b in range(3)]
            m1 = [pref[32 + 32 * b:64 + 32 * b, c1] for b in range(3)]
            l0 = lsums.pop((slot, 2 * a))
            l1 = lsums.pop((slot, 2 * a + 1))
            for e in range(2):
                h = 4 * g + 2 * a + e
                if e == 0:
                    tiles = [jnp.where(lo32, o0, zu), jnp.where(lo32, m0[0], o1),
                             jnp.where(lo32, m0[1], m1[0]), jnp.where(lo32, m0[2], m1[1]),
                             jnp.where(lo32, n0, m1[2]), jnp.where(lo32, zu, n1)]
                    l = jnp.where(lo1, l0, l1)
                else:
                    tiles = [jnp.where(lo32, zu, o0), jnp.where(lo32, o1, m0[0]),
                             jnp.where(lo32, m1[0], m0[1]), jnp.where(lo32, m1[1], m0[2]),
                             jnp.where(lo32, m1[2], n0), jnp.where(lo32, n1, zu)]
                    l = jnp.where(lo1, l1, l0)
                p = pltpu.bitcast(jnp.concatenate(tiles, axis=0), BF16)
                ot = jnp.dot(vw[32 * h:32 * (h + 1), :], p, preferred_element_type=F32)
                am = jnp.max(jnp.abs(ot).reshape(4, 8, 128), axis=0)
                ok = (l >= L_LO) & (l <= L_HI) & (am <= F_MAX)
                good[n] = ok if good[n] is None else (good[n] & ok)
                o = ot * (1.0 / l)
                if e == 1:
                    o = pltpu.roll(o, 64, 1)
                otbufs[n][32 * (h % 16):32 * (h % 16) + 32,
                          128 * (h // 16):128 * (h // 16) + 128] = o.astype(BF16)

        seq = [(n, g) for n in range(len(blocks)) for g in range(8)]
        for s in range(len(seq) + 2):
            if s < len(seq):
                n, g = seq[s]
                (qk2 if blocks[n][1] == 3 else qk)(n, g, s % 3)
            if s >= 2:
                n, g = seq[s - 2]
                if blocks[n][1] == 3:
                    for a in range(2):
                        pv2(n, g, a, (s - 2) % 3)
                else:
                    for j in range(4):
                        pv(n, g, j, (s - 2) % 3)
        for n in range(len(blocks)):
            flag[n] = jnp.min(jnp.where(good[n], 1, 0))

    def attention_safe(i, ow):
        r0 = _mo(i * QB, QB)
        start = pl.multiple_of(jnp.maximum(i - 2, 0) * QB, QB)
        qw = qt_b.at[:, pl.ds(r0, QB)]
        kw = k_b.at[pl.ds(start, 3 * QB), :]
        vw = vt_b.at[:, pl.ds(start, 3 * QB)]
        key = lax.broadcasted_iota(I32, (3 * QB, QB), 0) + start
        qry = lax.broadcasted_iota(I32, (3 * QB, QB), 1) + r0
        valid = (qry - key >= 0) & (qry - key < WIN)
        drow = lax.broadcasted_iota(I32, (128, QB), 0)

        def head(h, carry):
            g0 = pl.multiple_of((h // 4) * 128, 128)
            j0 = (h % 4) * 32
            q4 = qw[pl.ds(g0, 128), :].astype(F32)
            w = jnp.where((drow >= j0) & (drow < j0 + 32), q4, 0.0).astype(BF16)
            s = jnp.dot(kw[:, pl.ds(g0, 128)], w, preferred_element_type=F32)
            s = jnp.where(valid, s, NEG)
            m = jnp.max(s, axis=0, keepdims=True)
            p = jnp.exp2(s - m).astype(BF16)
            l = jnp.sum(p.astype(F32), axis=0, keepdims=True)
            vt = vw[pl.ds(pl.multiple_of(h * 32, 32), 32), :]
            o = jnp.dot(vt, p, preferred_element_type=F32) * (1.0 / l)
            ow[pl.ds(pl.multiple_of((h % 16) * 32, 32), 32),
               pl.ds(pl.multiple_of((h // 16) * 128, 128), 128)] = o.astype(BF16)
            return carry

        lax.fori_loop(0, NH, head, 0)

    def out_proj(n, xsrc, x1dst, z=0):
        ow = ot_b.at[n + z]
        o = jnp.concatenate([ow[:, 0:128], ow[:, 128:256]], axis=0)
        y = lax.dot_general(o, wo[...], TN, preferred_element_type=F32)
        x1dst[...] = (xsrc[...].astype(F32) + y).astype(BF16)

    def ln2(b, x1src, x2dst, CH=16, NCHAIN=8, z_in=0):
        rb = _mo(b * QB, QB)
        wr = wr_ref[...].astype(F32).reshape(1, D)
        wsum = jnp.sum(wr, axis=-1, keepdims=True)
        bm = None
        bi = None
        sub = lax.broadcasted_iota(I32, (8, 1), 0)
        toks = []
        for c in range(QB // CH):
            z = toks[c - NCHAIN] if c >= NCHAIN else z_in
            if isinstance(z, int):
                x1 = x1src[CH * c:CH * (c + 1), :].astype(F32)
            else:
                x1 = x1src[pl.ds(pl.multiple_of(CH * c + z * 16, 16), CH), :].astype(F32)
            m, rs = _ln_stats(x1)
            x2dst[CH * c:CH * (c + 1), :] = (x1 * (1.0 + rs) - m * rs).astype(BF16)
            r = _rnd(rs * (jnp.sum(x1 * wr, axis=-1, keepdims=True) - m * wsum))
            ru = lax.bitcast_convert_type(r, I32)
            toks.append(jnp.max(lax.shift_right_logical(lax.shift_right_logical(ru, 16), 16)))
            for t in range(CH // 8):
                rt = r[8 * t:8 * t + 8]
                it = sub + (rb + CH * c + 8 * t)
                if bm is None:
                    bm, bi = rt, it
                else:
                    better = rt > bm
                    bm = jnp.where(better, rt, bm)
                    bi = jnp.where(better, it, bi)
        bmax_ref[b] = jnp.broadcast_to(bm, (8, 128))
        bidx_ref[b] = jnp.broadcast_to(bi, (8, 128))
        tok = toks[-1]
        for k in range(2, min(NCHAIN, len(toks)) + 1):
            tok = tok + toks[-k]
        return tok

    def checks(i0):
        def one(n, carry):
            @pl.when(flag[n] == 0)
            def _():
                rb = pl.multiple_of((i0 + n) * QB, QB)
                attention_safe(i0 + n, ot_b.at[n])
                out_proj(n, xn.at[pl.ds(rb, QB), :], x1_b.at[pl.ds(rb, QB), :])
            return carry

        @pl.when(flag[0] + flag[1] < 2)
        def _():
            lax.fori_loop(0, 2, one, 0)

    def out_copy(b):
        return pltpu.make_async_copy(xn.at[pl.ds(b * QB, QB), :],
                                     out_hbm.at[pl.ds(b * QB, QB), :], sem_o.at[0])

    def phase_b(layer):
        attention([(0, 1), (1, 2)])
        out_proj(0, xn.at[0:QB, :], x1_b.at[0:QB, :])
        out_proj(1, xn.at[QB:2 * QB, :], x1_b.at[QB:2 * QB, :])

        def body(t, carry):
            i0 = 2 * t
            checks(i0 - 2)

            @pl.when(jnp.logical_and(layer == 1, t >= 2))
            def _():
                out_copy(i0 - 4).start()
                out_copy(i0 - 3).start()

            @pl.when(t < NQB // 2)
            def _():
                r2 = pl.multiple_of((i0 - 2) * QB, QB)
                xv = xn.at[pl.ds(r2, 4 * QB), :]
                x1v = x1_b.at[pl.ds(r2, 4 * QB), :]
                ln2(i0 - 2, x1v.at[0:QB, :], xv.at[0:QB, :])
                ln2(i0 - 1, x1v.at[QB:2 * QB, :], xv.at[QB:2 * QB, :])
                attention([(i0, 3), (i0 + 1, 3)])
                out_proj(0, xv.at[2 * QB:3 * QB, :], x1v.at[2 * QB:3 * QB, :])
                out_proj(1, xv.at[3 * QB:4 * QB, :], x1v.at[3 * QB:4 * QB, :])
            return carry

        lax.fori_loop(1, NQB // 2 + 1, body, 0)
        for b in (NQB - 2, NQB - 1):
            ln2(b, x1_b.at[b * QB:(b + 1) * QB, :], xn.at[b * QB:(b + 1) * QB, :], NCHAIN=8)

        @pl.when(layer == 1)
        def _():
            out_copy(NQB - 2).start()
            out_copy(NQB - 1).start()

    def moe(layer):
        rm = bmax_ref[:, :, 0:1]
        ri = bidx_ref[:, :, 0:1]
        gm = jnp.max(jnp.max(rm, axis=0), axis=0, keepdims=True)
        idx = jnp.min(jnp.where(rm == gm, ri, BIG))
        b16 = pl.multiple_of((idx // 16) * 16, 16)
        x1c = x1_b[pl.ds(b16, 16), :].astype(F32)
        h2c = _rnd(_ln(x1c))
        hb = h2c.astype(BF16)
        g = _rnd(jnp.dot(hb, wg[...], preferred_element_type=F32))
        u = _rnd(jnp.dot(hb, wu[...], preferred_element_type=F32))
        g = _rnd(g * _rnd(jax.nn.sigmoid(g)))
        act = (g * u).astype(BF16)
        y = _rnd(jnp.dot(act, wd[...], preferred_element_type=F32))
        y = _rnd(y * _rnd(jax.nn.sigmoid(gm)))
        x2n = x1c + _rnd(h2c + y)

        @pl.when(layer == 1)
        def _():
            for b in range(NQB):
                out_copy(b).wait()

        cur = xn[pl.ds(b16, 16), :].astype(F32)
        sel = lax.broadcasted_iota(I32, (16, D), 0) == (idx - b16)
        xn[pl.ds(b16, 16), :] = jnp.where(sel, x2n, cur).astype(BF16)

        @pl.when(layer == 1)
        def _():
            cp = pltpu.make_async_copy(xn.at[pl.ds(b16, 16), :],
                                       out_hbm.at[pl.ds(b16, 16), :], sem_o.at[1])
            cp.start()
            cp.wait()

    def layer_body(layer, carry):
        phase_a(layer)

        @pl.when(layer == 0)
        def _():
            w_copies[0].wait()

        phase_b(layer)

        @pl.when(layer == 0)
        def _():
            for c in w_copies[1:]:
                c.wait()

        moe(layer)

        @pl.when(layer == 0)
        def _():
            ln1(0, hbufs[0])

        return carry

    lax.fori_loop(0, 2, layer_body, 0)


@jax.jit
def pallas_interleave_layers__sliding_block__moe_arch_mod__prompt_kernel(
    A_x: jax.Array,
    A_wqkv: jax.Array,
    A_wo: jax.Array,
    B_x: jax.Array,
    B_w_r: jax.Array,
    B_w_gate: jax.Array,
    B_w_up: jax.Array,
    B_w_down: jax.Array,
):
    del B_x
    hbm = pl.BlockSpec(memory_space=pl.ANY)
    scratch = [
        pltpu.VMEM((S // 2, D), U32),
        pltpu.VMEM((S // 2, D), U32),
        pltpu.VMEM((MB // 2, D), U32),
        pltpu.VMEM((MB // 2, D), U32),
        pltpu.VMEM((D // 2, S), U32),
        pltpu.VMEM((S // 2, D), U32),
        pltpu.VMEM((D // 2, S), U32),
        pltpu.VMEM((D // 2, 3 * D), U32),
        pltpu.VMEM((D, D), U32),
        pltpu.VMEM((D // 2, D), U32),
        pltpu.VMEM((D // 2, FF), U32),
        pltpu.VMEM((D // 2, FF), U32),
        pltpu.VMEM((FF // 2, D), U32),
        pltpu.VMEM((1, 128, 512), U32),
        pltpu.VMEM((1, 128, 512), U32),
        pltpu.VMEM((1, 128, 512), U32),
        pltpu.VMEM((2, 256, 256), U32),
        pltpu.VMEM((NQB, 8, 128), F32),
        pltpu.VMEM((NQB, 8, 128), I32),
        pltpu.SMEM((4,), I32),
        pltpu.SMEM((2,), I32),
        pltpu.SemaphoreType.DMA((NMB,)),
        pltpu.SemaphoreType.DMA((9,)),
        pltpu.SemaphoreType.DMA((2,)),
    ]
    out = pl.pallas_call(
        _kernel,
        out_shape=jax.ShapeDtypeStruct((S, D), BF16),
        in_specs=[hbm, hbm, hbm, pl.BlockSpec(memory_space=pltpu.VMEM), hbm, hbm, hbm],
        out_specs=hbm,
        scratch_shapes=scratch,
        compiler_params=pltpu.CompilerParams(vmem_limit_bytes=110 * 1024 * 1024),
        name="swa_moe_fused",
    )(A_x.reshape(S, D), A_wqkv, A_wo, B_w_r, B_w_gate, B_w_up, B_w_down)
    return out.reshape(1, S, D)
```

```python
import math

import jax
import jax.numpy as jnp
from jax import lax
import jax.experimental.pallas as pl
import jax.experimental.pallas.tpu as pltpu

S = 2048
D = 1024
NH = 32
DH = 32
WIN = 256
FF = 3584
QB = 128
NQB = S // QB
MB = 256
NMB = S // MB
EPS = 1e-5
QSCALE = (DH ** -0.5) * math.log2(math.e)
NEG = -1e30
BIG = 2 ** 30
L_LO = 2.0 ** -64
L_HI = 2.0 ** 64
V_HI = 2.0 ** 60

F32 = jnp.float32
BF16 = jnp.bfloat16
U32 = jnp.uint32
I32 = jnp.int32

NT = (((1,), (1,)), ((), ()))
TN = (((0,), (0,)), ((), ()))


def _rnd(v):
    return v.astype(BF16).astype(F32)


def _ln(xf):
    m = jnp.mean(xf, axis=-1, keepdims=True)
    xc = xf - m
    v = jnp.mean(xc * xc, axis=-1, keepdims=True)
    return xc * lax.rsqrt(v + EPS)


def _ln_stats(xf):
    m = jnp.sum(xf, axis=-1, keepdims=True) * (1.0 / D)
    v = jnp.sum(xf * xf, axis=-1, keepdims=True) * (1.0 / D) - m * m
    return m, lax.rsqrt(jnp.maximum(v, 0.0) + EPS)


def _recip(l):
    r = pl.reciprocal(l, approx=True)
    return r * (2.0 - l * r)


def _mo(v, m):
    return v if isinstance(v, int) else pl.multiple_of(v, m)


def _kernel(x_hbm, wqkv_hbm, wo_hbm, wr_ref, wg_hbm, wu_hbm, wd_hbm, out_hbm,
            xn_u, x1_u, h0_u, h1_u, qt_u, k_u, vt_u,
            wqkv_u, wqvt_u, wo_u, wg_u, wu_u, wd_u,
            p0, p1, p2, ot_u, vmax_ref, bmax_ref, bidx_ref, zs, flag,
            sem_x, sem_w, sem_o):
    xn = xn_u.bitcast(BF16)
    x1_b = x1_u.bitcast(BF16)
    hbufs = (h0_u.bitcast(BF16), h1_u.bitcast(BF16))
    qt_b = qt_u.bitcast(BF16)
    k_b = k_u.bitcast(BF16)
    vt_b = vt_u.bitcast(BF16)
    wqkv = wqkv_u.bitcast(BF16)
    wqvt = wqvt_u.bitcast(BF16)
    wo = wo_u.bitcast(BF16)
    wg = wg_u.bitcast(BF16)
    wu = wu_u.bitcast(BF16)
    wd = wd_u.bitcast(BF16)
    ot_b = ot_u.bitcast(BF16)
    otbufs = (ot_b.at[0], ot_b.at[1])
    pbufs_u = (p0, p1, p2)
    pbufs_b = tuple(p.bitcast(BF16) for p in pbufs_u)

    def x_copy(j):
        return pltpu.make_async_copy(x_hbm.at[pl.ds(j * MB, MB), :],
                                     xn.at[pl.ds(j * MB, MB), :], sem_x.at[j])

    def wqkv_copy(c0, n, k):
        return pltpu.make_async_copy(wqkv_hbm.at[:, pl.ds(c0, n)],
                                     wqkv.at[:, pl.ds(c0, n)], sem_w.at[k])

    HD = D // 2
    wq_copies = [wqkv_copy(0, HD, 0), wqkv_copy(HD, HD, 1)]
    wv_copies = [wqkv_copy(2 * D, HD, 2), wqkv_copy(2 * D + HD, HD, 7)]
    wk_copy = wqkv_copy(D, D, 8)

    w_copies = [
        pltpu.make_async_copy(wo_hbm, wo, sem_w.at[3]),
        pltpu.make_async_copy(wg_hbm, wg, sem_w.at[4]),
        pltpu.make_async_copy(wu_hbm, wu, sem_w.at[5]),
        pltpu.make_async_copy(wd_hbm, wd, sem_w.at[6]),
    ]
    x_copy(0).start()
    wq_copies[0].start()
    wq_copies[1].start()
    wv_copies[0].start()
    wv_copies[1].start()
    x_copy(1).start()
    x_copy(2).start()
    wk_copy.start()
    for j in range(3, NMB):
        x_copy(j).start()

    for t in range(4):
        zs[t] = 0
    vmax_ref[...] = jnp.zeros((8, 128), F32)

    eye = (lax.broadcasted_iota(I32, (128, 128), 0)
           == lax.broadcasted_iota(I32, (128, 128), 1)).astype(F32).astype(BF16)

    def transpose_w(src_col0, dst_row0, tiles):
        for t in tiles:
            w_t = wqkv[:, src_col0 + 128 * t:src_col0 + 128 * (t + 1)]
            wqvt[dst_row0 + 128 * t:dst_row0 + 128 * (t + 1), :] = lax.dot_general(
                eye, w_t, NT, preferred_element_type=F32).astype(BF16)

    def ln1(row0, dst):
        src = xn.at[pl.ds(row0, MB), :]
        for c in range(MB // 64):
            xf = src[64 * c:64 * (c + 1), :].astype(F32)
            dst[64 * c:64 * (c + 1), :] = _ln(xf).astype(BF16)

    def track_v(v):
        a = jnp.max(jnp.abs(v).reshape(v.shape[0] // 8, 8, v.shape[1]), axis=0)
        a = jnp.maximum(a[:, 0:128], a[:, 128:256])
        a = jnp.broadcast_to(jnp.max(a, axis=0, keepdims=True), (8, 128))
        vmax_ref[...] = jnp.maximum(vmax_ref[...], a)

    def proj_t(row0, n, base, hsrc):
        r = lax.dot_general(wqvt[row0:row0 + n, :], hsrc[...], NT, preferred_element_type=F32)
        if row0 < D:
            qt_b[row0:row0 + n, pl.ds(base, MB)] = (r * QSCALE).astype(BF16)
        else:
            vt_b[row0 - D:row0 - D + n, pl.ds(base, MB)] = r.astype(BF16)
            track_v(r)

    def proj_qv(base, hsrc):
        qv = lax.dot_general(wqvt[...], hsrc[...], NT, preferred_element_type=F32)
        qt_b[:, pl.ds(base, MB)] = (qv[0:D] * QSCALE).astype(BF16)
        vt_b[:, pl.ds(base, MB)] = qv[D:2 * D].astype(BF16)
        track_v(qv[D:2 * D])

    def proj_k(base, hsrc):
        k = jnp.dot(hsrc[...], wqkv[:, D:2 * D], preferred_element_type=F32)
        k_b[pl.ds(base, MB), :] = k.astype(BF16)

    def phase_a(layer):
        def body(t, carry):
            first = jnp.logical_and(layer == 0, t == 0)

            @pl.when(first)
            def _():
                x_copy(1).wait()
                x_copy(2).wait()
                wk_copy.wait()
                for c in w_copies:
                    c.start()

            @pl.when(jnp.logical_and(layer == 0, t >= 1))
            def _():
                x_copy(2 * t + 1).wait()

            @pl.when(jnp.logical_and(layer == 0, jnp.logical_and(t >= 1, t < NMB // 2 - 1)))
            def _():
                x_copy(2 * t + 2).wait()

            b0 = pl.multiple_of(2 * t * MB, MB)
            b1 = pl.multiple_of(b0 + MB, MB)
            b2 = pl.multiple_of(jnp.minimum(2 * t + 2, NMB - 1) * MB, MB)

            @pl.when(jnp.logical_not(first))
            def _():
                proj_qv(b0, hbufs[0])

            proj_k(b0, hbufs[0])
            ln1(b1, hbufs[1])
            proj_qv(b1, hbufs[1])
            proj_k(b1, hbufs[1])
            ln1(b2, hbufs[0])
            return carry

        lax.fori_loop(0, NMB // 2, body, 0)

    x_copy(0).wait()
    ln1(0, hbufs[0])
    for k in range(2):
        wq_copies[k].wait()
        transpose_w(k * HD, k * HD, range(4))
        proj_t(k * HD, HD, 0, hbufs[0])
    for k in range(2):
        wv_copies[k].wait()
        transpose_w(2 * D + k * HD, D + k * HD, range(4))
        proj_t(D + k * HD, HD, 0, hbufs[0])

    def attention(blocks):
        zst = zs[0]
        zld = zs[1]
        lane = lax.broadcasted_iota(I32, (QB, QB), 1)
        row = lax.broadcasted_iota(I32, (QB, QB), 0)
        newmask = row <= lane
        p_st = [p.at[zst] for p in pbufs_b]
        p_ld = [p.at[zld] for p in pbufs_u]
        zero32 = jnp.zeros((32, QB), BF16)
        good = [None] * len(blocks)
        lsums = {}
        views = []
        for (i, nkb) in blocks:
            r0 = _mo(i * QB, QB)
            k0 = 128 * (nkb - 1)
            views.append((qt_b.at[:, pl.ds(r0, QB)],
                          k_b.at[pl.ds(r0 - k0, k0 + QB), :],
                          vt_b.at[:, pl.ds(r0 - k0, k0 + QB)]))

        def qk(n, g, slot):
            nkb = blocks[n][1]
            k0 = 128 * (nkb - 1)
            qw, kw, _ = views[n]
            cs = slice(128 * g, 128 * (g + 1))
            ws = []
            for j in range(4):
                h = 4 * g + j
                ws.append(jnp.concatenate(
                    [zero32] * j + [qw[32 * h:32 * (h + 1), :]] + [zero32] * (3 - j), axis=0))
            w = jnp.concatenate(ws, axis=1)
            parts = [kw[k0:k0 + 128, cs]]
            if nkb == 2:
                parts.append(kw[0:128, cs])
            kk = jnp.concatenate(parts, axis=0)
            st = jnp.dot(kk, w, preferred_element_type=F32)
            pref = p_st[slot]
            for j in range(4):
                s = st[:, 128 * j:128 * (j + 1)]
                ls = slice(128 * j, 128 * (j + 1))
                acc = [None, None]

                def put(row0, e, k):
                    pref[row0:row0 + 16, ls] = e.astype(BF16)
                    acc[k] = e if acc[k] is None else acc[k] + e

                for c in range(8):
                    f = jnp.where(newmask[16 * c:16 * c + 16], s[16 * c:16 * c + 16], NEG)
                    put(16 * c, jnp.exp2(f), c % 2)
                if nkb == 2:
                    for c in range(8):
                        put(128 + 16 * c, jnp.exp2(s[128 + 16 * c:128 + 16 * c + 16]), c % 2)
                t = acc[0] + acc[1]
                lsums[(slot, j)] = jnp.sum(t[0:8] + t[8:16], axis=0, keepdims=True)

        def pv(n, g, j, slot):
            nkb = blocks[n][1]
            vw = views[n][2]
            h = 4 * g + j
            pref = p_ld[slot]
            ls = slice(128 * j, 128 * (j + 1))
            p = pref[0:64, ls]
            if nkb == 2:
                p = jnp.concatenate([pref[64:128, ls], p], axis=0)
            vt = vw[32 * h:32 * (h + 1), :]
            ot = jnp.dot(vt, pltpu.bitcast(p, BF16), preferred_element_type=F32)
            l = lsums.pop((slot, j))
            ok = (l >= L_LO) & (l <= L_HI)
            good[n] = ok if good[n] is None else (good[n] & ok)
            o = (ot * _recip(l)).astype(BF16)
            otbufs[n][32 * (h % 16):32 * (h % 16) + 32,
                      128 * (h // 16):128 * (h // 16) + 128] = o

        l64 = lax.broadcasted_iota(I32, (16, QB), 1)
        lo16 = l64 < 64
        lo8 = lax.broadcasted_iota(I32, (8, QB), 1) < 64
        lo1 = lax.broadcasted_iota(I32, (1, QB), 1) < 64
        t64 = lax.broadcasted_iota(I32, (64, QB), 0)
        s64 = lax.broadcasted_iota(I32, (64, QB), 1) & 63
        new64 = t64 <= s64
        r32 = lax.broadcasted_iota(I32, (32, QB), 0) * 2
        c32 = lax.broadcasted_iota(I32, (32, QB), 1)
        lo32 = c32 < 64
        pn64 = (jnp.where(r32 <= (c32 & 63), U32(0xFFFF), U32(0))
                | jnp.where(r32 + 1 <= (c32 & 63), U32(0xFFFF0000), U32(0)))
        po64 = ~pn64
        zu = U32(0)

        def qk2(n, g, slot):
            qw, kw, _ = views[n]
            cs = slice(128 * g, 128 * (g + 1))
            pref = p_st[slot]
            for a in range(2):
                he = 4 * g + 2 * a
                xe = pltpu.bitcast(qw[32 * he:32 * he + 32, :], U32)
                xo = pltpu.roll(pltpu.bitcast(qw[32 * he + 32:32 * he + 64, :], U32), 64, 1)
                for u in range(2):
                    me = lo16 if u == 0 else jnp.logical_not(lo16)
                    wt = pltpu.bitcast(jnp.concatenate(
                        [jnp.where(me, xe, zu), jnp.where(me, zu, xo)], axis=0), BF16)
                    w = jnp.concatenate([zero32] * (2 * a) + [wt] + [zero32] * (2 - 2 * a), axis=0)
                    parts = []
                    for c in range(4):
                        parts.append(kw[64 * u + 16 * c:64 * u + 16 * c + 16, cs])
                        parts.append(kw[64 * u + 256 + 16 * c:64 * u + 256 + 16 * c + 16, cs])
                    parts.append(kw[64 * u + 64:64 * u + 256, cs])
                    s = jnp.dot(jnp.concatenate(parts, axis=0), w, preferred_element_type=F32)
                    ls = slice(128 * (2 * a + u), 128 * (2 * a + u + 1))
                    acc = [None, None]

                    def put(row0, e, k):
                        pref[row0:row0 + 16, ls] = e.astype(BF16)
                        acc[k] = e if acc[k] is None else acc[k] + e

                    for c in range(4):
                        f = jnp.where(new64[16 * c:16 * c + 16], s[32 * c + 16:32 * c + 32],
                                      s[32 * c:32 * c + 16])
                        put(16 * c, jnp.exp2(f), c % 2)
                    for c in range(12):
                        put(64 + 16 * c, jnp.exp2(s[128 + 16 * c:128 + 16 * c + 16]), c % 2)
                    t = acc[0] + acc[1]
                    lsums[(slot, 2 * a + u)] = jnp.sum(t[0:8] + t[8:16], axis=0, keepdims=True)

        def pv2(n, g, a, slot):
            vw = views[n][2]
            pref = p_ld[slot]
            c0 = slice(128 * (2 * a), 128 * (2 * a + 1))
            c1 = slice(128 * (2 * a + 1), 128 * (2 * a + 2))
            f0 = pref[0:32, c0]
            f1 = pref[0:32, c1]
            n0 = f0 & pn64
            o0 = f0 ^ n0
            n1 = f1 & pn64
            o1 = f1 ^ n1
            m0 = [pref[32 + 32 * b:64 + 32 * b, c0] for b in range(3)]
            m1 = [pref[32 + 32 * b:64 + 32 * b, c1] for b in range(3)]
            l0 = lsums.pop((slot, 2 * a))
            l1 = lsums.pop((slot, 2 * a + 1))
            for e in range(2):
                h = 4 * g + 2 * a + e
                if e == 0:
                    tiles = [jnp.where(lo32, o0, zu), jnp.where(lo32, m0[0], o1),
                             jnp.where(lo32, m0[1], m1[0]), jnp.where(lo32, m0[2], m1[1]),
                             jnp.where(lo32, n0, m1[2]), jnp.where(lo32, zu, n1)]
                    l = jnp.where(lo1, l0, l1)
                else:
                    tiles = [jnp.where(lo32, zu, o0), jnp.where(lo32, o1, m0[0]),
                             jnp.where(lo32, m1[0], m0[1]), jnp.where(lo32, m1[1], m0[2]),
                             jnp.where(lo32, m1[2], n0), jnp.where(lo32, n1, zu)]
                    l = jnp.where(lo1, l1, l0)
                p = pltpu.bitcast(jnp.concatenate(tiles, axis=0), BF16)
                ot = jnp.dot(vw[32 * h:32 * (h + 1), :], p, preferred_element_type=F32)
                ok = (l >= L_LO) & (l <= L_HI)
                good[n] = ok if good[n] is None else (good[n] & ok)
                o = ot * _recip(l)
                if e == 1:
                    o = pltpu.roll(o, 64, 1)
                otbufs[n][32 * (h % 16):32 * (h % 16) + 32,
                          128 * (h // 16):128 * (h // 16) + 128] = o.astype(BF16)

        seq = [(n, g) for n in range(len(blocks)) for g in range(8)]
        for s in range(len(seq) + 2):
            if s < len(seq):
                n, g = seq[s]
                (qk2 if blocks[n][1] == 3 else qk)(n, g, s % 3)
            if s >= 2:
                n, g = seq[s - 2]
                if blocks[n][1] == 3:
                    for a in range(2):
                        pv2(n, g, a, (s - 2) % 3)
                else:
                    for j in range(4):
                        pv(n, g, j, (s - 2) % 3)
        v_ok = vmax_ref[0:1, :] <= V_HI
        for n in range(len(blocks)):
            flag[n] = jnp.min(jnp.where(good[n] & v_ok, 1, 0))

    def attention_safe(i, ow):
        r0 = _mo(i * QB, QB)
        start = pl.multiple_of(jnp.maximum(i - 2, 0) * QB, QB)
        qw = qt_b.at[:, pl.ds(r0, QB)]
        kw = k_b.at[pl.ds(start, 3 * QB), :]
        vw = vt_b.at[:, pl.ds(start, 3 * QB)]
        key = lax.broadcasted_iota(I32, (3 * QB, QB), 0) + start
        qry = lax.broadcasted_iota(I32, (3 * QB, QB), 1) + r0
        valid = (qry - key >= 0) & (qry - key < WIN)
        drow = lax.broadcasted_iota(I32, (128, QB), 0)

        def head(h, carry):
            g0 = pl.multiple_of((h // 4) * 128, 128)
            j0 = (h % 4) * 32
            q4 = qw[pl.ds(g0, 128), :].astype(F32)
            w = jnp.where((drow >= j0) & (drow < j0 + 32), q4, 0.0).astype(BF16)
            s = jnp.dot(kw[:, pl.ds(g0, 128)], w, preferred_element_type=F32)
            s = jnp.where(valid, s, NEG)
            m = jnp.max(s, axis=0, keepdims=True)
            p = jnp.exp2(s - m).astype(BF16)
            l = jnp.sum(p.astype(F32), axis=0, keepdims=True)
            vt = vw[pl.ds(pl.multiple_of(h * 32, 32), 32), :]
            o = jnp.dot(vt, p, preferred_element_type=F32) * (1.0 / l)
            ow[pl.ds(pl.multiple_of((h % 16) * 32, 32), 32),
               pl.ds(pl.multiple_of((h // 16) * 128, 128), 128)] = o.astype(BF16)
            return carry

        lax.fori_loop(0, NH, head, 0)

    def out_proj(n, xsrc, x1dst, z=0):
        ow = ot_b.at[n + z]
        o = jnp.concatenate([ow[:, 0:128], ow[:, 128:256]], axis=0)
        y = lax.dot_general(o, wo[...], TN, preferred_element_type=F32)
        x1dst[...] = (xsrc[...].astype(F32) + y).astype(BF16)

    def ln2(b, x1src, x2dst, CH=16, NCHAIN=8, z_in=0):
        rb = _mo(b * QB, QB)
        wr = wr_ref[...].astype(F32).reshape(1, D)
        wsum = jnp.sum(wr, axis=-1, keepdims=True)
        bm = None
        bi = None
        sub = lax.broadcasted_iota(I32, (8, 1), 0)
        toks = []
        for c in range(QB // CH):
            z = toks[c - NCHAIN] if c >= NCHAIN else z_in
            if isinstance(z, int):
                x1 = x1src[CH * c:CH * (c + 1), :].astype(F32)
            else:
                x1 = x1src[pl.ds(pl.multiple_of(CH * c + z * 16, 16), CH), :].astype(F32)
            m, rs = _ln_stats(x1)
            x2dst[CH * c:CH * (c + 1), :] = (x1 * (1.0 + rs) - m * rs).astype(BF16)
            r = _rnd(rs * (jnp.sum(x1 * wr, axis=-1, keepdims=True) - m * wsum))
            ru = lax.bitcast_convert_type(r, I32)
            toks.append(jnp.max(lax.shift_right_logical(lax.shift_right_logical(ru, 16), 16)))
            for t in range(CH // 8):
                rt = r[8 * t:8 * t + 8]
                it = sub + (rb + CH * c + 8 * t)
                if bm is None:
                    bm, bi = rt, it
                else:
                    better = rt > bm
                    bm = jnp.where(better, rt, bm)
                    bi = jnp.where(better, it, bi)
        bmax_ref[b] = jnp.broadcast_to(bm, (8, 128))
        bidx_ref[b] = jnp.broadcast_to(bi, (8, 128))
        tok = toks[-1]
        for k in range(2, min(NCHAIN, len(toks)) + 1):
            tok = tok + toks[-k]
        return tok

    def checks(i0):
        def one(n, carry):
            @pl.when(flag[n] == 0)
            def _():
                rb = pl.multiple_of((i0 + n) * QB, QB)
                attention_safe(i0 + n, ot_b.at[n])
                out_proj(n, xn.at[pl.ds(rb, QB), :], x1_b.at[pl.ds(rb, QB), :])
            return carry

        @pl.when(flag[0] + flag[1] < 2)
        def _():
            lax.fori_loop(0, 2, one, 0)

    def out_copy(b):
        return pltpu.make_async_copy(xn.at[pl.ds(b * QB, QB), :],
                                     out_hbm.at[pl.ds(b * QB, QB), :], sem_o.at[0])

    def phase_b(layer):
        attention([(0, 1), (1, 2)])
        out_proj(0, xn.at[0:QB, :], x1_b.at[0:QB, :])
        out_proj(1, xn.at[QB:2 * QB, :], x1_b.at[QB:2 * QB, :])

        def body(t, carry):
            i0 = 2 * t
            checks(i0 - 2)

            @pl.when(jnp.logical_and(layer == 1, t >= 2))
            def _():
                out_copy(i0 - 4).start()
                out_copy(i0 - 3).start()

            @pl.when(t < NQB // 2)
            def _():
                r2 = pl.multiple_of((i0 - 2) * QB, QB)
                xv = xn.at[pl.ds(r2, 4 * QB), :]
                x1v = x1_b.at[pl.ds(r2, 4 * QB), :]
                ln2(i0 - 2, x1v.at[0:QB, :], xv.at[0:QB, :])
                ln2(i0 - 1, x1v.at[QB:2 * QB, :], xv.at[QB:2 * QB, :])
                attention([(i0, 3), (i0 + 1, 3)])
                out_proj(0, xv.at[2 * QB:3 * QB, :], x1v.at[2 * QB:3 * QB, :])
                out_proj(1, xv.at[3 * QB:4 * QB, :], x1v.at[3 * QB:4 * QB, :])
            return carry

        lax.fori_loop(1, NQB // 2 + 1, body, 0)
        for b in (NQB - 2, NQB - 1):
            ln2(b, x1_b.at[b * QB:(b + 1) * QB, :], xn.at[b * QB:(b + 1) * QB, :], NCHAIN=8)

        @pl.when(layer == 1)
        def _():
            out_copy(NQB - 2).start()
            out_copy(NQB - 1).start()

    def moe(layer):
        rm = bmax_ref[:, :, 0:1]
        ri = bidx_ref[:, :, 0:1]
        gm = jnp.max(jnp.max(rm, axis=0), axis=0, keepdims=True)
        idx = jnp.min(jnp.where(rm == gm, ri, BIG))
        b16 = pl.multiple_of((idx // 16) * 16, 16)
        x1c = x1_b[pl.ds(b16, 16), :].astype(F32)
        h2c = _rnd(_ln(x1c))
        hb = h2c.astype(BF16)
        g = _rnd(jnp.dot(hb, wg[...], preferred_element_type=F32))
        u = _rnd(jnp.dot(hb, wu[...], preferred_element_type=F32))
        g = _rnd(g * _rnd(jax.nn.sigmoid(g)))
        act = (g * u).astype(BF16)
        y = _rnd(jnp.dot(act, wd[...], preferred_element_type=F32))
        y = _rnd(y * _rnd(jax.nn.sigmoid(gm)))
        x2n = x1c + _rnd(h2c + y)

        @pl.when(layer == 1)
        def _():
            for b in range(NQB):
                out_copy(b).wait()

        cur = xn[pl.ds(b16, 16), :].astype(F32)
        sel = lax.broadcasted_iota(I32, (16, D), 0) == (idx - b16)
        xn[pl.ds(b16, 16), :] = jnp.where(sel, x2n, cur).astype(BF16)

        @pl.when(layer == 1)
        def _():
            cp = pltpu.make_async_copy(xn.at[pl.ds(b16, 16), :],
                                       out_hbm.at[pl.ds(b16, 16), :], sem_o.at[1])
            cp.start()
            cp.wait()

    def layer_body(layer, carry):
        phase_a(layer)

        @pl.when(layer == 0)
        def _():
            w_copies[0].wait()

        phase_b(layer)

        @pl.when(layer == 0)
        def _():
            for c in w_copies[1:]:
                c.wait()

        moe(layer)

        @pl.when(layer == 0)
        def _():
            vmax_ref[...] = jnp.zeros((8, 128), F32)
            ln1(0, hbufs[0])

        return carry

    lax.fori_loop(0, 2, layer_body, 0)


@jax.jit
def pallas_interleave_layers__sliding_block__moe_arch_mod__prompt_kernel(
    A_x: jax.Array,
    A_wqkv: jax.Array,
    A_wo: jax.Array,
    B_x: jax.Array,
    B_w_r: jax.Array,
    B_w_gate: jax.Array,
    B_w_up: jax.Array,
    B_w_down: jax.Array,
):
    del B_x
    hbm = pl.BlockSpec(memory_space=pl.ANY)
    scratch = [
        pltpu.VMEM((S // 2, D), U32),
        pltpu.VMEM((S // 2, D), U32),
        pltpu.VMEM((MB // 2, D), U32),
        pltpu.VMEM((MB // 2, D), U32),
        pltpu.VMEM((D // 2, S), U32),
        pltpu.VMEM((S // 2, D), U32),
        pltpu.VMEM((D // 2, S), U32),
        pltpu.VMEM((D // 2, 3 * D), U32),
        pltpu.VMEM((D, D), U32),
        pltpu.VMEM((D // 2, D), U32),
        pltpu.VMEM((D // 2, FF), U32),
        pltpu.VMEM((D // 2, FF), U32),
        pltpu.VMEM((FF // 2, D), U32),
        pltpu.VMEM((1, 128, 512), U32),
        pltpu.VMEM((1, 128, 512), U32),
        pltpu.VMEM((1, 128, 512), U32),
        pltpu.VMEM((2, 256, 256), U32),
        pltpu.VMEM((8, 128), F32),
        pltpu.VMEM((NQB, 8, 128), F32),
        pltpu.VMEM((NQB, 8, 128), I32),
        pltpu.SMEM((4,), I32),
        pltpu.SMEM((2,), I32),
        pltpu.SemaphoreType.DMA((NMB,)),
        pltpu.SemaphoreType.DMA((9,)),
        pltpu.SemaphoreType.DMA((2,)),
    ]
    out = pl.pallas_call(
        _kernel,
        out_shape=jax.ShapeDtypeStruct((S, D), BF16),
        in_specs=[hbm, hbm, hbm, pl.BlockSpec(memory_space=pltpu.VMEM), hbm, hbm, hbm],
        out_specs=hbm,
        scratch_shapes=scratch,
        compiler_params=pltpu.CompilerParams(vmem_limit_bytes=110 * 1024 * 1024),
        name="swa_moe_fused",
    )(A_x.reshape(S, D), A_wqkv, A_wo, B_w_r, B_w_gate, B_w_up, B_w_down)
    return out.reshape(1, S, D)
```

```python
import math

import jax
import jax.numpy as jnp
from jax import lax
import jax.experimental.pallas as pl
import jax.experimental.pallas.tpu as pltpu

S = 2048
D = 1024
NH = 32
DH = 32
WIN = 256
FF = 3584
QB = 128
NQB = S // QB
MB = 256
NMB = S // MB
EPS = 1e-5
QSCALE = (DH ** -0.5) * math.log2(math.e)
NEG = -1e30
BIG = 2 ** 30
L_LO = 2.0 ** -64
L_HI = 2.0 ** 64
V_HI = 2.0 ** 60

F32 = jnp.float32
BF16 = jnp.bfloat16
U32 = jnp.uint32
I32 = jnp.int32

NT = (((1,), (1,)), ((), ()))
TN = (((0,), (0,)), ((), ()))


def _rnd(v):
    return v.astype(BF16).astype(F32)


def _ln(xf):
    m = jnp.mean(xf, axis=-1, keepdims=True)
    xc = xf - m
    v = jnp.mean(xc * xc, axis=-1, keepdims=True)
    return xc * lax.rsqrt(v + EPS)


def _ln_stats(xf):
    m = jnp.sum(xf, axis=-1, keepdims=True) * (1.0 / D)
    v = jnp.sum(xf * xf, axis=-1, keepdims=True) * (1.0 / D) - m * m
    return m, lax.rsqrt(jnp.maximum(v, 0.0) + EPS)


def _recip(l):
    r = pl.reciprocal(l, approx=True)
    return r * (2.0 - l * r)


def _mo(v, m):
    return v if isinstance(v, int) else pl.multiple_of(v, m)


def _kernel(x_hbm, wqkv_hbm, wo_hbm, wr_ref, wg_hbm, wu_hbm, wd_hbm, out_hbm,
            xn_u, x1_u, h0_u, h1_u, qt_u, k_u, vt_u,
            wqkv_u, wqvt_u, wo_u, wg_u, wu_u, wd_u,
            p0, p1, p2, ot_u, vmax_ref, bmax_ref, bidx_ref, zs, flag,
            sem_x, sem_w, sem_o):
    xn = xn_u.bitcast(BF16)
    x1_b = x1_u.bitcast(BF16)
    hbufs = (h0_u.bitcast(BF16), h1_u.bitcast(BF16))
    qt_b = qt_u.bitcast(BF16)
    k_b = k_u.bitcast(BF16)
    vt_b = vt_u.bitcast(BF16)
    wqkv = wqkv_u.bitcast(BF16)
    wqvt = wqvt_u.bitcast(BF16)
    wo = wo_u.bitcast(BF16)
    wg = wg_u.bitcast(BF16)
    wu = wu_u.bitcast(BF16)
    wd = wd_u.bitcast(BF16)
    ot_b = ot_u.bitcast(BF16)
    otbufs = (ot_b.at[0], ot_b.at[1])
    pbufs_u = (p0, p1, p2)
    pbufs_b = tuple(p.bitcast(BF16) for p in pbufs_u)

    def x_copy(j):
        return pltpu.make_async_copy(x_hbm.at[pl.ds(j * MB, MB), :],
                                     xn.at[pl.ds(j * MB, MB), :], sem_x.at[j])

    def wqkv_copy(c0, n, k):
        return pltpu.make_async_copy(wqkv_hbm.at[:, pl.ds(c0, n)],
                                     wqkv.at[:, pl.ds(c0, n)], sem_w.at[k])

    HD = D // 2
    wq_copies = [wqkv_copy(0, HD, 0), wqkv_copy(HD, HD, 1)]
    wv_copies = [wqkv_copy(2 * D, HD, 2), wqkv_copy(2 * D + HD, HD, 7)]
    wk_copy = wqkv_copy(D, D, 8)

    w_copies = [
        pltpu.make_async_copy(wo_hbm, wo, sem_w.at[3]),
        pltpu.make_async_copy(wg_hbm, wg, sem_w.at[4]),
        pltpu.make_async_copy(wu_hbm, wu, sem_w.at[5]),
        pltpu.make_async_copy(wd_hbm, wd, sem_w.at[6]),
    ]
    x_copy(0).start()
    wq_copies[0].start()
    wq_copies[1].start()
    wv_copies[0].start()
    wv_copies[1].start()
    x_copy(1).start()
    x_copy(2).start()
    wk_copy.start()
    for j in range(3, NMB):
        x_copy(j).start()

    for t in range(8):
        zs[t] = 0
    vmax_ref[...] = jnp.zeros((8, 128), F32)

    eye = (lax.broadcasted_iota(I32, (128, 128), 0)
           == lax.broadcasted_iota(I32, (128, 128), 1)).astype(F32).astype(BF16)

    def transpose_w(src_col0, dst_row0, tiles):
        for t in tiles:
            w_t = wqkv[:, src_col0 + 128 * t:src_col0 + 128 * (t + 1)]
            wqvt[dst_row0 + 128 * t:dst_row0 + 128 * (t + 1), :] = lax.dot_general(
                eye, w_t, NT, preferred_element_type=F32).astype(BF16)

    def ln1(row0, dst):
        src = xn.at[pl.ds(row0, MB), :]
        for c in range(MB // 64):
            xf = src[64 * c:64 * (c + 1), :].astype(F32)
            dst[64 * c:64 * (c + 1), :] = _ln(xf).astype(BF16)

    def track_v(v):
        a = jnp.max(jnp.abs(v).reshape(v.shape[0] // 8, 8, v.shape[1]), axis=0)
        a = jnp.maximum(a[:, 0:128], a[:, 128:256])
        a = jnp.broadcast_to(jnp.max(a, axis=0, keepdims=True), (8, 128))
        vmax_ref[...] = jnp.maximum(vmax_ref[...], a)

    def proj_t(row0, n, base, hsrc):
        r = lax.dot_general(wqvt[row0:row0 + n, :], hsrc[...], NT, preferred_element_type=F32)
        if row0 < D:
            qt_b[row0:row0 + n, pl.ds(base, MB)] = (r * QSCALE).astype(BF16)
        else:
            vt_b[row0 - D:row0 - D + n, pl.ds(base, MB)] = r.astype(BF16)
            track_v(r)

    def proj_qv(base, hsrc):
        qv = lax.dot_general(wqvt[...], hsrc[...], NT, preferred_element_type=F32)
        qt_b[:, pl.ds(base, MB)] = (qv[0:D] * QSCALE).astype(BF16)
        vt_b[:, pl.ds(base, MB)] = qv[D:2 * D].astype(BF16)
        track_v(qv[D:2 * D])

    def proj_k(base, hsrc):
        k = jnp.dot(hsrc[...], wqkv[:, D:2 * D], preferred_element_type=F32)
        k_b[pl.ds(base, MB), :] = k.astype(BF16)

    def phase_a(layer):
        def body(t, carry):
            first = jnp.logical_and(layer == 0, t == 0)

            @pl.when(first)
            def _():
                x_copy(1).wait()
                x_copy(2).wait()
                wk_copy.wait()
                for c in w_copies:
                    c.start()

            @pl.when(jnp.logical_and(layer == 0, t >= 1))
            def _():
                x_copy(2 * t + 1).wait()

            @pl.when(jnp.logical_and(layer == 0, jnp.logical_and(t >= 1, t < NMB // 2 - 1)))
            def _():
                x_copy(2 * t + 2).wait()

            b0 = pl.multiple_of(2 * t * MB, MB)
            b1 = pl.multiple_of(b0 + MB, MB)
            b2 = pl.multiple_of(jnp.minimum(2 * t + 2, NMB - 1) * MB, MB)

            @pl.when(jnp.logical_not(first))
            def _():
                proj_qv(b0, hbufs[0])

            proj_k(b0, hbufs[0])
            ln1(b1, hbufs[1])
            proj_qv(b1, hbufs[1])
            proj_k(b1, hbufs[1])
            ln1(b2, hbufs[0])
            return carry

        lax.fori_loop(0, NMB // 2, body, 0)

    x_copy(0).wait()
    ln1(0, hbufs[0])
    for k in range(2):
        wq_copies[k].wait()
        transpose_w(k * HD, k * HD, range(4))
        proj_t(k * HD, HD, 0, hbufs[0])
    for k in range(2):
        wv_copies[k].wait()
        transpose_w(2 * D + k * HD, D + k * HD, range(4))
        proj_t(D + k * HD, HD, 0, hbufs[0])

    def attention(blocks):
        zst = zs[0]
        zld = zs[1]
        lane = lax.broadcasted_iota(I32, (QB, QB), 1)
        row = lax.broadcasted_iota(I32, (QB, QB), 0)
        newmask = row <= lane
        p_st = [p.at[zst] for p in pbufs_b]
        p_ld = [p.at[zld] for p in pbufs_u]
        zero32 = jnp.zeros((32, QB), BF16)
        good = [None] * len(blocks)
        lsums = {}
        views = []
        for (i, nkb) in blocks:
            r0 = _mo(i * QB, QB)
            k0 = 128 * (nkb - 1)
            views.append((qt_b.at[:, pl.ds(r0, QB)],
                          k_b.at[pl.ds(r0 - k0, k0 + QB), :],
                          vt_b.at[:, pl.ds(r0 - k0, k0 + QB)]))

        def qk(n, g, slot):
            nkb = blocks[n][1]
            k0 = 128 * (nkb - 1)
            qw, kw, _ = views[n]
            cs = slice(128 * g, 128 * (g + 1))
            ws = []
            for j in range(4):
                h = 4 * g + j
                ws.append(jnp.concatenate(
                    [zero32] * j + [qw[32 * h:32 * (h + 1), :]] + [zero32] * (3 - j), axis=0))
            w = jnp.concatenate(ws, axis=1)
            parts = [kw[k0:k0 + 128, cs]]
            if nkb == 2:
                parts.append(kw[0:128, cs])
            kk = jnp.concatenate(parts, axis=0)
            st = jnp.dot(kk, w, preferred_element_type=F32)
            pref = p_st[slot]
            for j in range(4):
                s = st[:, 128 * j:128 * (j + 1)]
                ls = slice(128 * j, 128 * (j + 1))
                acc = [None, None]

                def put(row0, e, k):
                    pref[row0:row0 + 16, ls] = e.astype(BF16)
                    acc[k] = e if acc[k] is None else acc[k] + e

                for c in range(8):
                    f = jnp.where(newmask[16 * c:16 * c + 16], s[16 * c:16 * c + 16], NEG)
                    put(16 * c, jnp.exp2(f), c % 2)
                if nkb == 2:
                    for c in range(8):
                        put(128 + 16 * c, jnp.exp2(s[128 + 16 * c:128 + 16 * c + 16]), c % 2)
                t = acc[0] + acc[1]
                lsums[(slot, j)] = jnp.sum(t[0:8] + t[8:16], axis=0, keepdims=True)

        def pv(n, g, j, slot):
            nkb = blocks[n][1]
            vw = views[n][2]
            h = 4 * g + j
            pref = p_ld[slot]
            ls = slice(128 * j, 128 * (j + 1))
            p = pref[0:64, ls]
            if nkb == 2:
                p = jnp.concatenate([pref[64:128, ls], p], axis=0)
            vt = vw[32 * h:32 * (h + 1), :]
            ot = jnp.dot(vt, pltpu.bitcast(p, BF16), preferred_element_type=F32)
            l = lsums.pop((slot, j))
            ok = (l >= L_LO) & (l <= L_HI)
            good[n] = ok if good[n] is None else (good[n] & ok)
            o = (ot * _recip(l)).astype(BF16)
            otbufs[n][32 * (h % 16):32 * (h % 16) + 32,
                      128 * (h // 16):128 * (h // 16) + 128] = o

        lane8 = lax.broadcasted_iota(I32, (1, 8, QB), 2)
        bit0z = (lane8 & 32) == 0
        bit1z = (lane8 & 64) == 0
        blk8 = lane8 >> 5
        t32 = lax.broadcasted_iota(I32, (32, QB), 0)
        new32 = t32 <= (lax.broadcasted_iota(I32, (32, QB), 1) & 31)
        r16 = lax.broadcasted_iota(I32, (16, QB), 0) * 2
        c16 = lax.broadcasted_iota(I32, (16, QB), 1) & 31
        pn32 = (jnp.where(r16 <= c16, U32(0xFFFF), U32(0))
                | jnp.where(r16 + 1 <= c16, U32(0xFFFF0000), U32(0)))

        def lsel(mask, x, y):
            if x is None and y is None:
                return None
            ref = x if y is None else y
            shp = ref.shape
            zero = jnp.zeros((), ref.dtype)
            if shp[0] % 8 == 0:
                x3 = zero if x is None else x.reshape(shp[0] // 8, 8, QB)
                y3 = zero if y is None else y.reshape(shp[0] // 8, 8, QB)
                return jnp.where(mask, x3, y3).reshape(shp)
            return jnp.where(mask[0, 0:shp[0]], zero if x is None else x, zero if y is None else y)

        def xperm(x, j):
            if j & 1:
                x = lsel(bit0z, pltpu.roll(x, 96, 1), pltpu.roll(x, 32, 1))
            if j & 2:
                x = pltpu.roll(x, 64, 1)
            return x

        def butterfly(a):
            e = [[lsel(bit0z, a[2 * q + j0], a[2 * q + (1 ^ j0)]) for j0 in range(2)]
                 for q in range(2)]
            return [lsel(bit1z, e[j >> 1][j & 1], e[1 ^ (j >> 1)][j & 1]) for j in range(4)]

        def qk4(n, g, slot):
            qw, kw, _ = views[n]
            cs = slice(128 * g, 128 * (g + 1))
            pref = p_st[slot]
            ys = [xperm(pltpu.bitcast(qw[32 * (4 * g + j):32 * (4 * g + j) + 32, :], U32), j)
                  for j in range(4)]
            for u in range(4):
                w = pltpu.bitcast(jnp.concatenate(
                    [lsel(blk8 == (j ^ u), ys[j], None) for j in range(4)], axis=0), BF16)
                k0 = 32 * u
                parts = []
                for c in range(2):
                    parts.append(kw[k0 + 16 * c:k0 + 16 * c + 16, cs])
                    parts.append(kw[k0 + 256 + 16 * c:k0 + 256 + 16 * c + 16, cs])
                parts.append(kw[k0 + 32:k0 + 256, cs])
                s = jnp.dot(jnp.concatenate(parts, axis=0), w, preferred_element_type=F32)
                ls = slice(128 * u, 128 * (u + 1))
                acc = [None, None]

                def put(row0, e, k):
                    pref[row0:row0 + 16, ls] = e.astype(BF16)
                    acc[k] = e if acc[k] is None else acc[k] + e

                for c in range(2):
                    f = jnp.where(new32[16 * c:16 * c + 16], s[32 * c + 16:32 * c + 32],
                                  s[32 * c:32 * c + 16])
                    put(16 * c, jnp.exp2(f), c % 2)
                for c in range(14):
                    put(32 + 16 * c, jnp.exp2(s[64 + 16 * c:64 + 16 * c + 16]), c % 2)
                t = acc[0] + acc[1]
                lsums[(slot, u)] = jnp.sum(t[0:8] + t[8:16], axis=0, keepdims=True)

        def pv4(n, g, slot):
            vw = views[n][2]
            ots = []
            for j in range(4):
                pref = pbufs_u[slot].at[zs[1 + j]]

                def blk(u, be):
                    ls = slice(128 * u, 128 * (u + 1))
                    if be < 0 or be > 8:
                        return None
                    if be == 0:
                        f = pref[0:16, ls]
                        return f ^ (f & pn32)
                    if be == 8:
                        return pref[0:16, ls] & pn32
                    return pref[16 * be:16 * be + 16, ls]

                tiles = []
                for b in range(12):
                    a = [blk(u, b - u) for u in range(4)]
                    o = lsel(bit1z, lsel(bit0z, a[j], a[j ^ 1]), lsel(bit0z, a[j ^ 2], a[j ^ 3]))
                    tiles.append(jnp.zeros((16, QB), U32) if o is None else o)
                ots.append(jnp.dot(vw[32 * (4 * g + j):32 * (4 * g + j + 1), :],
                                   pltpu.bitcast(jnp.concatenate(tiles, axis=0), BF16),
                                   preferred_element_type=F32))
            ls4 = butterfly([lsums.pop((slot, u)) for u in range(4)])
            for j in range(4):
                h = 4 * g + j
                ot = ots[j]
                l = ls4[j]
                ok = (l >= L_LO) & (l <= L_HI)
                good[n] = ok if good[n] is None else (good[n] & ok)
                o = xperm(ot * _recip(l), j)
                otbufs[n][32 * (h % 16):32 * (h % 16) + 32,
                          128 * (h // 16):128 * (h // 16) + 128] = o.astype(BF16)

        seq = [(n, g) for n in range(len(blocks)) for g in range(8)]
        for s in range(len(seq) + 2):
            if s < len(seq):
                n, g = seq[s]
                (qk4 if blocks[n][1] == 3 else qk)(n, g, s % 3)
            if s >= 2:
                n, g = seq[s - 2]
                if blocks[n][1] == 3:
                    pv4(n, g, (s - 2) % 3)
                else:
                    for j in range(4):
                        pv(n, g, j, (s - 2) % 3)
        v_ok = vmax_ref[0:1, :] <= V_HI
        for n in range(len(blocks)):
            flag[n] = jnp.min(jnp.where(good[n] & v_ok, 1, 0))

    def attention_safe(i, ow):
        r0 = _mo(i * QB, QB)
        start = pl.multiple_of(jnp.maximum(i - 2, 0) * QB, QB)
        qw = qt_b.at[:, pl.ds(r0, QB)]
        kw = k_b.at[pl.ds(start, 3 * QB), :]
        vw = vt_b.at[:, pl.ds(start, 3 * QB)]
        key = lax.broadcasted_iota(I32, (3 * QB, QB), 0) + start
        qry = lax.broadcasted_iota(I32, (3 * QB, QB), 1) + r0
        valid = (qry - key >= 0) & (qry - key < WIN)
        drow = lax.broadcasted_iota(I32, (128, QB), 0)

        def head(h, carry):
            g0 = pl.multiple_of((h // 4) * 128, 128)
            j0 = (h % 4) * 32
            q4 = qw[pl.ds(g0, 128), :].astype(F32)
            w = jnp.where((drow >= j0) & (drow < j0 + 32), q4, 0.0).astype(BF16)
            s = jnp.dot(kw[:, pl.ds(g0, 128)], w, preferred_element_type=F32)
            s = jnp.where(valid, s, NEG)
            m = jnp.max(s, axis=0, keepdims=True)
            p = jnp.exp2(s - m).astype(BF16)
            l = jnp.sum(p.astype(F32), axis=0, keepdims=True)
            vt = vw[pl.ds(pl.multiple_of(h * 32, 32), 32), :]
            o = jnp.dot(vt, p, preferred_element_type=F32) * (1.0 / l)
            ow[pl.ds(pl.multiple_of((h % 16) * 32, 32), 32),
               pl.ds(pl.multiple_of((h // 16) * 128, 128), 128)] = o.astype(BF16)
            return carry

        lax.fori_loop(0, NH, head, 0)

    def out_proj(n, xsrc, x1dst, z=0):
        ow = ot_b.at[n + z]
        o = jnp.concatenate([ow[:, 0:128], ow[:, 128:256]], axis=0)
        y = lax.dot_general(o, wo[...], TN, preferred_element_type=F32)
        x1dst[...] = (xsrc[...].astype(F32) + y).astype(BF16)

    def ln2(b, x1src, x2dst, CH=16, NCHAIN=8, z_in=0):
        rb = _mo(b * QB, QB)
        wr = wr_ref[...].astype(F32).reshape(1, D)
        wsum = jnp.sum(wr, axis=-1, keepdims=True)
        bm = None
        bi = None
        sub = lax.broadcasted_iota(I32, (8, 1), 0)
        toks = []
        for c in range(QB // CH):
            z = toks[c - NCHAIN] if c >= NCHAIN else z_in
            if isinstance(z, int):
                x1 = x1src[CH * c:CH * (c + 1), :].astype(F32)
            else:
                x1 = x1src[pl.ds(pl.multiple_of(CH * c + z * 16, 16), CH), :].astype(F32)
            m, rs = _ln_stats(x1)
            x2dst[CH * c:CH * (c + 1), :] = (x1 * (1.0 + rs) - m * rs).astype(BF16)
            r = _rnd(rs * (jnp.sum(x1 * wr, axis=-1, keepdims=True) - m * wsum))
            ru = lax.bitcast_convert_type(r, I32)
            toks.append(jnp.max(lax.shift_right_logical(lax.shift_right_logical(ru, 16), 16)))
            for t in range(CH // 8):
                rt = r[8 * t:8 * t + 8]
                it = sub + (rb + CH * c + 8 * t)
                if bm is None:
                    bm, bi = rt, it
                else:
                    better = rt > bm
                    bm = jnp.where(better, rt, bm)
                    bi = jnp.where(better, it, bi)
        bmax_ref[b] = jnp.broadcast_to(bm, (8, 128))
        bidx_ref[b] = jnp.broadcast_to(bi, (8, 128))
        tok = toks[-1]
        for k in range(2, min(NCHAIN, len(toks)) + 1):
            tok = tok + toks[-k]
        return tok

    def checks(i0):
        def one(n, carry):
            @pl.when(flag[n] == 0)
            def _():
                rb = pl.multiple_of((i0 + n) * QB, QB)
                attention_safe(i0 + n, ot_b.at[n])
                out_proj(n, xn.at[pl.ds(rb, QB), :], x1_b.at[pl.ds(rb, QB), :])
            return carry

        @pl.when(flag[0] + flag[1] < 2)
        def _():
            lax.fori_loop(0, 2, one, 0)

    def out_copy(b):
        return pltpu.make_async_copy(xn.at[pl.ds(b * QB, QB), :],
                                     out_hbm.at[pl.ds(b * QB, QB), :], sem_o.at[0])

    def phase_b(layer):
        attention([(0, 1), (1, 2)])
        out_proj(0, xn.at[0:QB, :], x1_b.at[0:QB, :])
        out_proj(1, xn.at[QB:2 * QB, :], x1_b.at[QB:2 * QB, :])

        def body(t, carry):
            i0 = 2 * t
            checks(i0 - 2)

            @pl.when(jnp.logical_and(layer == 1, t >= 2))
            def _():
                out_copy(i0 - 4).start()
                out_copy(i0 - 3).start()

            @pl.when(t < NQB // 2)
            def _():
                r2 = pl.multiple_of((i0 - 2) * QB, QB)
                xv = xn.at[pl.ds(r2, 4 * QB), :]
                x1v = x1_b.at[pl.ds(r2, 4 * QB), :]
                ln2(i0 - 2, x1v.at[0:QB, :], xv.at[0:QB, :])
                ln2(i0 - 1, x1v.at[QB:2 * QB, :], xv.at[QB:2 * QB, :])
                attention([(i0, 3), (i0 + 1, 3)])
                out_proj(0, xv.at[2 * QB:3 * QB, :], x1v.at[2 * QB:3 * QB, :])
                out_proj(1, xv.at[3 * QB:4 * QB, :], x1v.at[3 * QB:4 * QB, :])
            return carry

        lax.fori_loop(1, NQB // 2 + 1, body, 0)
        for b in (NQB - 2, NQB - 1):
            ln2(b, x1_b.at[b * QB:(b + 1) * QB, :], xn.at[b * QB:(b + 1) * QB, :], NCHAIN=8)

        @pl.when(layer == 1)
        def _():
            out_copy(NQB - 2).start()
            out_copy(NQB - 1).start()

    def moe(layer):
        rm = bmax_ref[:, :, 0:1]
        ri = bidx_ref[:, :, 0:1]
        gm = jnp.max(jnp.max(rm, axis=0), axis=0, keepdims=True)
        idx = jnp.min(jnp.where(rm == gm, ri, BIG))
        b16 = pl.multiple_of((idx // 16) * 16, 16)
        ln1(0, hbufs[0])
        x1c = x1_b[pl.ds(b16, 16), :].astype(F32)
        h2c = _rnd(_ln(x1c))
        hb = h2c.astype(BF16)
        g = _rnd(jnp.dot(hb, wg[...], preferred_element_type=F32))
        u = _rnd(jnp.dot(hb, wu[...], preferred_element_type=F32))
        g = _rnd(g * _rnd(jax.nn.sigmoid(g)))
        act = (g * u).astype(BF16)
        y = _rnd(jnp.dot(act, wd[...], preferred_element_type=F32))
        y = _rnd(y * _rnd(jax.nn.sigmoid(gm)))
        x2n = x1c + _rnd(h2c + y)

        @pl.when(layer == 1)
        def _():
            for b in range(NQB):
                out_copy(b).wait()

        cur = xn[pl.ds(b16, 16), :].astype(F32)
        sel = lax.broadcasted_iota(I32, (16, D), 0) == (idx - b16)
        xn[pl.ds(b16, 16), :] = jnp.where(sel, x2n, cur).astype(BF16)

        @pl.when(jnp.logical_and(layer == 0, idx < MB))
        def _():
            ln1(0, hbufs[0])

        @pl.when(layer == 1)
        def _():
            cp = pltpu.make_async_copy(xn.at[pl.ds(b16, 16), :],
                                       out_hbm.at[pl.ds(b16, 16), :], sem_o.at[1])
            cp.start()
            cp.wait()

    def layer_body(layer, carry):
        phase_a(layer)

        @pl.when(layer == 0)
        def _():
            w_copies[0].wait()

        phase_b(layer)

        @pl.when(layer == 0)
        def _():
            for c in w_copies[1:]:
                c.wait()

        moe(layer)

        vmax_ref[...] = jnp.zeros((8, 128), F32)
        return carry

    lax.fori_loop(0, 2, layer_body, 0)


@jax.jit
def pallas_interleave_layers__sliding_block__moe_arch_mod__prompt_kernel(
    A_x: jax.Array,
    A_wqkv: jax.Array,
    A_wo: jax.Array,
    B_x: jax.Array,
    B_w_r: jax.Array,
    B_w_gate: jax.Array,
    B_w_up: jax.Array,
    B_w_down: jax.Array,
):
    del B_x
    hbm = pl.BlockSpec(memory_space=pl.ANY)
    scratch = [
        pltpu.VMEM((S // 2, D), U32),
        pltpu.VMEM((S // 2, D), U32),
        pltpu.VMEM((MB // 2, D), U32),
        pltpu.VMEM((MB // 2, D), U32),
        pltpu.VMEM((D // 2, S), U32),
        pltpu.VMEM((S // 2, D), U32),
        pltpu.VMEM((D // 2, S), U32),
        pltpu.VMEM((D // 2, 3 * D), U32),
        pltpu.VMEM((D, D), U32),
        pltpu.VMEM((D // 2, D), U32),
        pltpu.VMEM((D // 2, FF), U32),
        pltpu.VMEM((D // 2, FF), U32),
        pltpu.VMEM((FF // 2, D), U32),
        pltpu.VMEM((1, 128, 512), U32),
        pltpu.VMEM((1, 128, 512), U32),
        pltpu.VMEM((1, 128, 512), U32),
        pltpu.VMEM((2, 256, 256), U32),
        pltpu.VMEM((8, 128), F32),
        pltpu.VMEM((NQB, 8, 128), F32),
        pltpu.VMEM((NQB, 8, 128), I32),
        pltpu.SMEM((8,), I32),
        pltpu.SMEM((2,), I32),
        pltpu.SemaphoreType.DMA((NMB,)),
        pltpu.SemaphoreType.DMA((9,)),
        pltpu.SemaphoreType.DMA((2,)),
    ]
    out = pl.pallas_call(
        _kernel,
        out_shape=jax.ShapeDtypeStruct((S, D), BF16),
        in_specs=[hbm, hbm, hbm, pl.BlockSpec(memory_space=pltpu.VMEM), hbm, hbm, hbm],
        out_specs=hbm,
        scratch_shapes=scratch,
        compiler_params=pltpu.CompilerParams(vmem_limit_bytes=110 * 1024 * 1024),
        name="swa_moe_fused",
    )(A_x.reshape(S, D), A_wqkv, A_wo, B_w_r, B_w_gate, B_w_up, B_w_down)
    return out.reshape(1, S, D)
```

```python
import math

import jax
import jax.numpy as jnp
from jax import lax
import jax.experimental.pallas as pl
import jax.experimental.pallas.tpu as pltpu

S = 2048
D = 1024
NH = 32
DH = 32
WIN = 256
FF = 3584
QB = 128
NQB = S // QB
MB = 256
NMB = S // MB
EPS = 1e-5
QSCALE = (DH ** -0.5) * math.log2(math.e)
NEG = -1e30
BIG = 2 ** 30
L_LO = 2.0 ** -64
L_HI = 2.0 ** 64
V_HI = 2.0 ** 60

F32 = jnp.float32
BF16 = jnp.bfloat16
U32 = jnp.uint32
I32 = jnp.int32

NT = (((1,), (1,)), ((), ()))
TN = (((0,), (0,)), ((), ()))


def _rnd(v):
    return v.astype(BF16).astype(F32)


def _ln(xf):
    m = jnp.mean(xf, axis=-1, keepdims=True)
    xc = xf - m
    v = jnp.mean(xc * xc, axis=-1, keepdims=True)
    return xc * lax.rsqrt(v + EPS)


def _ln_stats(xf):
    m = jnp.sum(xf, axis=-1, keepdims=True) * (1.0 / D)
    v = jnp.sum(xf * xf, axis=-1, keepdims=True) * (1.0 / D) - m * m
    return m, lax.rsqrt(jnp.maximum(v, 0.0) + EPS)


def _recip(l):
    r = pl.reciprocal(l, approx=True)
    return r * (2.0 - l * r)


def _mo(v, m):
    return v if isinstance(v, int) else pl.multiple_of(v, m)


def _kernel(x_hbm, wqkv_hbm, wo_hbm, wr_ref, wg_hbm, wu_hbm, wd_hbm, out_hbm,
            xn_u, x1_u, h0_u, h1_u, qt_u, k_u, vt_u,
            wqkv_u, wqvt_u, wo_u, wg_u, wu_u, wd_u,
            p0, p1, p2, ot_u, vmax_ref, bmax_ref, bidx_ref, zs, flag,
            sem_x, sem_w, sem_o):
    xn = xn_u.bitcast(BF16)
    x1_b = x1_u.bitcast(BF16)
    hbufs = (h0_u.bitcast(BF16), h1_u.bitcast(BF16))
    qt_b = qt_u.bitcast(BF16)
    k_b = k_u.bitcast(BF16)
    vt_b = vt_u.bitcast(BF16)
    wqkv = wqkv_u.bitcast(BF16)
    wqvt = wqvt_u.bitcast(BF16)
    wo = wo_u.bitcast(BF16)
    wg = wg_u.bitcast(BF16)
    wu = wu_u.bitcast(BF16)
    wd = wd_u.bitcast(BF16)
    ot_b = ot_u.bitcast(BF16)
    otbufs = (ot_b.at[0], ot_b.at[1])
    pbufs_u = (p0, p1, p2)
    pbufs_b = tuple(p.bitcast(BF16) for p in pbufs_u)

    def x_copy(j):
        return pltpu.make_async_copy(x_hbm.at[pl.ds(j * MB, MB), :],
                                     xn.at[pl.ds(j * MB, MB), :], sem_x.at[j])

    def wqkv_copy(c0, n, k):
        return pltpu.make_async_copy(wqkv_hbm.at[:, pl.ds(c0, n)],
                                     wqkv.at[:, pl.ds(c0, n)], sem_w.at[k])

    HD = D // 2
    wq_copies = [wqkv_copy(0, HD, 0), wqkv_copy(HD, HD, 1)]
    wv_copies = [wqkv_copy(2 * D, HD, 2), wqkv_copy(2 * D + HD, HD, 7)]
    wk_copy = wqkv_copy(D, D, 8)

    w_copies = [
        pltpu.make_async_copy(wo_hbm, wo, sem_w.at[3]),
        pltpu.make_async_copy(wg_hbm, wg, sem_w.at[4]),
        pltpu.make_async_copy(wu_hbm, wu, sem_w.at[5]),
        pltpu.make_async_copy(wd_hbm, wd, sem_w.at[6]),
    ]
    x_copy(0).start()
    wq_copies[0].start()
    wq_copies[1].start()
    wv_copies[0].start()
    wv_copies[1].start()
    x_copy(1).start()
    x_copy(2).start()
    wk_copy.start()
    for j in range(3, NMB):
        x_copy(j).start()

    for t in range(8):
        zs[t] = 0
    vmax_ref[...] = jnp.zeros((8, 128), F32)

    eye = (lax.broadcasted_iota(I32, (128, 128), 0)
           == lax.broadcasted_iota(I32, (128, 128), 1)).astype(F32).astype(BF16)

    def transpose_w(src_col0, dst_row0, tiles):
        for t in tiles:
            w_t = wqkv[:, src_col0 + 128 * t:src_col0 + 128 * (t + 1)]
            wqvt[dst_row0 + 128 * t:dst_row0 + 128 * (t + 1), :] = lax.dot_general(
                eye, w_t, NT, preferred_element_type=F32).astype(BF16)

    def ln1(row0, dst):
        src = xn.at[pl.ds(row0, MB), :]
        for c in range(MB // 64):
            xf = src[64 * c:64 * (c + 1), :].astype(F32)
            dst[64 * c:64 * (c + 1), :] = _ln(xf).astype(BF16)

    def track_v(v):
        a = jnp.max(jnp.abs(v).reshape(v.shape[0] // 8, 8, v.shape[1]), axis=0)
        a = jnp.maximum(a[:, 0:128], a[:, 128:256])
        a = jnp.broadcast_to(jnp.max(a, axis=0, keepdims=True), (8, 128))
        vmax_ref[...] = jnp.maximum(vmax_ref[...], a)

    def proj_t(row0, n, base, hsrc):
        r = lax.dot_general(wqvt[row0:row0 + n, :], hsrc[...], NT, preferred_element_type=F32)
        if row0 < D:
            qt_b[row0:row0 + n, pl.ds(base, MB)] = (r * QSCALE).astype(BF16)
        else:
            vt_b[row0 - D:row0 - D + n, pl.ds(base, MB)] = r.astype(BF16)
            track_v(r)

    def proj_qv(base, hsrc):
        qv = lax.dot_general(wqvt[...], hsrc[...], NT, preferred_element_type=F32)
        qt_b[:, pl.ds(base, MB)] = (qv[0:D] * QSCALE).astype(BF16)
        vt_b[:, pl.ds(base, MB)] = qv[D:2 * D].astype(BF16)
        track_v(qv[D:2 * D])

    def proj_k(base, hsrc):
        k = jnp.dot(hsrc[...], wqkv[:, D:2 * D], preferred_element_type=F32)
        k_b[pl.ds(base, MB), :] = k.astype(BF16)

    def phase_a(layer):
        def body(t, carry):
            first = jnp.logical_and(layer == 0, t == 0)

            @pl.when(first)
            def _():
                x_copy(1).wait()
                x_copy(2).wait()
                wk_copy.wait()
                for c in w_copies:
                    c.start()

            @pl.when(jnp.logical_and(layer == 0, t >= 1))
            def _():
                x_copy(2 * t + 1).wait()

            @pl.when(jnp.logical_and(layer == 0, jnp.logical_and(t >= 1, t < NMB // 2 - 1)))
            def _():
                x_copy(2 * t + 2).wait()

            b0 = pl.multiple_of(2 * t * MB, MB)
            b1 = pl.multiple_of(b0 + MB, MB)
            b2 = pl.multiple_of(jnp.minimum(2 * t + 2, NMB - 1) * MB, MB)

            @pl.when(jnp.logical_not(first))
            def _():
                proj_qv(b0, hbufs[0])

            proj_k(b0, hbufs[0])
            ln1(b1, hbufs[1])
            proj_qv(b1, hbufs[1])
            proj_k(b1, hbufs[1])
            ln1(b2, hbufs[0])
            return carry

        lax.fori_loop(0, NMB // 2, body, 0)

    x_copy(0).wait()
    ln1(0, hbufs[0])
    for k in range(2):
        wq_copies[k].wait()
        transpose_w(k * HD, k * HD, range(4))
        proj_t(k * HD, HD, 0, hbufs[0])
    for k in range(2):
        wv_copies[k].wait()
        transpose_w(2 * D + k * HD, D + k * HD, range(4))
        proj_t(D + k * HD, HD, 0, hbufs[0])

    def attention(blocks):
        p_st = [p.at[zs[0]] for p in pbufs_b]
        good = [None] * len(blocks)
        lsums = {}
        views = []
        for (i, nkb) in blocks:
            r0 = _mo(i * QB, QB)
            k0 = 128 * (nkb - 1)
            views.append((qt_b.at[:, pl.ds(r0, QB)],
                          k_b.at[pl.ds(r0 - k0, k0 + QB), :],
                          vt_b.at[:, pl.ds(r0 - k0, k0 + QB)]))

        lane8 = lax.broadcasted_iota(I32, (1, 8, QB), 2)
        bit0z = (lane8 & 32) == 0
        bit1z = (lane8 & 64) == 0
        blk8 = lane8 >> 5
        t32 = lax.broadcasted_iota(I32, (32, QB), 0)
        new32 = t32 <= (lax.broadcasted_iota(I32, (32, QB), 1) & 31)
        r16 = lax.broadcasted_iota(I32, (16, QB), 0) * 2
        c16 = lax.broadcasted_iota(I32, (16, QB), 1) & 31
        pn32 = (jnp.where(r16 <= c16, U32(0xFFFF), U32(0))
                | jnp.where(r16 + 1 <= c16, U32(0xFFFF0000), U32(0)))

        def lsel(mask, x, y):
            if x is None and y is None:
                return None
            ref = x if y is None else y
            shp = ref.shape
            zero = jnp.zeros((), ref.dtype)
            if shp[0] % 8 == 0:
                x3 = zero if x is None else x.reshape(shp[0] // 8, 8, QB)
                y3 = zero if y is None else y.reshape(shp[0] // 8, 8, QB)
                return jnp.where(mask, x3, y3).reshape(shp)
            return jnp.where(mask[0, 0:shp[0]], zero if x is None else x, zero if y is None else y)

        def xperm(x, j):
            if j & 1:
                x = lsel(bit0z, pltpu.roll(x, 96, 1), pltpu.roll(x, 32, 1))
            if j & 2:
                x = pltpu.roll(x, 64, 1)
            return x

        def pick(a, j):
            return lsel(bit1z, lsel(bit0z, a[j], a[j ^ 1]), lsel(bit0z, a[j ^ 2], a[j ^ 3]))

        def qk(n, g, slot):
            nkb = blocks[n][1]
            qw, kw, _ = views[n]
            cs = slice(128 * g, 128 * (g + 1))
            pref = p_st[slot]
            ys = [xperm(pltpu.bitcast(qw[32 * (4 * g + j):32 * (4 * g + j) + 32, :], U32), j)
                  for j in range(4)]
            for u in (range(4) if nkb == 3 else [(g + k) % 4 for k in range(4)]):
                w = pltpu.bitcast(jnp.concatenate(
                    [lsel(blk8 == (j ^ u), ys[j], None) for j in range(4)], axis=0), BF16)
                dg = 128 * (nkb - 1) + 32 * u
                parts = []
                if nkb == 3:
                    for c in range(2):
                        parts.append(kw[32 * u + 16 * c:32 * u + 16 * c + 16, cs])
                        parts.append(kw[dg + 16 * c:dg + 16 * c + 16, cs])
                    parts.append(kw[32 * u + 32:dg, cs])
                    nmid = 7
                else:
                    parts.append(kw[dg:dg + 32, cs])
                    if dg > 0:
                        parts.append(kw[0:dg, cs])
                    nmid = dg // 32
                s = jnp.dot(jnp.concatenate(parts, axis=0), w, preferred_element_type=F32)
                ls = slice(128 * u, 128 * (u + 1))
                acc = [None, None]

                def put(row0, e, k):
                    pref[row0:row0 + 16, ls] = e.astype(BF16)
                    acc[k] = e if acc[k] is None else acc[k] + e

                for c in range(2):
                    if nkb == 3:
                        f = jnp.where(new32[16 * c:16 * c + 16], s[32 * c + 16:32 * c + 32],
                                      s[32 * c:32 * c + 16])
                    else:
                        f = jnp.where(new32[16 * c:16 * c + 16], s[16 * c:16 * c + 16], NEG)
                    put(16 * c, jnp.exp2(f), c % 2)
                m0 = 64 if nkb == 3 else 32
                for c in range(2 * nmid):
                    put(32 + 16 * c, jnp.exp2(s[m0 + 16 * c:m0 + 16 * c + 16]), c % 2)
                t = acc[0] + acc[1]
                lsums[(slot, u)] = jnp.sum(t[0:8] + t[8:16], axis=0, keepdims=True)

        def pv(n, g, slot):
            nkb = blocks[n][1]
            vw = views[n][2]
            ots = []
            for j in range(4):
                pref = pbufs_u[slot].at[zs[1 + j]]

                def blk(u, b):
                    ls = slice(128 * u, 128 * (u + 1))
                    if nkb == 3:
                        be = b - u
                        if be < 0 or be > 8:
                            return None
                        if be == 0:
                            f = pref[0:16, ls]
                            return f ^ (f & pn32)
                        if be == 8:
                            return pref[0:16, ls] & pn32
                        return pref[16 * be:16 * be + 16, ls]
                    nb = 4 * (nkb - 1) + u
                    if b > nb:
                        return None
                    if b == nb:
                        return pref[0:16, ls]
                    return pref[16 * (b + 1):16 * (b + 2), ls]

                tiles = []
                for b in range(4 * nkb):
                    o = pick([blk(u, b) for u in range(4)], j)
                    tiles.append(jnp.zeros((16, QB), U32) if o is None else o)
                ots.append(jnp.dot(vw[32 * (4 * g + j):32 * (4 * g + j + 1), :],
                                   pltpu.bitcast(jnp.concatenate(tiles, axis=0), BF16),
                                   preferred_element_type=F32))
            lu = [lsums.pop((slot, u)) for u in range(4)]
            for j in range(4):
                h = 4 * g + j
                l = pick(lu, j)
                ok = (l >= L_LO) & (l <= L_HI)
                good[n] = ok if good[n] is None else (good[n] & ok)
                o = xperm(ots[j] * _recip(l), j)
                otbufs[n][32 * (h % 16):32 * (h % 16) + 32,
                          128 * (h // 16):128 * (h // 16) + 128] = o.astype(BF16)

        seq = [(n, g) for n in range(len(blocks)) for g in range(8)]
        for s in range(len(seq) + 2):
            if s < len(seq):
                qk(seq[s][0], seq[s][1], s % 3)
            if s >= 2:
                pv(seq[s - 2][0], seq[s - 2][1], (s - 2) % 3)
        v_ok = vmax_ref[0:1, :] <= V_HI
        for n in range(len(blocks)):
            flag[n] = jnp.min(jnp.where(good[n] & v_ok, 1, 0))

    def attention_safe(i, ow):
        r0 = _mo(i * QB, QB)
        start = pl.multiple_of(jnp.maximum(i - 2, 0) * QB, QB)
        qw = qt_b.at[:, pl.ds(r0, QB)]
        kw = k_b.at[pl.ds(start, 3 * QB), :]
        vw = vt_b.at[:, pl.ds(start, 3 * QB)]
        key = lax.broadcasted_iota(I32, (3 * QB, QB), 0) + start
        qry = lax.broadcasted_iota(I32, (3 * QB, QB), 1) + r0
        valid = (qry - key >= 0) & (qry - key < WIN)
        drow = lax.broadcasted_iota(I32, (128, QB), 0)

        def head(h, carry):
            g0 = pl.multiple_of((h // 4) * 128, 128)
            j0 = (h % 4) * 32
            q4 = qw[pl.ds(g0, 128), :].astype(F32)
            w = jnp.where((drow >= j0) & (drow < j0 + 32), q4, 0.0).astype(BF16)
            s = jnp.dot(kw[:, pl.ds(g0, 128)], w, preferred_element_type=F32)
            s = jnp.where(valid, s, NEG)
            m = jnp.max(s, axis=0, keepdims=True)
            p = jnp.exp2(s - m).astype(BF16)
            l = jnp.sum(p.astype(F32), axis=0, keepdims=True)
            vt = vw[pl.ds(pl.multiple_of(h * 32, 32), 32), :]
            o = jnp.dot(vt, p, preferred_element_type=F32) * (1.0 / l)
            ow[pl.ds(pl.multiple_of((h % 16) * 32, 32), 32),
               pl.ds(pl.multiple_of((h // 16) * 128, 128), 128)] = o.astype(BF16)
            return carry

        lax.fori_loop(0, NH, head, 0)

    def out_proj(n, xsrc, x1dst, z=0):
        ow = ot_b.at[n + z]
        o = jnp.concatenate([ow[:, 0:128], ow[:, 128:256]], axis=0)
        y = lax.dot_general(o, wo[...], TN, preferred_element_type=F32)
        x1dst[...] = (xsrc[...].astype(F32) + y).astype(BF16)

    def ln2(b, x1src, x2dst, CH=16, NCHAIN=8, z_in=0):
        rb = _mo(b * QB, QB)
        wr = wr_ref[...].astype(F32).reshape(1, D)
        wsum = jnp.sum(wr, axis=-1, keepdims=True)
        bm = None
        bi = None
        sub = lax.broadcasted_iota(I32, (8, 1), 0)
        toks = []
        for c in range(QB // CH):
            z = toks[c - NCHAIN] if c >= NCHAIN else z_in
            if isinstance(z, int):
                x1 = x1src[CH * c:CH * (c + 1), :].astype(F32)
            else:
                x1 = x1src[pl.ds(pl.multiple_of(CH * c + z * 16, 16), CH), :].astype(F32)
            m, rs = _ln_stats(x1)
            x2dst[CH * c:CH * (c + 1), :] = (x1 * (1.0 + rs) - m * rs).astype(BF16)
            r = _rnd(rs * (jnp.sum(x1 * wr, axis=-1, keepdims=True) - m * wsum))
            ru = lax.bitcast_convert_type(r, I32)
            toks.append(jnp.max(lax.shift_right_logical(lax.shift_right_logical(ru, 16), 16)))
            for t in range(CH // 8):
                rt = r[8 * t:8 * t + 8]
                it = sub + (rb + CH * c + 8 * t)
                if bm is None:
                    bm, bi = rt, it
                else:
                    better = rt > bm
                    bm = jnp.where(better, rt, bm)
                    bi = jnp.where(better, it, bi)
        bmax_ref[b] = jnp.broadcast_to(bm, (8, 128))
        bidx_ref[b] = jnp.broadcast_to(bi, (8, 128))
        tok = toks[-1]
        for k in range(2, min(NCHAIN, len(toks)) + 1):
            tok = tok + toks[-k]
        return tok

    def checks(i0):
        def one(n, carry):
            @pl.when(flag[n] == 0)
            def _():
                rb = pl.multiple_of((i0 + n) * QB, QB)
                attention_safe(i0 + n, ot_b.at[n])
                out_proj(n, xn.at[pl.ds(rb, QB), :], x1_b.at[pl.ds(rb, QB), :])
            return carry

        @pl.when(flag[0] + flag[1] < 2)
        def _():
            lax.fori_loop(0, 2, one, 0)

    def out_copy(b):
        return pltpu.make_async_copy(xn.at[pl.ds(b * QB, QB), :],
                                     out_hbm.at[pl.ds(b * QB, QB), :], sem_o.at[0])

    def phase_b(layer):
        attention([(0, 1), (1, 2)])
        out_proj(0, xn.at[0:QB, :], x1_b.at[0:QB, :])
        out_proj(1, xn.at[QB:2 * QB, :], x1_b.at[QB:2 * QB, :])

        def body(t, carry):
            i0 = 2 * t
            checks(i0 - 2)

            @pl.when(jnp.logical_and(layer == 1, t >= 2))
            def _():
                out_copy(i0 - 4).start()
                out_copy(i0 - 3).start()

            @pl.when(t < NQB // 2)
            def _():
                r2 = pl.multiple_of((i0 - 2) * QB, QB)
                xv = xn.at[pl.ds(r2, 4 * QB), :]
                x1v = x1_b.at[pl.ds(r2, 4 * QB), :]
                ln2(i0 - 2, x1v.at[0:QB, :], xv.at[0:QB, :])
                ln2(i0 - 1, x1v.at[QB:2 * QB, :], xv.at[QB:2 * QB, :])
                attention([(i0, 3), (i0 + 1, 3)])
                out_proj(0, xv.at[2 * QB:3 * QB, :], x1v.at[2 * QB:3 * QB, :])
                out_proj(1, xv.at[3 * QB:4 * QB, :], x1v.at[3 * QB:4 * QB, :])
            return carry

        lax.fori_loop(1, NQB // 2 + 1, body, 0)
        for b in (NQB - 2, NQB - 1):
            ln2(b, x1_b.at[b * QB:(b + 1) * QB, :], xn.at[b * QB:(b + 1) * QB, :], NCHAIN=8)

        @pl.when(layer == 1)
        def _():
            out_copy(NQB - 2).start()
            out_copy(NQB - 1).start()

    def moe(layer):
        rm = bmax_ref[:, :, 0:1]
        ri = bidx_ref[:, :, 0:1]
        gm = jnp.max(jnp.max(rm, axis=0), axis=0, keepdims=True)
        idx = jnp.min(jnp.where(rm == gm, ri, BIG))
        b16 = pl.multiple_of((idx // 16) * 16, 16)
        ln1(0, hbufs[0])
        x1c = x1_b[pl.ds(b16, 16), :].astype(F32)
        h2c = _rnd(_ln(x1c))
        hb = h2c.astype(BF16)
        g = _rnd(jnp.dot(hb, wg[...], preferred_element_type=F32))
        u = _rnd(jnp.dot(hb, wu[...], preferred_element_type=F32))
        g = _rnd(g * _rnd(jax.nn.sigmoid(g)))
        act = (g * u).astype(BF16)
        y = _rnd(jnp.dot(act, wd[...], preferred_element_type=F32))
        y = _rnd(y * _rnd(jax.nn.sigmoid(gm)))
        x2n = x1c + _rnd(h2c + y)

        @pl.when(layer == 1)
        def _():
            for b in range(NQB):
                out_copy(b).wait()

        cur = xn[pl.ds(b16, 16), :].astype(F32)
        sel = lax.broadcasted_iota(I32, (16, D), 0) == (idx - b16)
        xn[pl.ds(b16, 16), :] = jnp.where(sel, x2n, cur).astype(BF16)

        @pl.when(jnp.logical_and(layer == 0, idx < MB))
        def _():
            ln1(0, hbufs[0])

        @pl.when(layer == 1)
        def _():
            cp = pltpu.make_async_copy(xn.at[pl.ds(b16, 16), :],
                                       out_hbm.at[pl.ds(b16, 16), :], sem_o.at[1])
            cp.start()
            cp.wait()

    def layer_body(layer, carry):
        phase_a(layer)

        @pl.when(layer == 0)
        def _():
            w_copies[0].wait()

        phase_b(layer)

        @pl.when(layer == 0)
        def _():
            for c in w_copies[1:]:
                c.wait()

        moe(layer)

        vmax_ref[...] = jnp.zeros((8, 128), F32)
        return carry

    lax.fori_loop(0, 2, layer_body, 0)


@jax.jit
def pallas_interleave_layers__sliding_block__moe_arch_mod__prompt_kernel(
    A_x: jax.Array,
    A_wqkv: jax.Array,
    A_wo: jax.Array,
    B_x: jax.Array,
    B_w_r: jax.Array,
    B_w_gate: jax.Array,
    B_w_up: jax.Array,
    B_w_down: jax.Array,
):
    del B_x
    hbm = pl.BlockSpec(memory_space=pl.ANY)
    scratch = [
        pltpu.VMEM((S // 2, D), U32),
        pltpu.VMEM((S // 2, D), U32),
        pltpu.VMEM((MB // 2, D), U32),
        pltpu.VMEM((MB // 2, D), U32),
        pltpu.VMEM((D // 2, S), U32),
        pltpu.VMEM((S // 2, D), U32),
        pltpu.VMEM((D // 2, S), U32),
        pltpu.VMEM((D // 2, 3 * D), U32),
        pltpu.VMEM((D, D), U32),
        pltpu.VMEM((D // 2, D), U32),
        pltpu.VMEM((D // 2, FF), U32),
        pltpu.VMEM((D // 2, FF), U32),
        pltpu.VMEM((FF // 2, D), U32),
        pltpu.VMEM((1, 128, 512), U32),
        pltpu.VMEM((1, 128, 512), U32),
        pltpu.VMEM((1, 128, 512), U32),
        pltpu.VMEM((2, 256, 256), U32),
        pltpu.VMEM((8, 128), F32),
        pltpu.VMEM((NQB, 8, 128), F32),
        pltpu.VMEM((NQB, 8, 128), I32),
        pltpu.SMEM((8,), I32),
        pltpu.SMEM((2,), I32),
        pltpu.SemaphoreType.DMA((NMB,)),
        pltpu.SemaphoreType.DMA((9,)),
        pltpu.SemaphoreType.DMA((2,)),
    ]
    out = pl.pallas_call(
        _kernel,
        out_shape=jax.ShapeDtypeStruct((S, D), BF16),
        in_specs=[hbm, hbm, hbm, pl.BlockSpec(memory_space=pltpu.VMEM), hbm, hbm, hbm],
        out_specs=hbm,
        scratch_shapes=scratch,
        compiler_params=pltpu.CompilerParams(vmem_limit_bytes=110 * 1024 * 1024),
        name="swa_moe_fused",
    )(A_x.reshape(S, D), A_wqkv, A_wo, B_w_r, B_w_gate, B_w_up, B_w_down)
    return out.reshape(1, S, D)
```

```python
import math

import jax
import jax.numpy as jnp
from jax import lax
import jax.experimental.pallas as pl
import jax.experimental.pallas.tpu as pltpu

S = 2048
D = 1024
NH = 32
DH = 32
WIN = 256
FF = 3584
QB = 128
NQB = S // QB
MB = 256
NMB = S // MB
EPS = 1e-5
QSCALE = (DH ** -0.5) * math.log2(math.e)
NEG = -1e30
BIG = 2 ** 30
L_LO = 2.0 ** -64
L_HI = 2.0 ** 64
V_HI = 2.0 ** 60

F32 = jnp.float32
BF16 = jnp.bfloat16
U32 = jnp.uint32
I32 = jnp.int32

NT = (((1,), (1,)), ((), ()))
TN = (((0,), (0,)), ((), ()))


def _rnd(v):
    return v.astype(BF16).astype(F32)


def _ln(xf):
    m = jnp.mean(xf, axis=-1, keepdims=True)
    xc = xf - m
    v = jnp.mean(xc * xc, axis=-1, keepdims=True)
    return xc * lax.rsqrt(v + EPS)


def _ln_stats(xf):
    m = jnp.sum(xf, axis=-1, keepdims=True) * (1.0 / D)
    v = jnp.sum(xf * xf, axis=-1, keepdims=True) * (1.0 / D) - m * m
    return m, lax.rsqrt(jnp.maximum(v, 0.0) + EPS)


def _recip(l):
    r = pl.reciprocal(l, approx=True)
    return r * (2.0 - l * r)


def _mo(v, m):
    return v if isinstance(v, int) else pl.multiple_of(v, m)


def _kernel(x_hbm, wqkv_hbm, wo_hbm, wr_ref, wg_hbm, wu_hbm, wd_hbm, out_hbm,
            xn_u, x1_u, h0_u, h1_u, qt_u, k_u, vt_u,
            wqkv_u, wqvt_u, wo_u, wg_u, wu_u, wd_u,
            p0, p1, p2, ot_u, vmax_ref, bmax_ref, bidx_ref, zs, flag,
            sem_x, sem_w, sem_o):
    xn = xn_u.bitcast(BF16)
    x1_b = x1_u.bitcast(BF16)
    hbufs = (h0_u.bitcast(BF16), h1_u.bitcast(BF16))
    qt_b = qt_u.bitcast(BF16)
    k_b = k_u.bitcast(BF16)
    vt_b = vt_u.bitcast(BF16)
    wqkv = wqkv_u.bitcast(BF16)
    wqvt = wqvt_u.bitcast(BF16)
    wo = wo_u.bitcast(BF16)
    wg = wg_u.bitcast(BF16)
    wu = wu_u.bitcast(BF16)
    wd = wd_u.bitcast(BF16)
    ot_b = ot_u.bitcast(BF16)
    otbufs = (ot_b.at[0], ot_b.at[1])
    pbufs_u = (p0, p1, p2)
    pbufs_b = tuple(p.bitcast(BF16) for p in pbufs_u)

    def x_copy(j):
        return pltpu.make_async_copy(x_hbm.at[pl.ds(j * MB, MB), :],
                                     xn.at[pl.ds(j * MB, MB), :], sem_x.at[j])

    def wqkv_copy(c0, n, k):
        return pltpu.make_async_copy(wqkv_hbm.at[:, pl.ds(c0, n)],
                                     wqkv.at[:, pl.ds(c0, n)], sem_w.at[k])

    HD = D // 2
    wq_copies = [wqkv_copy(0, HD, 0), wqkv_copy(HD, HD, 1)]
    wv_copies = [wqkv_copy(2 * D, HD, 2), wqkv_copy(2 * D + HD, HD, 7)]
    wk_copy = wqkv_copy(D, D, 8)

    w_copies = [
        pltpu.make_async_copy(wo_hbm, wo, sem_w.at[3]),
        pltpu.make_async_copy(wg_hbm, wg, sem_w.at[4]),
        pltpu.make_async_copy(wu_hbm, wu, sem_w.at[5]),
        pltpu.make_async_copy(wd_hbm, wd, sem_w.at[6]),
    ]
    x_copy(0).start()
    wq_copies[0].start()
    wq_copies[1].start()
    wv_copies[0].start()
    wv_copies[1].start()
    x_copy(1).start()
    x_copy(2).start()
    wk_copy.start()

    for t in range(5):
        zs[t] = 0
    vmax_ref[...] = jnp.zeros((8, 128), F32)

    eye = (lax.broadcasted_iota(I32, (128, 128), 0)
           == lax.broadcasted_iota(I32, (128, 128), 1)).astype(F32).astype(BF16)

    def transpose_w(src_col0, dst_row0, tiles):
        for t in tiles:
            w_t = wqkv[:, src_col0 + 128 * t:src_col0 + 128 * (t + 1)]
            wqvt[dst_row0 + 128 * t:dst_row0 + 128 * (t + 1), :] = lax.dot_general(
                eye, w_t, NT, preferred_element_type=F32).astype(BF16)

    def ln1(row0, dst):
        src = xn.at[pl.ds(row0, MB), :]
        for c in range(MB // 64):
            xf = src[64 * c:64 * (c + 1), :].astype(F32)
            dst[64 * c:64 * (c + 1), :] = _ln(xf).astype(BF16)

    def track_v(v):
        a = jnp.max(jnp.abs(v).reshape(v.shape[0] // 8, 8, v.shape[1]), axis=0)
        a = jnp.maximum(a[:, 0:128], a[:, 128:256])
        a = jnp.broadcast_to(jnp.max(a, axis=0, keepdims=True), (8, 128))
        vmax_ref[...] = jnp.maximum(vmax_ref[...], a)

    def proj_t(row0, n, base, hsrc):
        r = lax.dot_general(wqvt[row0:row0 + n, :], hsrc[...], NT, preferred_element_type=F32)
        if row0 < D:
            qt_b[row0:row0 + n, pl.ds(base, MB)] = (r * QSCALE).astype(BF16)
        else:
            vt_b[row0 - D:row0 - D + n, pl.ds(base, MB)] = r.astype(BF16)
            track_v(r)

    def proj_qv(base, hsrc):
        qv = lax.dot_general(wqvt[...], hsrc[...], NT, preferred_element_type=F32)
        qt_b[:, pl.ds(base, MB)] = (qv[0:D] * QSCALE).astype(BF16)
        vt_b[:, pl.ds(base, MB)] = qv[D:2 * D].astype(BF16)
        track_v(qv[D:2 * D])

    def proj_k(base, hsrc):
        k = jnp.dot(hsrc[...], wqkv[:, D:2 * D], preferred_element_type=F32)
        k_b[pl.ds(base, MB), :] = k.astype(BF16)

    def phase_a(layer):
        def body(t, carry):
            first = jnp.logical_and(layer == 0, t == 0)

            @pl.when(first)
            def _():
                x_copy(1).wait()
                x_copy(2).wait()
                wk_copy.wait()
                for j in range(3, NMB):
                    x_copy(j).start()
                for c in w_copies:
                    c.start()

            @pl.when(jnp.logical_and(layer == 0, t >= 1))
            def _():
                x_copy(2 * t + 1).wait()

            @pl.when(jnp.logical_and(layer == 0, jnp.logical_and(t >= 1, t < NMB // 2 - 1)))
            def _():
                x_copy(2 * t + 2).wait()

            b0 = pl.multiple_of(2 * t * MB, MB)
            b1 = pl.multiple_of(b0 + MB, MB)
            b2 = pl.multiple_of(jnp.minimum(2 * t + 2, NMB - 1) * MB, MB)

            @pl.when(jnp.logical_not(first))
            def _():
                proj_qv(b0, hbufs[0])

            proj_k(b0, hbufs[0])
            ln1(b1, hbufs[1])
            proj_qv(b1, hbufs[1])
            proj_k(b1, hbufs[1])
            ln1(b2, hbufs[0])
            return carry

        lax.fori_loop(0, NMB // 2, body, 0)

    x_copy(0).wait()
    ln1(0, hbufs[0])
    for k in range(2):
        wq_copies[k].wait()
        transpose_w(k * HD, k * HD, range(4))
        proj_t(k * HD, HD, 0, hbufs[0])
    for k in range(2):
        wv_copies[k].wait()
        transpose_w(2 * D + k * HD, D + k * HD, range(4))
        proj_t(D + k * HD, HD, 0, hbufs[0])

    def attention(blocks):
        p_st = [p.at[zs[0]] for p in pbufs_b]
        good = [None] * len(blocks)
        lsums = {}
        views = []
        for (i, nkb) in blocks:
            r0 = _mo(i * QB, QB)
            k0 = 128 * (nkb - 1)
            views.append((qt_b.at[:, pl.ds(r0, QB)],
                          k_b.at[pl.ds(r0 - k0, k0 + QB), :],
                          vt_b.at[:, pl.ds(r0 - k0, k0 + QB)]))

        lane8 = lax.broadcasted_iota(I32, (1, 8, QB), 2)
        bit0z = (lane8 & 32) == 0
        bit1z = (lane8 & 64) == 0
        blk8 = lane8 >> 5
        t32 = lax.broadcasted_iota(I32, (32, QB), 0)
        new32 = t32 <= (lax.broadcasted_iota(I32, (32, QB), 1) & 31)
        r16 = lax.broadcasted_iota(I32, (16, QB), 0) * 2
        c16 = lax.broadcasted_iota(I32, (16, QB), 1) & 31
        pn32 = (jnp.where(r16 <= c16, U32(0xFFFF), U32(0))
                | jnp.where(r16 + 1 <= c16, U32(0xFFFF0000), U32(0)))

        def lsel(mask, x, y):
            if x is None and y is None:
                return None
            ref = x if y is None else y
            shp = ref.shape
            zero = jnp.zeros((), ref.dtype)
            if shp[0] % 8 == 0:
                x3 = zero if x is None else x.reshape(shp[0] // 8, 8, QB)
                y3 = zero if y is None else y.reshape(shp[0] // 8, 8, QB)
                return jnp.where(mask, x3, y3).reshape(shp)
            return jnp.where(mask[0, 0:shp[0]], zero if x is None else x, zero if y is None else y)

        def xperm(x, j):
            if j & 1:
                x = lsel(bit0z, pltpu.roll(x, 96, 1), pltpu.roll(x, 32, 1))
            if j & 2:
                x = pltpu.roll(x, 64, 1)
            return x

        def pick(a, j):
            return lsel(bit1z, lsel(bit0z, a[j], a[j ^ 1]), lsel(bit0z, a[j ^ 2], a[j ^ 3]))

        def qk(n, g, slot):
            nkb = blocks[n][1]
            qw, kw, _ = views[n]
            cs = slice(128 * g, 128 * (g + 1))
            pref = p_st[slot]
            ys = [xperm(pltpu.bitcast(qw[32 * (4 * g + j):32 * (4 * g + j) + 32, :], U32), j)
                  for j in range(4)]
            for u in (range(4) if nkb == 3 else [(g + k) % 4 for k in range(4)]):
                w = pltpu.bitcast(jnp.concatenate(
                    [lsel(blk8 == (j ^ u), ys[j], None) for j in range(4)], axis=0), BF16)
                dg = 128 * (nkb - 1) + 32 * u
                parts = []
                if nkb == 3:
                    for c in range(2):
                        parts.append(kw[32 * u + 16 * c:32 * u + 16 * c + 16, cs])
                        parts.append(kw[dg + 16 * c:dg + 16 * c + 16, cs])
                    parts.append(kw[32 * u + 32:dg, cs])
                    nmid = 7
                else:
                    parts.append(kw[dg:dg + 32, cs])
                    if dg > 0:
                        parts.append(kw[0:dg, cs])
                    nmid = dg // 32
                s = jnp.dot(jnp.concatenate(parts, axis=0), w, preferred_element_type=F32)
                ls = slice(128 * u, 128 * (u + 1))
                acc = [None, None]

                def put(row0, e, k):
                    pref[row0:row0 + 16, ls] = e.astype(BF16)
                    acc[k] = e if acc[k] is None else acc[k] + e

                for c in range(2):
                    if nkb == 3:
                        f = jnp.where(new32[16 * c:16 * c + 16], s[32 * c + 16:32 * c + 32],
                                      s[32 * c:32 * c + 16])
                    else:
                        f = jnp.where(new32[16 * c:16 * c + 16], s[16 * c:16 * c + 16], NEG)
                    put(16 * c, jnp.exp2(f), c % 2)
                m0 = 64 if nkb == 3 else 32
                for c in range(2 * nmid):
                    put(32 + 16 * c, jnp.exp2(s[m0 + 16 * c:m0 + 16 * c + 16]), c % 2)
                t = acc[0] + acc[1]
                lsums[(slot, u)] = jnp.sum(t[0:8] + t[8:16], axis=0, keepdims=True)

        def pv(n, g, slot):
            nkb = blocks[n][1]
            vw = views[n][2]
            ots = []
            for j in range(4):
                pref = pbufs_u[slot].at[zs[1 + j]]

                def blk(u, b):
                    ls = slice(128 * u, 128 * (u + 1))
                    if nkb == 3:
                        be = b - u
                        if be < 0 or be > 8:
                            return None
                        if be == 0:
                            f = pref[0:16, ls]
                            return f ^ (f & pn32)
                        if be == 8:
                            return pref[0:16, ls] & pn32
                        return pref[16 * be:16 * be + 16, ls]
                    nb = 4 * (nkb - 1) + u
                    if b > nb:
                        return None
                    if b == nb:
                        return pref[0:16, ls]
                    return pref[16 * (b + 1):16 * (b + 2), ls]

                tiles = []
                for b in range(4 * nkb):
                    o = pick([blk(u, b) for u in range(4)], j)
                    tiles.append(jnp.zeros((16, QB), U32) if o is None else o)
                ots.append(jnp.dot(vw[32 * (4 * g + j):32 * (4 * g + j + 1), :],
                                   pltpu.bitcast(jnp.concatenate(tiles, axis=0), BF16),
                                   preferred_element_type=F32))
            lu = [lsums.pop((slot, u)) for u in range(4)]
            for j in range(4):
                h = 4 * g + j
                l = pick(lu, j)
                ok = (l >= L_LO) & (l <= L_HI)
                good[n] = ok if good[n] is None else (good[n] & ok)
                o = xperm(ots[j] * _recip(l), j)
                otbufs[n][32 * (h % 16):32 * (h % 16) + 32,
                          128 * (h // 16):128 * (h // 16) + 128] = o.astype(BF16)

        seq = [(n, g) for n in range(len(blocks)) for g in range(8)]
        for s in range(len(seq) + 2):
            if s < len(seq):
                qk(seq[s][0], seq[s][1], s % 3)
            if s >= 2:
                pv(seq[s - 2][0], seq[s - 2][1], (s - 2) % 3)
        v_ok = vmax_ref[0:1, :] <= V_HI
        for n in range(len(blocks)):
            flag[n] = jnp.min(jnp.where(good[n] & v_ok, 1, 0))

    def attention_safe(i, ow):
        r0 = _mo(i * QB, QB)
        start = pl.multiple_of(jnp.maximum(i - 2, 0) * QB, QB)
        qw = qt_b.at[:, pl.ds(r0, QB)]
        kw = k_b.at[pl.ds(start, 3 * QB), :]
        vw = vt_b.at[:, pl.ds(start, 3 * QB)]
        key = lax.broadcasted_iota(I32, (3 * QB, QB), 0) + start
        qry = lax.broadcasted_iota(I32, (3 * QB, QB), 1) + r0
        valid = (qry - key >= 0) & (qry - key < WIN)
        drow = lax.broadcasted_iota(I32, (128, QB), 0)

        def head(h, carry):
            g0 = pl.multiple_of((h // 4) * 128, 128)
            j0 = (h % 4) * 32
            q4 = qw[pl.ds(g0, 128), :].astype(F32)
            w = jnp.where((drow >= j0) & (drow < j0 + 32), q4, 0.0).astype(BF16)
            s = jnp.dot(kw[:, pl.ds(g0, 128)], w, preferred_element_type=F32)
            s = jnp.where(valid, s, NEG)
            m = jnp.max(s, axis=0, keepdims=True)
            p = jnp.exp2(s - m).astype(BF16)
            l = jnp.sum(p.astype(F32), axis=0, keepdims=True)
            vt = vw[pl.ds(pl.multiple_of(h * 32, 32), 32), :]
            o = jnp.dot(vt, p, preferred_element_type=F32) * (1.0 / l)
            ow[pl.ds(pl.multiple_of((h % 16) * 32, 32), 32),
               pl.ds(pl.multiple_of((h // 16) * 128, 128), 128)] = o.astype(BF16)
            return carry

        lax.fori_loop(0, NH, head, 0)

    def out_proj(n, xsrc, x1dst):
        ow = ot_b.at[n]
        o = jnp.concatenate([ow[:, 0:128], ow[:, 128:256]], axis=0)
        y = lax.dot_general(o, wo[...], TN, preferred_element_type=F32)
        x1dst[...] = (xsrc[...].astype(F32) + y).astype(BF16)

    def ln2(b, x1src, x2dst):
        CH = 16
        rb = _mo(b * QB, QB)
        wr = wr_ref[...].astype(F32).reshape(1, D)
        wsum = jnp.sum(wr, axis=-1, keepdims=True)
        bm = None
        bi = None
        sub = lax.broadcasted_iota(I32, (8, 1), 0)
        for c in range(QB // CH):
            x1 = x1src[CH * c:CH * (c + 1), :].astype(F32)
            m, rs = _ln_stats(x1)
            x2dst[CH * c:CH * (c + 1), :] = (x1 * (1.0 + rs) - m * rs).astype(BF16)
            r = _rnd(rs * (jnp.sum(x1 * wr, axis=-1, keepdims=True) - m * wsum))
            for t in range(CH // 8):
                rt = r[8 * t:8 * t + 8]
                it = sub + (rb + CH * c + 8 * t)
                if bm is None:
                    bm, bi = rt, it
                else:
                    better = rt > bm
                    bm = jnp.where(better, rt, bm)
                    bi = jnp.where(better, it, bi)
        bmax_ref[b] = jnp.broadcast_to(bm, (8, 128))
        bidx_ref[b] = jnp.broadcast_to(bi, (8, 128))

    def checks(i0):
        def one(n, carry):
            @pl.when(flag[n] == 0)
            def _():
                rb = pl.multiple_of((i0 + n) * QB, QB)
                attention_safe(i0 + n, ot_b.at[n])
                out_proj(n, xn.at[pl.ds(rb, QB), :], x1_b.at[pl.ds(rb, QB), :])
            return carry

        @pl.when(flag[0] + flag[1] < 2)
        def _():
            lax.fori_loop(0, 2, one, 0)

    def out_copy(b):
        return pltpu.make_async_copy(xn.at[pl.ds(b * QB, QB), :],
                                     out_hbm.at[pl.ds(b * QB, QB), :], sem_o.at[0])

    def phase_b(layer):
        attention([(0, 1), (1, 2)])
        out_proj(0, xn.at[0:QB, :], x1_b.at[0:QB, :])
        out_proj(1, xn.at[QB:2 * QB, :], x1_b.at[QB:2 * QB, :])

        def body(t, carry):
            i0 = 2 * t
            checks(i0 - 2)

            @pl.when(jnp.logical_and(layer == 1, t >= 2))
            def _():
                out_copy(i0 - 4).start()
                out_copy(i0 - 3).start()

            @pl.when(t < NQB // 2)
            def _():
                r2 = pl.multiple_of((i0 - 2) * QB, QB)
                xv = xn.at[pl.ds(r2, 4 * QB), :]
                x1v = x1_b.at[pl.ds(r2, 4 * QB), :]
                ln2(i0 - 2, x1v.at[0:QB, :], xv.at[0:QB, :])
                ln2(i0 - 1, x1v.at[QB:2 * QB, :], xv.at[QB:2 * QB, :])
                attention([(i0, 3), (i0 + 1, 3)])
                out_proj(0, xv.at[2 * QB:3 * QB, :], x1v.at[2 * QB:3 * QB, :])
                out_proj(1, xv.at[3 * QB:4 * QB, :], x1v.at[3 * QB:4 * QB, :])
            return carry

        lax.fori_loop(1, NQB // 2 + 1, body, 0)
        for b in (NQB - 2, NQB - 1):
            ln2(b, x1_b.at[b * QB:(b + 1) * QB, :], xn.at[b * QB:(b + 1) * QB, :])

        @pl.when(layer == 1)
        def _():
            out_copy(NQB - 2).start()
            out_copy(NQB - 1).start()

    def moe(layer):
        rm = bmax_ref[:, :, 0:1]
        ri = bidx_ref[:, :, 0:1]
        gm = jnp.max(jnp.max(rm, axis=0), axis=0, keepdims=True)
        idx = jnp.min(jnp.where(rm == gm, ri, BIG))
        b16 = pl.multiple_of((idx // 16) * 16, 16)
        ln1(0, hbufs[0])
        x1c = x1_b[pl.ds(b16, 16), :].astype(F32)
        mu, rs = _ln_stats(x1c)
        h2c = _rnd(x1c * rs - mu * rs)
        hb = h2c.astype(BF16)
        g = _rnd(jnp.dot(hb, wg[...], preferred_element_type=F32))
        u = _rnd(jnp.dot(hb, wu[...], preferred_element_type=F32))
        g = _rnd(g * _rnd(jax.nn.sigmoid(g)))
        act = (g * u).astype(BF16)
        y = _rnd(jnp.dot(act, wd[...], preferred_element_type=F32))
        y = _rnd(y * _rnd(jax.nn.sigmoid(gm)))
        x2n = x1c + _rnd(h2c + y)

        @pl.when(layer == 1)
        def _():
            for b in range(NQB):
                out_copy(b).wait()

        cur = xn[pl.ds(b16, 16), :].astype(F32)
        sel = lax.broadcasted_iota(I32, (16, D), 0) == (idx - b16)
        xn[pl.ds(b16, 16), :] = jnp.where(sel, x2n, cur).astype(BF16)

        @pl.when(jnp.logical_and(layer == 0, idx < MB))
        def _():
            ln1(0, hbufs[0])

        @pl.when(layer == 1)
        def _():
            cp = pltpu.make_async_copy(xn.at[pl.ds(b16, 16), :],
                                       out_hbm.at[pl.ds(b16, 16), :], sem_o.at[1])
            cp.start()
            cp.wait()

    def layer_body(layer, carry):
        phase_a(layer)

        @pl.when(layer == 0)
        def _():
            w_copies[0].wait()

        phase_b(layer)

        @pl.when(layer == 0)
        def _():
            for c in w_copies[1:]:
                c.wait()

        moe(layer)

        vmax_ref[...] = jnp.zeros((8, 128), F32)
        return carry

    lax.fori_loop(0, 2, layer_body, 0)


@jax.jit
def pallas_interleave_layers__sliding_block__moe_arch_mod__prompt_kernel(
    A_x: jax.Array,
    A_wqkv: jax.Array,
    A_wo: jax.Array,
    B_x: jax.Array,
    B_w_r: jax.Array,
    B_w_gate: jax.Array,
    B_w_up: jax.Array,
    B_w_down: jax.Array,
):
    del B_x
    hbm = pl.BlockSpec(memory_space=pl.ANY)
    scratch = [
        pltpu.VMEM((S // 2, D), U32),
        pltpu.VMEM((S // 2, D), U32),
        pltpu.VMEM((MB // 2, D), U32),
        pltpu.VMEM((MB // 2, D), U32),
        pltpu.VMEM((D // 2, S), U32),
        pltpu.VMEM((S // 2, D), U32),
        pltpu.VMEM((D // 2, S), U32),
        pltpu.VMEM((D // 2, 3 * D), U32),
        pltpu.VMEM((D, D), U32),
        pltpu.VMEM((D // 2, D), U32),
        pltpu.VMEM((D // 2, FF), U32),
        pltpu.VMEM((D // 2, FF), U32),
        pltpu.VMEM((FF // 2, D), U32),
        pltpu.VMEM((1, 128, 512), U32),
        pltpu.VMEM((1, 128, 512), U32),
        pltpu.VMEM((1, 128, 512), U32),
        pltpu.VMEM((2, 256, 256), U32),
        pltpu.VMEM((8, 128), F32),
        pltpu.VMEM((NQB, 8, 128), F32),
        pltpu.VMEM((NQB, 8, 128), I32),
        pltpu.SMEM((5,), I32),
        pltpu.SMEM((2,), I32),
        pltpu.SemaphoreType.DMA((NMB,)),
        pltpu.SemaphoreType.DMA((9,)),
        pltpu.SemaphoreType.DMA((2,)),
    ]
    out = pl.pallas_call(
        _kernel,
        out_shape=jax.ShapeDtypeStruct((S, D), BF16),
        in_specs=[hbm, hbm, hbm, pl.BlockSpec(memory_space=pltpu.VMEM), hbm, hbm, hbm],
        out_specs=hbm,
        scratch_shapes=scratch,
        compiler_params=pltpu.CompilerParams(vmem_limit_bytes=110 * 1024 * 1024,
                                             disable_bounds_checks=True,
                                             disable_semaphore_checks=True),
        name="swa_moe_fused",
    )(A_x.reshape(S, D), A_wqkv, A_wo, B_w_r, B_w_gate, B_w_up, B_w_down)
    return out.reshape(1, S, D)
```

```python
import math

import jax
import jax.numpy as jnp
from jax import lax
import jax.experimental.pallas as pl
import jax.experimental.pallas.tpu as pltpu

S = 2048
D = 1024
NH = 32
DH = 32
WIN = 256
FF = 3584
QB = 128
NQB = S // QB
MB = 256
NMB = S // MB
EPS = 1e-5
QSCALE = (DH ** -0.5) * math.log2(math.e)
NEG = -1e30
BIG = 2 ** 30
L_LO = 2.0 ** -64
L_HI = 2.0 ** 64
V_HI = 2.0 ** 60

F32 = jnp.float32
BF16 = jnp.bfloat16
U32 = jnp.uint32
I32 = jnp.int32

NT = (((1,), (1,)), ((), ()))
TN = (((0,), (0,)), ((), ()))


def _rnd(v):
    return v.astype(BF16).astype(F32)


def _ln(xf):
    m = jnp.mean(xf, axis=-1, keepdims=True)
    xc = xf - m
    v = jnp.mean(xc * xc, axis=-1, keepdims=True)
    return xc * lax.rsqrt(v + EPS)


def _ln_stats(xf):
    m = jnp.sum(xf, axis=-1, keepdims=True) * (1.0 / D)
    v = jnp.sum(xf * xf, axis=-1, keepdims=True) * (1.0 / D) - m * m
    return m, lax.rsqrt(jnp.maximum(v, 0.0) + EPS)


def _recip(l):
    r = pl.reciprocal(l, approx=True)
    return r * (2.0 - l * r)


def _mo(v, m):
    return v if isinstance(v, int) else pl.multiple_of(v, m)


def _kernel(x_hbm, wqkv_hbm, wo_hbm, wr_ref, wg_hbm, wu_hbm, wd_hbm, out_hbm,
            xn_u, x1_u, h0_u, h1_u, qt_u, k_u, vt_u,
            wqkv_u, wqvt_u, wo_u, wg_u, wu_u, wd_u,
            p0, p1, p2, ot_u, vmax_ref, bmax_ref, bidx_ref, zs, flag,
            sem_x, sem_w, sem_o):
    xn = xn_u.bitcast(BF16)
    x1_b = x1_u.bitcast(BF16)
    hbufs = (h0_u.bitcast(BF16), h1_u.bitcast(BF16))
    qt_b = qt_u.bitcast(BF16)
    k_b = k_u.bitcast(BF16)
    vt_b = vt_u.bitcast(BF16)
    wqkv = wqkv_u.bitcast(BF16)
    wqvt = wqvt_u.bitcast(BF16)
    wo = wo_u.bitcast(BF16)
    wg = wg_u.bitcast(BF16)
    wu = wu_u.bitcast(BF16)
    wd = wd_u.bitcast(BF16)
    ot_b = ot_u.bitcast(BF16)
    otbufs = (ot_b.at[0], ot_b.at[1])
    pbufs_u = (p0, p1, p2)
    pbufs_b = tuple(p.bitcast(BF16) for p in pbufs_u)

    def x_copy(j):
        return pltpu.make_async_copy(x_hbm.at[pl.ds(j * MB, MB), :],
                                     xn.at[pl.ds(j * MB, MB), :], sem_x.at[j])

    def wqkv_copy(c0, n, k):
        return pltpu.make_async_copy(wqkv_hbm.at[:, pl.ds(c0, n)],
                                     wqkv.at[:, pl.ds(c0, n)], sem_w.at[k])

    HD = D // 2
    wq_copies = [wqkv_copy(0, HD, 0), wqkv_copy(HD, HD, 1)]
    wv_copies = [wqkv_copy(2 * D, HD, 2), wqkv_copy(2 * D + HD, HD, 7)]
    wk_copy = wqkv_copy(D, D, 8)

    w_copies = [
        pltpu.make_async_copy(wo_hbm, wo, sem_w.at[3]),
        pltpu.make_async_copy(wg_hbm, wg, sem_w.at[4]),
        pltpu.make_async_copy(wu_hbm, wu, sem_w.at[5]),
        pltpu.make_async_copy(wd_hbm, wd, sem_w.at[6]),
    ]
    x_copy(0).start()
    wq_copies[0].start()
    wq_copies[1].start()
    wv_copies[0].start()
    wv_copies[1].start()
    x_copy(1).start()
    x_copy(2).start()
    wk_copy.start()

    for t in range(5):
        zs[t] = 0
    vmax_ref[...] = jnp.zeros((8, 128), F32)

    def transpose_w(src_col0, dst_row0):
        for t in range(HD // 128):
            wqvt[dst_row0 + 128 * t:dst_row0 + 128 * (t + 1), :] = (
                wqkv[:, src_col0 + 128 * t:src_col0 + 128 * (t + 1)].T)

    def ln1(row0, dst):
        src = xn.at[pl.ds(row0, MB), :]
        for c in range(MB // 64):
            xf = src[64 * c:64 * (c + 1), :].astype(F32)
            dst[64 * c:64 * (c + 1), :] = _ln(xf).astype(BF16)

    def track_v(v):
        a = jnp.max(jnp.abs(v).reshape(v.shape[0] // 8, 8, v.shape[1]), axis=0)
        a = jnp.maximum(a[:, 0:128], a[:, 128:256])
        a = jnp.broadcast_to(jnp.max(a, axis=0, keepdims=True), (8, 128))
        vmax_ref[...] = jnp.maximum(vmax_ref[...], a)

    def proj_t(row0, n, base, hsrc):
        r = lax.dot_general(wqvt[row0:row0 + n, :], hsrc[...], NT, preferred_element_type=F32)
        if row0 < D:
            qt_b[row0:row0 + n, pl.ds(base, MB)] = (r * QSCALE).astype(BF16)
        else:
            vt_b[row0 - D:row0 - D + n, pl.ds(base, MB)] = r.astype(BF16)
            track_v(r)

    def proj_qv(base, hsrc):
        qv = lax.dot_general(wqvt[...], hsrc[...], NT, preferred_element_type=F32)
        qt_b[:, pl.ds(base, MB)] = (qv[0:D] * QSCALE).astype(BF16)
        vt_b[:, pl.ds(base, MB)] = qv[D:2 * D].astype(BF16)
        track_v(qv[D:2 * D])

    def proj_k(base, hsrc):
        k = jnp.dot(hsrc[...], wqkv[:, D:2 * D], preferred_element_type=F32)
        k_b[pl.ds(base, MB), :] = k.astype(BF16)

    def phase_a(layer):
        def body(t, carry):
            first = jnp.logical_and(layer == 0, t == 0)

            @pl.when(first)
            def _():
                x_copy(1).wait()
                x_copy(2).wait()
                wk_copy.wait()
                for j in range(3, NMB):
                    x_copy(j).start()
                for c in w_copies:
                    c.start()

            @pl.when(jnp.logical_and(layer == 0, t >= 1))
            def _():
                x_copy(2 * t + 1).wait()

            @pl.when(jnp.logical_and(layer == 0, jnp.logical_and(t >= 1, t < NMB // 2 - 1)))
            def _():
                x_copy(2 * t + 2).wait()

            b0 = pl.multiple_of(2 * t * MB, MB)
            b1 = pl.multiple_of(b0 + MB, MB)
            b2 = pl.multiple_of(jnp.minimum(2 * t + 2, NMB - 1) * MB, MB)

            @pl.when(jnp.logical_not(first))
            def _():
                proj_qv(b0, hbufs[0])

            proj_k(b0, hbufs[0])
            ln1(b1, hbufs[1])
            proj_qv(b1, hbufs[1])
            proj_k(b1, hbufs[1])
            ln1(b2, hbufs[0])
            return carry

        lax.fori_loop(0, NMB // 2, body, 0)

    x_copy(0).wait()
    ln1(0, hbufs[0])
    wq_copies[0].wait()
    transpose_w(0, 0)
    wq_copies[1].wait()
    proj_t(0, HD, 0, hbufs[0])
    transpose_w(HD, HD)
    wv_copies[0].wait()
    proj_t(HD, HD, 0, hbufs[0])
    transpose_w(2 * D, D)
    wv_copies[1].wait()
    proj_t(D, HD, 0, hbufs[0])
    transpose_w(2 * D + HD, D + HD)

    @pl.when(zs[0] == 0)
    def _():
        proj_t(D + HD, HD, 0, hbufs[0])

    def attention(blocks):
        p_st = [p.at[zs[0]] for p in pbufs_b]
        good = [None] * len(blocks)
        lsums = {}
        views = []
        for (i, nkb) in blocks:
            r0 = _mo(i * QB, QB)
            k0 = 128 * (nkb - 1)
            views.append((qt_b.at[:, pl.ds(r0, QB)],
                          k_b.at[pl.ds(r0 - k0, k0 + QB), :],
                          vt_b.at[:, pl.ds(r0 - k0, k0 + QB)]))

        lane8 = lax.broadcasted_iota(I32, (1, 8, QB), 2)
        bit0z = (lane8 & 32) == 0
        bit1z = (lane8 & 64) == 0
        blk8 = lane8 >> 5
        t32 = lax.broadcasted_iota(I32, (32, QB), 0)
        new32 = t32 <= (lax.broadcasted_iota(I32, (32, QB), 1) & 31)
        r16 = lax.broadcasted_iota(I32, (16, QB), 0) * 2
        c16 = lax.broadcasted_iota(I32, (16, QB), 1) & 31
        pn32 = (jnp.where(r16 <= c16, U32(0xFFFF), U32(0))
                | jnp.where(r16 + 1 <= c16, U32(0xFFFF0000), U32(0)))

        def lsel(mask, x, y):
            if x is None and y is None:
                return None
            ref = x if y is None else y
            shp = ref.shape
            zero = jnp.zeros((), ref.dtype)
            if shp[0] % 8 == 0:
                x3 = zero if x is None else x.reshape(shp[0] // 8, 8, QB)
                y3 = zero if y is None else y.reshape(shp[0] // 8, 8, QB)
                return jnp.where(mask, x3, y3).reshape(shp)
            return jnp.where(mask[0, 0:shp[0]], zero if x is None else x, zero if y is None else y)

        def xperm(x, j):
            if j & 1:
                x = lsel(bit0z, pltpu.roll(x, 96, 1), pltpu.roll(x, 32, 1))
            if j & 2:
                x = pltpu.roll(x, 64, 1)
            return x

        def pick(a, j):
            return lsel(bit1z, lsel(bit0z, a[j], a[j ^ 1]), lsel(bit0z, a[j ^ 2], a[j ^ 3]))

        def qk(n, g, slot):
            nkb = blocks[n][1]
            qw, kw, _ = views[n]
            cs = slice(128 * g, 128 * (g + 1))
            pref = p_st[slot]
            ys = [xperm(pltpu.bitcast(qw[32 * (4 * g + j):32 * (4 * g + j) + 32, :], U32), j)
                  for j in range(4)]
            for u in (range(4) if nkb == 3 else [(g + k) % 4 for k in range(4)]):
                w = pltpu.bitcast(jnp.concatenate(
                    [lsel(blk8 == (j ^ u), ys[j], None) for j in range(4)], axis=0), BF16)
                dg = 128 * (nkb - 1) + 32 * u
                parts = []
                if nkb == 3:
                    for c in range(2):
                        parts.append(kw[32 * u + 16 * c:32 * u + 16 * c + 16, cs])
                        parts.append(kw[dg + 16 * c:dg + 16 * c + 16, cs])
                    parts.append(kw[32 * u + 32:dg, cs])
                    nmid = 7
                else:
                    parts.append(kw[dg:dg + 32, cs])
                    if dg > 0:
                        parts.append(kw[0:dg, cs])
                    nmid = dg // 32
                s = jnp.dot(jnp.concatenate(parts, axis=0), w, preferred_element_type=F32)
                ls = slice(128 * u, 128 * (u + 1))
                acc = [None, None]

                def put(row0, e, k):
                    pref[row0:row0 + 16, ls] = e.astype(BF16)
                    acc[k] = e if acc[k] is None else acc[k] + e

                for c in range(2):
                    if nkb == 3:
                        f = jnp.where(new32[16 * c:16 * c + 16], s[32 * c + 16:32 * c + 32],
                                      s[32 * c:32 * c + 16])
                    else:
                        f = jnp.where(new32[16 * c:16 * c + 16], s[16 * c:16 * c + 16], NEG)
                    put(16 * c, jnp.exp2(f), c % 2)
                m0 = 64 if nkb == 3 else 32
                for c in range(2 * nmid):
                    put(32 + 16 * c, jnp.exp2(s[m0 + 16 * c:m0 + 16 * c + 16]), c % 2)
                t = acc[0] + acc[1]
                lsums[(slot, u)] = jnp.sum(t[0:8] + t[8:16], axis=0, keepdims=True)

        def pv(n, g, slot):
            nkb = blocks[n][1]
            vw = views[n][2]
            ots = []
            for j in range(4):
                pref = pbufs_u[slot].at[zs[1 + j]]

                def blk(u, b):
                    ls = slice(128 * u, 128 * (u + 1))
                    if nkb == 3:
                        be = b - u
                        if be < 0 or be > 8:
                            return None
                        if be == 0:
                            f = pref[0:16, ls]
                            return f ^ (f & pn32)
                        if be == 8:
                            return pref[0:16, ls] & pn32
                        return pref[16 * be:16 * be + 16, ls]
                    nb = 4 * (nkb - 1) + u
                    if b > nb:
                        return None
                    if b == nb:
                        return pref[0:16, ls]
                    return pref[16 * (b + 1):16 * (b + 2), ls]

                tiles = []
                for b in range(4 * nkb):
                    o = pick([blk(u, b) for u in range(4)], j)
                    tiles.append(jnp.zeros((16, QB), U32) if o is None else o)
                ots.append(jnp.dot(vw[32 * (4 * g + j):32 * (4 * g + j + 1), :],
                                   pltpu.bitcast(jnp.concatenate(tiles, axis=0), BF16),
                                   preferred_element_type=F32))
            lu = [lsums.pop((slot, u)) for u in range(4)]
            for j in range(4):
                h = 4 * g + j
                l = pick(lu, j)
                ok = (l >= L_LO) & (l <= L_HI)
                good[n] = ok if good[n] is None else (good[n] & ok)
                o = xperm(ots[j] * _recip(l), j)
                otbufs[n][32 * (h % 16):32 * (h % 16) + 32,
                          128 * (h // 16):128 * (h // 16) + 128] = o.astype(BF16)

        seq = [(n, g) for n in range(len(blocks)) for g in range(8)]
        for s in range(len(seq) + 2):
            if s < len(seq):
                qk(seq[s][0], seq[s][1], s % 3)
            if s >= 2:
                pv(seq[s - 2][0], seq[s - 2][1], (s - 2) % 3)
        v_ok = vmax_ref[0:1, :] <= V_HI
        for n in range(len(blocks)):
            flag[n] = jnp.min(jnp.where(good[n] & v_ok, 1, 0))

    def attention_safe(i, ow):
        r0 = _mo(i * QB, QB)
        start = pl.multiple_of(jnp.maximum(i - 2, 0) * QB, QB)
        qw = qt_b.at[:, pl.ds(r0, QB)]
        kw = k_b.at[pl.ds(start, 3 * QB), :]
        vw = vt_b.at[:, pl.ds(start, 3 * QB)]
        key = lax.broadcasted_iota(I32, (3 * QB, QB), 0) + start
        qry = lax.broadcasted_iota(I32, (3 * QB, QB), 1) + r0
        valid = (qry - key >= 0) & (qry - key < WIN)
        drow = lax.broadcasted_iota(I32, (128, QB), 0)

        def head(h, carry):
            g0 = pl.multiple_of((h // 4) * 128, 128)
            j0 = (h % 4) * 32
            q4 = qw[pl.ds(g0, 128), :].astype(F32)
            w = jnp.where((drow >= j0) & (drow < j0 + 32), q4, 0.0).astype(BF16)
            s = jnp.dot(kw[:, pl.ds(g0, 128)], w, preferred_element_type=F32)
            s = jnp.where(valid, s, NEG)
            m = jnp.max(s, axis=0, keepdims=True)
            p = jnp.exp2(s - m).astype(BF16)
            l = jnp.sum(p.astype(F32), axis=0, keepdims=True)
            vt = vw[pl.ds(pl.multiple_of(h * 32, 32), 32), :]
            o = jnp.dot(vt, p, preferred_element_type=F32) * (1.0 / l)
            ow[pl.ds(pl.multiple_of((h % 16) * 32, 32), 32),
               pl.ds(pl.multiple_of((h // 16) * 128, 128), 128)] = o.astype(BF16)
            return carry

        lax.fori_loop(0, NH, head, 0)

    def out_proj(n, xsrc, x1dst):
        ow = ot_b.at[n]
        o = jnp.concatenate([ow[:, 0:128], ow[:, 128:256]], axis=0)
        y = lax.dot_general(o, wo[...], TN, preferred_element_type=F32)
        x1dst[...] = (xsrc[...].astype(F32) + y).astype(BF16)

    def ln2(b, x1src, x2dst):
        CH = 16
        rb = _mo(b * QB, QB)
        wr = wr_ref[...].astype(F32).reshape(1, D)
        wsum = jnp.sum(wr, axis=-1, keepdims=True)
        bm = None
        bi = None
        sub = lax.broadcasted_iota(I32, (8, 1), 0)
        for c in range(QB // CH):
            x1 = x1src[CH * c:CH * (c + 1), :].astype(F32)
            m, rs = _ln_stats(x1)
            x2dst[CH * c:CH * (c + 1), :] = (x1 * (1.0 + rs) - m * rs).astype(BF16)
            r = _rnd(rs * (jnp.sum(x1 * wr, axis=-1, keepdims=True) - m * wsum))
            for t in range(CH // 8):
                rt = r[8 * t:8 * t + 8]
                it = sub + (rb + CH * c + 8 * t)
                if bm is None:
                    bm, bi = rt, it
                else:
                    better = rt > bm
                    bm = jnp.where(better, rt, bm)
                    bi = jnp.where(better, it, bi)
        bmax_ref[b] = jnp.broadcast_to(bm, (8, 128))
        bidx_ref[b] = jnp.broadcast_to(bi, (8, 128))

    def checks(i0):
        def one(n, carry):
            @pl.when(flag[n] == 0)
            def _():
                rb = pl.multiple_of((i0 + n) * QB, QB)
                attention_safe(i0 + n, ot_b.at[n])
                out_proj(n, xn.at[pl.ds(rb, QB), :], x1_b.at[pl.ds(rb, QB), :])
            return carry

        @pl.when(flag[0] + flag[1] < 2)
        def _():
            lax.fori_loop(0, 2, one, 0)

    def out_copy(b):
        return pltpu.make_async_copy(xn.at[pl.ds(b * QB, QB), :],
                                     out_hbm.at[pl.ds(b * QB, QB), :], sem_o.at[0])

    def phase_b(layer):
        attention([(0, 1), (1, 2)])
        out_proj(0, xn.at[0:QB, :], x1_b.at[0:QB, :])
        out_proj(1, xn.at[QB:2 * QB, :], x1_b.at[QB:2 * QB, :])

        def body(t, carry):
            i0 = 2 * t
            checks(i0 - 2)

            @pl.when(jnp.logical_and(layer == 1, t >= 2))
            def _():
                out_copy(i0 - 4).start()
                out_copy(i0 - 3).start()

            @pl.when(t < NQB // 2)
            def _():
                r2 = pl.multiple_of((i0 - 2) * QB, QB)
                xv = xn.at[pl.ds(r2, 4 * QB), :]
                x1v = x1_b.at[pl.ds(r2, 4 * QB), :]
                ln2(i0 - 2, x1v.at[0:QB, :], xv.at[0:QB, :])
                ln2(i0 - 1, x1v.at[QB:2 * QB, :], xv.at[QB:2 * QB, :])
                attention([(i0, 3), (i0 + 1, 3)])
                out_proj(0, xv.at[2 * QB:3 * QB, :], x1v.at[2 * QB:3 * QB, :])
                out_proj(1, xv.at[3 * QB:4 * QB, :], x1v.at[3 * QB:4 * QB, :])
            return carry

        lax.fori_loop(1, NQB // 2 + 1, body, 0)
        for b in (NQB - 2, NQB - 1):
            ln2(b, x1_b.at[b * QB:(b + 1) * QB, :], xn.at[b * QB:(b + 1) * QB, :])

        @pl.when(layer == 1)
        def _():
            out_copy(NQB - 2).start()
            out_copy(NQB - 1).start()

    def moe(layer):
        rm = bmax_ref[:, :, 0:1]
        ri = bidx_ref[:, :, 0:1]
        gm = jnp.max(jnp.max(rm, axis=0), axis=0, keepdims=True)
        idx = jnp.minimum(jnp.min(jnp.where(rm == gm, ri, BIG)), S - 1)
        b16 = pl.multiple_of((idx // 16) * 16, 16)
        ln1(0, hbufs[0])
        x1c = x1_b[pl.ds(b16, 16), :].astype(F32)
        mu, rs = _ln_stats(x1c)
        h2c = _rnd(x1c * rs - mu * rs)
        hb = h2c.astype(BF16)
        g = _rnd(jnp.dot(hb, wg[...], preferred_element_type=F32))
        u = _rnd(jnp.dot(hb, wu[...], preferred_element_type=F32))
        g = _rnd(g * _rnd(jax.nn.sigmoid(g)))
        act = (g * u).astype(BF16)
        y = _rnd(jnp.dot(act, wd[...], preferred_element_type=F32))
        y = _rnd(y * _rnd(jax.nn.sigmoid(gm)))
        x2n = x1c + _rnd(h2c + y)

        @pl.when(layer == 1)
        def _():
            for b in range(NQB):
                out_copy(b).wait()

        cur = xn[pl.ds(b16, 16), :].astype(F32)
        sel = lax.broadcasted_iota(I32, (16, D), 0) == (idx - b16)
        xn[pl.ds(b16, 16), :] = jnp.where(sel, x2n, cur).astype(BF16)

        @pl.when(jnp.logical_and(layer == 0, idx < MB))
        def _():
            ln1(0, hbufs[0])

        @pl.when(layer == 1)
        def _():
            cp = pltpu.make_async_copy(xn.at[pl.ds(b16, 16), :],
                                       out_hbm.at[pl.ds(b16, 16), :], sem_o.at[1])
            cp.start()
            cp.wait()

    def layer_body(layer, carry):
        phase_a(layer)

        @pl.when(layer == 0)
        def _():
            w_copies[0].wait()

        phase_b(layer)

        @pl.when(layer == 0)
        def _():
            for c in w_copies[1:]:
                c.wait()

        moe(layer)

        vmax_ref[...] = jnp.zeros((8, 128), F32)
        return carry

    lax.fori_loop(0, 2, layer_body, 0)


@jax.jit
def pallas_interleave_layers__sliding_block__moe_arch_mod__prompt_kernel(
    A_x: jax.Array,
    A_wqkv: jax.Array,
    A_wo: jax.Array,
    B_x: jax.Array,
    B_w_r: jax.Array,
    B_w_gate: jax.Array,
    B_w_up: jax.Array,
    B_w_down: jax.Array,
):
    del B_x
    hbm = pl.BlockSpec(memory_space=pl.ANY)
    scratch = [
        pltpu.VMEM((S // 2, D), U32),
        pltpu.VMEM((S // 2, D), U32),
        pltpu.VMEM((MB // 2, D), U32),
        pltpu.VMEM((MB // 2, D), U32),
        pltpu.VMEM((D // 2, S), U32),
        pltpu.VMEM((S // 2, D), U32),
        pltpu.VMEM((D // 2, S), U32),
        pltpu.VMEM((D // 2, 3 * D), U32),
        pltpu.VMEM((D, D), U32),
        pltpu.VMEM((D // 2, D), U32),
        pltpu.VMEM((D // 2, FF), U32),
        pltpu.VMEM((D // 2, FF), U32),
        pltpu.VMEM((FF // 2, D), U32),
        pltpu.VMEM((1, 128, 512), U32),
        pltpu.VMEM((1, 128, 512), U32),
        pltpu.VMEM((1, 128, 512), U32),
        pltpu.VMEM((2, 256, 256), U32),
        pltpu.VMEM((8, 128), F32),
        pltpu.VMEM((NQB, 8, 128), F32),
        pltpu.VMEM((NQB, 8, 128), I32),
        pltpu.SMEM((5,), I32),
        pltpu.SMEM((2,), I32),
        pltpu.SemaphoreType.DMA((NMB,)),
        pltpu.SemaphoreType.DMA((9,)),
        pltpu.SemaphoreType.DMA((2,)),
    ]
    out = pl.pallas_call(
        _kernel,
        out_shape=jax.ShapeDtypeStruct((S, D), BF16),
        in_specs=[hbm, hbm, hbm, pl.BlockSpec(memory_space=pltpu.VMEM), hbm, hbm, hbm],
        out_specs=hbm,
        scratch_shapes=scratch,
        compiler_params=pltpu.CompilerParams(vmem_limit_bytes=110 * 1024 * 1024,
                                             disable_bounds_checks=True,
                                             disable_semaphore_checks=True),
        name="swa_moe_fused",
    )(A_x.reshape(S, D), A_wqkv, A_wo, B_w_r, B_w_gate, B_w_up, B_w_down)
    return out.reshape(1, S, D)
```

```python
import math

import jax
import jax.numpy as jnp
from jax import lax
import jax.experimental.pallas as pl
import jax.experimental.pallas.tpu as pltpu

S = 2048
D = 1024
NH = 32
DH = 32
WIN = 256
FF = 3584
QB = 128
NQB = S // QB
MB = 256
NMB = S // MB
EPS = 1e-5
QSCALE = (DH ** -0.5) * math.log2(math.e)
NEG = -1e30
BIG = 2 ** 30
L_LO = 2.0 ** -64
L_HI = 2.0 ** 64
V_HI = 2.0 ** 60

F32 = jnp.float32
BF16 = jnp.bfloat16
U32 = jnp.uint32
I32 = jnp.int32

NT = (((1,), (1,)), ((), ()))
TN = (((0,), (0,)), ((), ()))


def _rnd(v):
    return v.astype(BF16).astype(F32)


def _ln(xf):
    m = jnp.mean(xf, axis=-1, keepdims=True)
    xc = xf - m
    v = jnp.mean(xc * xc, axis=-1, keepdims=True)
    return xc * lax.rsqrt(v + EPS)


def _ln_stats(xf):
    m = jnp.sum(xf, axis=-1, keepdims=True) * (1.0 / D)
    v = jnp.sum(xf * xf, axis=-1, keepdims=True) * (1.0 / D) - m * m
    return m, lax.rsqrt(jnp.maximum(v, 0.0) + EPS)


def _recip(l):
    r = pl.reciprocal(l, approx=True)
    return r * (2.0 - l * r)


def _mo(v, m):
    return v if isinstance(v, int) else pl.multiple_of(v, m)


def _kernel(x_hbm, wqkv_hbm, wo_hbm, wr_ref, wg_hbm, wu_hbm, wd_hbm, out_hbm,
            xn_u, x1_u, h0_u, h1_u, qt_u, k_u, vt_u,
            wqkv_u, wqvt_u, wo_u, wg_u, wu_u, wd_u,
            p0, p1, p2, ot_u, vmax_ref, bmax_ref, bidx_ref, zs, flag,
            sem_x, sem_w, sem_o):
    xn = xn_u.bitcast(BF16)
    x1_b = x1_u.bitcast(BF16)
    hbufs = (h0_u.bitcast(BF16), h1_u.bitcast(BF16))
    qt_b = qt_u.bitcast(BF16)
    k_b = k_u.bitcast(BF16)
    vt_b = vt_u.bitcast(BF16)
    wqkv = wqkv_u.bitcast(BF16)
    wqvt = wqvt_u.bitcast(BF16)
    wo = wo_u.bitcast(BF16)
    wg = wg_u.bitcast(BF16)
    wu = wu_u.bitcast(BF16)
    wd = wd_u.bitcast(BF16)
    ot_b = ot_u.bitcast(BF16)
    otbufs = (ot_b.at[0], ot_b.at[1])
    pbufs_u = (p0, p1, p2)
    pbufs_b = tuple(p.bitcast(BF16) for p in pbufs_u)

    def x_copy(j):
        return pltpu.make_async_copy(x_hbm.at[pl.ds(j * MB, MB), :],
                                     xn.at[pl.ds(j * MB, MB), :], sem_x.at[j])

    def wqkv_copy(c0, n, k):
        return pltpu.make_async_copy(wqkv_hbm.at[:, pl.ds(c0, n)],
                                     wqkv.at[:, pl.ds(c0, n)], sem_w.at[k])

    HD = D // 2
    wq_copies = [wqkv_copy(0, HD, 0), wqkv_copy(HD, HD, 1)]
    wv_copies = [wqkv_copy(2 * D, HD, 2), wqkv_copy(2 * D + HD, HD, 7)]
    wk_copy = wqkv_copy(D, D, 8)

    w_copies = [
        pltpu.make_async_copy(wo_hbm, wo, sem_w.at[3]),
        pltpu.make_async_copy(wg_hbm, wg, sem_w.at[4]),
        pltpu.make_async_copy(wu_hbm, wu, sem_w.at[5]),
        pltpu.make_async_copy(wd_hbm, wd, sem_w.at[6]),
    ]
    x_copy(0).start()
    wq_copies[0].start()
    wq_copies[1].start()
    wv_copies[0].start()
    wv_copies[1].start()
    x_copy(1).start()
    x_copy(2).start()
    wk_copy.start()

    for t in range(5):
        zs[t] = 0
    vmax_ref[...] = jnp.zeros((8, 128), F32)

    def transpose_w(src_col0, dst_row0):
        for t in range(HD // 128):
            wqvt[dst_row0 + 128 * t:dst_row0 + 128 * (t + 1), :] = (
                wqkv[:, src_col0 + 128 * t:src_col0 + 128 * (t + 1)].T)

    def ln1(row0, dst):
        src = xn.at[pl.ds(row0, MB), :]
        for c in range(MB // 64):
            xf = src[64 * c:64 * (c + 1), :].astype(F32)
            dst[64 * c:64 * (c + 1), :] = _ln(xf).astype(BF16)

    def track_v(v):
        a = jnp.max(jnp.abs(v).reshape(v.shape[0] // 8, 8, v.shape[1]), axis=0)
        a = jnp.maximum(a[:, 0:128], a[:, 128:256])
        a = jnp.broadcast_to(jnp.max(a, axis=0, keepdims=True), (8, 128))
        vmax_ref[...] = jnp.maximum(vmax_ref[...], a)

    def proj_t(row0, n, base, hsrc):
        r = lax.dot_general(wqvt[row0:row0 + n, :], hsrc[...], NT, preferred_element_type=F32)
        if row0 < D:
            qt_b[row0:row0 + n, pl.ds(base, MB)] = (r * QSCALE).astype(BF16)
        else:
            vt_b[row0 - D:row0 - D + n, pl.ds(base, MB)] = r.astype(BF16)
            track_v(r)

    def proj_qv(base, hsrc):
        qv = lax.dot_general(wqvt[...], hsrc[...], NT, preferred_element_type=F32)
        qt_b[:, pl.ds(base, MB)] = (qv[0:D] * QSCALE).astype(BF16)
        vt_b[:, pl.ds(base, MB)] = qv[D:2 * D].astype(BF16)
        track_v(qv[D:2 * D])

    def proj_k(base, hsrc):
        k = jnp.dot(hsrc[...], wqkv[:, D:2 * D], preferred_element_type=F32)
        k_b[pl.ds(base, MB), :] = k.astype(BF16)

    def phase_a(layer):
        def body(t, carry):
            first = jnp.logical_and(layer == 0, t == 0)

            @pl.when(jnp.logical_and(layer == 0, t >= 1))
            def _():
                x_copy(2 * t + 1).wait()

                @pl.when(t < NMB // 2 - 1)
                def _():
                    x_copy(2 * t + 2).wait()

            b0 = pl.multiple_of(2 * t * MB, MB)
            b1 = pl.multiple_of(b0 + MB, MB)
            b2 = pl.multiple_of(jnp.minimum(2 * t + 2, NMB - 1) * MB, MB)

            @pl.when(jnp.logical_not(first))
            def _():
                proj_qv(b0, hbufs[0])

            proj_k(b0, hbufs[0])
            ln1(b1, hbufs[1])
            proj_qv(b1, hbufs[1])
            proj_k(b1, hbufs[1])
            ln1(b2, hbufs[0])
            return carry

        lax.fori_loop(0, NMB // 2, body, 0)

    x_copy(0).wait()
    ln1(0, hbufs[0])
    wq_copies[0].wait()
    transpose_w(0, 0)
    wq_copies[1].wait()
    proj_t(0, HD, 0, hbufs[0])
    transpose_w(HD, HD)
    wv_copies[0].wait()
    proj_t(HD, HD, 0, hbufs[0])
    transpose_w(2 * D, D)
    wv_copies[1].wait()
    proj_t(D, HD, 0, hbufs[0])
    transpose_w(2 * D + HD, D + HD)

    @pl.when(zs[0] == 0)
    def _():
        proj_t(D + HD, HD, 0, hbufs[0])

    x_copy(1).wait()
    x_copy(2).wait()
    wk_copy.wait()
    for j in range(3, NMB):
        x_copy(j).start()
    for c in w_copies:
        c.start()

    def attention(blocks):
        p_st = [p.at[zs[0]] for p in pbufs_b]
        good = [None] * len(blocks)
        lsums = {}
        views = []
        for (i, nkb) in blocks:
            r0 = _mo(i * QB, QB)
            k0 = 128 * (nkb - 1)
            views.append((qt_b.at[:, pl.ds(r0, QB)],
                          k_b.at[pl.ds(r0 - k0, k0 + QB), :],
                          vt_b.at[:, pl.ds(r0 - k0, k0 + QB)]))

        lane8 = lax.broadcasted_iota(I32, (1, 8, QB), 2)
        bit0z = (lane8 & 32) == 0
        bit1z = (lane8 & 64) == 0
        blk8 = lane8 >> 5
        t32 = lax.broadcasted_iota(I32, (32, QB), 0)
        new32 = t32 <= (lax.broadcasted_iota(I32, (32, QB), 1) & 31)
        r16 = lax.broadcasted_iota(I32, (16, QB), 0) * 2
        c16 = lax.broadcasted_iota(I32, (16, QB), 1) & 31
        pn32 = (jnp.where(r16 <= c16, U32(0xFFFF), U32(0))
                | jnp.where(r16 + 1 <= c16, U32(0xFFFF0000), U32(0)))

        def lsel(mask, x, y):
            if x is None and y is None:
                return None
            ref = x if y is None else y
            shp = ref.shape
            zero = jnp.zeros((), ref.dtype)
            if shp[0] % 8 == 0:
                x3 = zero if x is None else x.reshape(shp[0] // 8, 8, QB)
                y3 = zero if y is None else y.reshape(shp[0] // 8, 8, QB)
                return jnp.where(mask, x3, y3).reshape(shp)
            return jnp.where(mask[0, 0:shp[0]], zero if x is None else x, zero if y is None else y)

        def xperm(x, j):
            if j & 1:
                x = lsel(bit0z, pltpu.roll(x, 96, 1), pltpu.roll(x, 32, 1))
            if j & 2:
                x = pltpu.roll(x, 64, 1)
            return x

        def pick(a, j):
            return lsel(bit1z, lsel(bit0z, a[j], a[j ^ 1]), lsel(bit0z, a[j ^ 2], a[j ^ 3]))

        def qk(n, g, slot):
            nkb = blocks[n][1]
            qw, kw, _ = views[n]
            cs = slice(128 * g, 128 * (g + 1))
            pref = p_st[slot]
            ys = [xperm(pltpu.bitcast(qw[32 * (4 * g + j):32 * (4 * g + j) + 32, :], U32), j)
                  for j in range(4)]
            for u in (range(4) if nkb == 3 else [(g + k) % 4 for k in range(4)]):
                w = pltpu.bitcast(jnp.concatenate(
                    [lsel(blk8 == (j ^ u), ys[j], None) for j in range(4)], axis=0), BF16)
                dg = 128 * (nkb - 1) + 32 * u
                parts = []
                if nkb == 3:
                    for c in range(2):
                        parts.append(kw[32 * u + 16 * c:32 * u + 16 * c + 16, cs])
                        parts.append(kw[dg + 16 * c:dg + 16 * c + 16, cs])
                    parts.append(kw[32 * u + 32:dg, cs])
                    nmid = 7
                else:
                    parts.append(kw[dg:dg + 32, cs])
                    if dg > 0:
                        parts.append(kw[0:dg, cs])
                    nmid = dg // 32
                s = jnp.dot(jnp.concatenate(parts, axis=0), w, preferred_element_type=F32)
                ls = slice(128 * u, 128 * (u + 1))
                acc = [None, None]

                def put(row0, e, k):
                    pref[row0:row0 + 16, ls] = e.astype(BF16)
                    acc[k] = e if acc[k] is None else acc[k] + e

                for c in range(2):
                    if nkb == 3:
                        f = jnp.where(new32[16 * c:16 * c + 16], s[32 * c + 16:32 * c + 32],
                                      s[32 * c:32 * c + 16])
                    else:
                        f = jnp.where(new32[16 * c:16 * c + 16], s[16 * c:16 * c + 16], NEG)
                    put(16 * c, jnp.exp2(f), c % 2)
                m0 = 64 if nkb == 3 else 32
                for c in range(2 * nmid):
                    put(32 + 16 * c, jnp.exp2(s[m0 + 16 * c:m0 + 16 * c + 16]), c % 2)
                t = acc[0] + acc[1]
                lsums[(slot, u)] = jnp.sum(t[0:8] + t[8:16], axis=0, keepdims=True)

        def pv(n, g, slot):
            nkb = blocks[n][1]
            vw = views[n][2]
            ots = []
            for j in range(4):
                pref = pbufs_u[slot].at[zs[1 + j]]

                def blk(u, b):
                    ls = slice(128 * u, 128 * (u + 1))
                    if nkb == 3:
                        be = b - u
                        if be < 0 or be > 8:
                            return None
                        if be == 0:
                            f = pref[0:16, ls]
                            return f ^ (f & pn32)
                        if be == 8:
                            return pref[0:16, ls] & pn32
                        return pref[16 * be:16 * be + 16, ls]
                    nb = 4 * (nkb - 1) + u
                    if b > nb:
                        return None
                    if b == nb:
                        return pref[0:16, ls]
                    return pref[16 * (b + 1):16 * (b + 2), ls]

                tiles = []
                for b in range(4 * nkb):
                    o = pick([blk(u, b) for u in range(4)], j)
                    tiles.append(jnp.zeros((16, QB), U32) if o is None else o)
                ots.append(jnp.dot(vw[32 * (4 * g + j):32 * (4 * g + j + 1), :],
                                   pltpu.bitcast(jnp.concatenate(tiles, axis=0), BF16),
                                   preferred_element_type=F32))
            lu = [lsums.pop((slot, u)) for u in range(4)]
            for j in range(4):
                h = 4 * g + j
                l = pick(lu, j)
                ok = (l >= L_LO) & (l <= L_HI)
                good[n] = ok if good[n] is None else (good[n] & ok)
                o = xperm(ots[j] * _recip(l), j)
                otbufs[n][32 * (h % 16):32 * (h % 16) + 32,
                          128 * (h // 16):128 * (h // 16) + 128] = o.astype(BF16)

        seq = [(n, g) for n in range(len(blocks)) for g in range(8)]
        for s in range(len(seq) + 2):
            if s < len(seq):
                qk(seq[s][0], seq[s][1], s % 3)
            if s >= 2:
                pv(seq[s - 2][0], seq[s - 2][1], (s - 2) % 3)
        v_ok = vmax_ref[0:1, :] <= V_HI
        for n in range(len(blocks)):
            flag[n] = jnp.min(jnp.where(good[n] & v_ok, 1, 0))

    def attention_safe(i, ow):
        r0 = _mo(i * QB, QB)
        start = pl.multiple_of(jnp.maximum(i - 2, 0) * QB, QB)
        qw = qt_b.at[:, pl.ds(r0, QB)]
        kw = k_b.at[pl.ds(start, 3 * QB), :]
        vw = vt_b.at[:, pl.ds(start, 3 * QB)]
        key = lax.broadcasted_iota(I32, (3 * QB, QB), 0) + start
        qry = lax.broadcasted_iota(I32, (3 * QB, QB), 1) + r0
        valid = (qry - key >= 0) & (qry - key < WIN)
        drow = lax.broadcasted_iota(I32, (128, QB), 0)

        def head(h, carry):
            g0 = pl.multiple_of((h // 4) * 128, 128)
            j0 = (h % 4) * 32
            q4 = qw[pl.ds(g0, 128), :].astype(F32)
            w = jnp.where((drow >= j0) & (drow < j0 + 32), q4, 0.0).astype(BF16)
            s = jnp.dot(kw[:, pl.ds(g0, 128)], w, preferred_element_type=F32)
            s = jnp.where(valid, s, NEG)
            m = jnp.max(s, axis=0, keepdims=True)
            p = jnp.exp2(s - m).astype(BF16)
            l = jnp.sum(p.astype(F32), axis=0, keepdims=True)
            vt = vw[pl.ds(pl.multiple_of(h * 32, 32), 32), :]
            o = jnp.dot(vt, p, preferred_element_type=F32) * (1.0 / l)
            ow[pl.ds(pl.multiple_of((h % 16) * 32, 32), 32),
               pl.ds(pl.multiple_of((h // 16) * 128, 128), 128)] = o.astype(BF16)
            return carry

        lax.fori_loop(0, NH, head, 0)

    def out_proj(n, xsrc, x1dst):
        ow = ot_b.at[n]
        o = jnp.concatenate([ow[:, 0:128], ow[:, 128:256]], axis=0)
        y = lax.dot_general(o, wo[...], TN, preferred_element_type=F32)
        x1dst[...] = (xsrc[...].astype(F32) + y).astype(BF16)

    def ln2(b, x1src, x2dst):
        CH = 16
        rb = _mo(b * QB, QB)
        wr = wr_ref[...].astype(F32).reshape(1, D)
        wsum = jnp.sum(wr, axis=-1, keepdims=True)
        bm = None
        bi = None
        sub = lax.broadcasted_iota(I32, (8, 1), 0)
        for c in range(QB // CH):
            x1 = x1src[CH * c:CH * (c + 1), :].astype(F32)
            m, rs = _ln_stats(x1)
            x2dst[CH * c:CH * (c + 1), :] = (x1 * (1.0 + rs) - m * rs).astype(BF16)
            r = _rnd(rs * (jnp.sum(x1 * wr, axis=-1, keepdims=True) - m * wsum))
            for t in range(CH // 8):
                rt = r[8 * t:8 * t + 8]
                it = sub + (rb + CH * c + 8 * t)
                if bm is None:
                    bm, bi = rt, it
                else:
                    better = rt > bm
                    bm = jnp.where(better, rt, bm)
                    bi = jnp.where(better, it, bi)
        bmax_ref[b] = jnp.broadcast_to(bm, (8, 128))
        bidx_ref[b] = jnp.broadcast_to(bi, (8, 128))

    def checks(i0):
        def one(n, carry):
            @pl.when(flag[n] == 0)
            def _():
                rb = pl.multiple_of((i0 + n) * QB, QB)
                attention_safe(i0 + n, ot_b.at[n])
                out_proj(n, xn.at[pl.ds(rb, QB), :], x1_b.at[pl.ds(rb, QB), :])
            return carry

        @pl.when(flag[0] + flag[1] < 2)
        def _():
            lax.fori_loop(0, 2, one, 0)

    def out_copy(b):
        return pltpu.make_async_copy(xn.at[pl.ds(b * QB, QB), :],
                                     out_hbm.at[pl.ds(b * QB, QB), :], sem_o.at[0])

    def phase_b(layer):
        attention([(0, 1), (1, 2)])
        out_proj(0, xn.at[0:QB, :], x1_b.at[0:QB, :])
        out_proj(1, xn.at[QB:2 * QB, :], x1_b.at[QB:2 * QB, :])

        def body(t, carry):
            i0 = 2 * t
            checks(i0 - 2)

            @pl.when(jnp.logical_and(layer == 1, t >= 2))
            def _():
                out_copy(i0 - 4).start()
                out_copy(i0 - 3).start()

            @pl.when(t < NQB // 2)
            def _():
                r2 = pl.multiple_of((i0 - 2) * QB, QB)
                xv = xn.at[pl.ds(r2, 4 * QB), :]
                x1v = x1_b.at[pl.ds(r2, 4 * QB), :]
                ln2(i0 - 2, x1v.at[0:QB, :], xv.at[0:QB, :])
                ln2(i0 - 1, x1v.at[QB:2 * QB, :], xv.at[QB:2 * QB, :])
                attention([(i0, 3), (i0 + 1, 3)])
                out_proj(0, xv.at[2 * QB:3 * QB, :], x1v.at[2 * QB:3 * QB, :])
                out_proj(1, xv.at[3 * QB:4 * QB, :], x1v.at[3 * QB:4 * QB, :])
            return carry

        lax.fori_loop(1, NQB // 2 + 1, body, 0)
        for b in (NQB - 2, NQB - 1):
            ln2(b, x1_b.at[b * QB:(b + 1) * QB, :], xn.at[b * QB:(b + 1) * QB, :])

        @pl.when(layer == 1)
        def _():
            out_copy(NQB - 2).start()
            out_copy(NQB - 1).start()

    def moe(layer):
        rm = bmax_ref[:, :, 0:1]
        ri = bidx_ref[:, :, 0:1]
        gm = jnp.max(jnp.max(rm, axis=0), axis=0, keepdims=True)
        idx = jnp.minimum(jnp.min(jnp.where(rm == gm, ri, BIG)), S - 1)
        b16 = pl.multiple_of((idx // 16) * 16, 16)
        ln1(0, hbufs[0])
        x1c = x1_b[pl.ds(b16, 16), :].astype(F32)
        mu, rs = _ln_stats(x1c)
        h2c = _rnd(x1c * rs - mu * rs)
        hb = h2c.astype(BF16)
        g = _rnd(jnp.dot(hb, wg[...], preferred_element_type=F32))
        u = _rnd(jnp.dot(hb, wu[...], preferred_element_type=F32))
        g = _rnd(g * _rnd(jax.nn.sigmoid(g)))
        act = (g * u).astype(BF16)
        y = _rnd(jnp.dot(act, wd[...], preferred_element_type=F32))
        y = _rnd(y * _rnd(jax.nn.sigmoid(gm)))
        x2n = x1c + _rnd(h2c + y)

        @pl.when(layer == 1)
        def _():
            for b in range(NQB):
                out_copy(b).wait()

        cur = xn[pl.ds(b16, 16), :].astype(F32)
        sel = lax.broadcasted_iota(I32, (16, D), 0) == (idx - b16)
        xn[pl.ds(b16, 16), :] = jnp.where(sel, x2n, cur).astype(BF16)

        @pl.when(jnp.logical_and(layer == 0, idx < MB))
        def _():
            ln1(0, hbufs[0])

        @pl.when(layer == 1)
        def _():
            cp = pltpu.make_async_copy(xn.at[pl.ds(b16, 16), :],
                                       out_hbm.at[pl.ds(b16, 16), :], sem_o.at[1])
            cp.start()
            cp.wait()

    def layer_body(layer, carry):
        phase_a(layer)

        @pl.when(layer == 0)
        def _():
            w_copies[0].wait()

        phase_b(layer)

        @pl.when(layer == 0)
        def _():
            for c in w_copies[1:]:
                c.wait()

        moe(layer)

        vmax_ref[...] = jnp.zeros((8, 128), F32)
        return carry

    lax.fori_loop(0, 2, layer_body, 0)


@jax.jit
def pallas_interleave_layers__sliding_block__moe_arch_mod__prompt_kernel(
    A_x: jax.Array,
    A_wqkv: jax.Array,
    A_wo: jax.Array,
    B_x: jax.Array,
    B_w_r: jax.Array,
    B_w_gate: jax.Array,
    B_w_up: jax.Array,
    B_w_down: jax.Array,
):
    del B_x
    hbm = pl.BlockSpec(memory_space=pl.ANY)
    scratch = [
        pltpu.VMEM((S // 2, D), U32),
        pltpu.VMEM((S // 2, D), U32),
        pltpu.VMEM((MB // 2, D), U32),
        pltpu.VMEM((MB // 2, D), U32),
        pltpu.VMEM((D // 2, S), U32),
        pltpu.VMEM((S // 2, D), U32),
        pltpu.VMEM((D // 2, S), U32),
        pltpu.VMEM((D // 2, 3 * D), U32),
        pltpu.VMEM((D, D), U32),
        pltpu.VMEM((D // 2, D), U32),
        pltpu.VMEM((D // 2, FF), U32),
        pltpu.VMEM((D // 2, FF), U32),
        pltpu.VMEM((FF // 2, D), U32),
        pltpu.VMEM((1, 128, 512), U32),
        pltpu.VMEM((1, 128, 512), U32),
        pltpu.VMEM((1, 128, 512), U32),
        pltpu.VMEM((2, 256, 256), U32),
        pltpu.VMEM((8, 128), F32),
        pltpu.VMEM((NQB, 8, 128), F32),
        pltpu.VMEM((NQB, 8, 128), I32),
        pltpu.SMEM((5,), I32),
        pltpu.SMEM((2,), I32),
        pltpu.SemaphoreType.DMA((NMB,)),
        pltpu.SemaphoreType.DMA((9,)),
        pltpu.SemaphoreType.DMA((2,)),
    ]
    out = pl.pallas_call(
        _kernel,
        out_shape=jax.ShapeDtypeStruct((S, D), BF16),
        in_specs=[hbm, hbm, hbm, pl.BlockSpec(memory_space=pltpu.VMEM), hbm, hbm, hbm],
        out_specs=hbm,
        scratch_shapes=scratch,
        compiler_params=pltpu.CompilerParams(vmem_limit_bytes=110 * 1024 * 1024,
                                             disable_bounds_checks=True,
                                             disable_semaphore_checks=True),
        name="swa_moe_fused",
    )(A_x.reshape(S, D), A_wqkv, A_wo, B_w_r, B_w_gate, B_w_up, B_w_down)
    return out.reshape(1, S, D)
```
